```python
import jax
import jax.numpy as jnp

def _softmax(x, axis=-1):
    return jax.nn.softmax(x, axis=axis)
def _gelu(x):
    return jax.nn.gelu(x, approximate=True)
def _silu(x):
    return jax.nn.silu(x)
def _sigmoid(x):
    return jax.nn.sigmoid(x)
def _layernorm(x, axis=-1, eps=1e-5):
    m = jnp.mean(x, axis=axis, keepdims=True)
    v = jnp.var(x, axis=axis, keepdims=True)
    return (x - m) / jnp.sqrt(v + eps)
def _scatter_add(tgt, idx, src, axis=0):
    return tgt.at[idx].add(src)
def _segment_sum(src, seg, n):
    return jax.ops.segment_sum(src, seg, n)
class _Rng:
    def __init__(self, key):
        self._k = key
    def _next(self):
        self._k, sub = jax.random.split(self._k)
        return sub
    def normal(self, shape):
        return jax.random.normal(self._next(), shape, dtype=jnp.bfloat16)
    def randint(self, lo, hi, shape):
        return jax.random.randint(self._next(), shape, lo, hi, dtype=jnp.int32)
    def uniform(self, shape, lo=0.0, hi=1.0):
        return jax.random.uniform(self._next(), shape, jnp.bfloat16, lo, hi)
    def permutation(self, n):
        return jax.random.permutation(self._next(), n)


kernel_name = 'interleave_layers__ssm_conv_s4__sliding_local_dilated__prompt'

def setup_inputs():
    _rng = _Rng(jax.random.key(int.from_bytes(__import__("os").urandom(4), "little")))
    _w = (lambda a: (lambda t: t.astype(jnp.bfloat16) if jnp.issubdtype(t.dtype, jnp.floating) else t)(jnp.asarray(a)))
    def _A_setup():
        B, L, D, N = 1, 2048, 512, 128
        A_re = -jnp.exp((lambda *s: _rng.normal(s) * 0.05)(D, N))
        A_im = jnp.pi * (lambda *s: _rng.normal(s) * 0.05)(D, N)
        B_re = (lambda *s: _rng.normal(s) * 0.05)(D, N)
        B_im = (lambda *s: _rng.normal(s) * 0.05)(D, N)
        C_re = (lambda *s: _rng.normal(s) * 0.05)(D, N)
        C_im = (lambda *s: _rng.normal(s) * 0.05)(D, N)
        log_dt = (lambda *s: _rng.normal(s) * 0.05)(D) * 0.5 - 4.0
        Dskip = (lambda *s: _rng.normal(s) * 0.05)(D)
        return {
            "u": _w((lambda *s: _rng.normal(s) * 0.05)(B, L, D)),
            "A_re": _w(A_re),
            "A_im": _w(A_im),
            "B_re": _w(B_re),
            "B_im": _w(B_im),
            "C_re": _w(C_re),
            "C_im": _w(C_im),
            "log_dt": _w(log_dt),
            "Dskip": _w(Dskip),
        }
    _A_in = _A_setup()

    def _B_setup():
        B, S, D = 1, 2048, 512
        return {
            "x": _w((lambda *s: _rng.normal(s) * 0.05)(B, S, D)),
            "wqkv": _w((lambda *s: _rng.normal(s) * 0.05)(D, 3 * D)),
            "wo": _w((lambda *s: _rng.normal(s) * 0.05)(D, D)),
        }
    _B_in = _B_setup()

    return {
        "A_u": _A_in["u"],
        "A_A_re": _A_in["A_re"],
        "A_A_im": _A_in["A_im"],
        "A_B_re": _A_in["B_re"],
        "A_B_im": _A_in["B_im"],
        "A_C_re": _A_in["C_re"],
        "A_C_im": _A_in["C_im"],
        "A_log_dt": _A_in["log_dt"],
        "A_Dskip": _A_in["Dskip"],
        "B_x": _B_in["x"],
        "B_wqkv": _B_in["wqkv"],
        "B_wo": _B_in["wo"],
    }

def reference(A_u, A_A_re, A_A_im, A_B_re, A_B_im, A_C_re, A_C_im, A_log_dt, A_Dskip, B_x, B_wqkv, B_wo):
    def _A_ref(u, A_re, A_im, B_re, B_im, C_re, C_im, log_dt, Dskip):
        Bsz, L, D = u.shape
        dt = jnp.exp(log_dt)[:, None]
        A = A_re + 1j * A_im
        Bc = B_re + 1j * B_im
        Cc = C_re + 1j * C_im
        logdA = dt * A
        dB = dt * Bc
        l = (lambda x, dt: x.astype(dt))(jnp.arange(L), A_re.dtype)
        P = jnp.exp(logdA[:, :, None] * l[None, None, :])
        K = jnp.einsum("dn,dnl,dn->dl", Cc, P, dB).real
        L2 = 2 * L
        Kp = jnp.pad(K, ((0, 0), (0, L)))
        up = (lambda x, *d: x.transpose(*d))(u, 0, 2, 1)
        up = jnp.pad(up, ((0, 0), (0, 0), (0, L)))
        Kf = (lambda x, axes=(-2,-1): jnp.fft.rfft2(x.astype(jnp.float32), axes=axes))(Kp[:, None, :], axes=(-2, -1))
        Uf = (lambda x, axes=(-2,-1): jnp.fft.rfft2(x.astype(jnp.float32), axes=axes))(up[:, :, None, :], axes=(-2, -1))
        Yf = Uf * Kf[None, :, :, :]
        y = (lambda x, s, axes=(-2,-1): jnp.fft.irfft2(x, s=s, axes=axes).astype(jnp.bfloat16))(Yf, (1, L2), axes=(-2, -1))[:, :, 0, :L]
        y = (lambda x, *d: x.transpose(*d))(y, 0, 2, 1) + u * Dskip[None, None, :]
        return y

    def _B_ref(x, wqkv, wo):
        B, S, D = x.shape
        H = 32; Dh = D // H
        W, dil = 8, 2
        qkv = (lambda x, *d: x.transpose(*d))((x @ wqkv).reshape(B, S, 3, H, Dh), 2, 0, 3, 1, 4)
        q, k, v = qkv[0], qkv[1], qkv[2]
        scale = Dh ** -0.5
        pos = jnp.arange(S)
        off = jnp.arange(W) * dil
        idx = pos[:, None] - off[None, :]
        mask = idx >= 0
        idx_c = jnp.where(mask, idx, 0).reshape(-1)
        kg = k[:, :, idx_c, :].reshape(B, H, S, W, Dh)
        vg = v[:, :, idx_c, :].reshape(B, H, S, W, Dh)
        logits = jnp.einsum("bhsd,bhswd->bhsw", q, kg) * scale
        logits = jnp.where(mask[None, None, :, :], logits, -1e9)
        attn = _softmax(logits, axis=-1)
        o = jnp.einsum("bhsw,bhswd->bhsd", attn, vg)
        return (lambda x, *d: x.transpose(*d))(o, 0, 2, 1, 3).reshape(B, S, D) @ wo

    x = A_u
    x = x + _A_ref(_layernorm(x, axis=-1), A_A_re, A_A_im, A_B_re, A_B_im, A_C_re, A_C_im, A_log_dt, A_Dskip)
    x = x + _B_ref(_layernorm(x, axis=-1), B_wqkv, B_wo)
    x = x + _A_ref(_layernorm(x, axis=-1), A_A_re, A_A_im, A_B_re, A_B_im, A_C_re, A_C_im, A_log_dt, A_Dskip)
    x = x + _B_ref(_layernorm(x, axis=-1), B_wqkv, B_wo)
    return x
```

```python
import ml_dtypes
import numpy as np

import jax
import jax.numpy as jnp
from jax import lax
import jax.experimental.pallas as pl
import jax.experimental.pallas.tpu as pltpu

L, D, N = 2048, 512, 128
R, C = 16, 128
DH, WIN = 16, 8
CB = 128
EPS = 1e-5
F32, BF16, U32 = jnp.float32, jnp.bfloat16, jnp.uint32
_NT = (((1,), (1,)), ((), ()))


def _dft_tables():
    t = R * np.arange(C)[None, :, None] + np.arange(R)[:, None, None]
    ang = 2.0 * np.pi * (np.arange(C)[None, None, :] + 0.5) * t / (2 * L)
    fwd = np.concatenate([np.cos(ang), -np.sin(ang)], axis=-1)
    p = (np.arange(C) - 7) % C
    fwd_k = fwd[:, 16 * (p % 8) + p // 8, :] / L
    inv = fwd.transpose(0, 2, 1)
    return tuple(np.ascontiguousarray(a).astype(ml_dtypes.bfloat16) for a in (fwd, fwd_k, inv))


def _tap_offsets():
    l = np.arange(L)
    lr = l.astype(np.float32).astype(ml_dtypes.bfloat16).astype(np.float32).astype(np.int64)
    rho = (lr - (l // R) * R).reshape(8, 16, R)
    assert (rho == rho[:, :1]).all()
    return rho[:, 0].tolist()


def _cmul(a, b):
    return a[0] * b[0] - a[1] * b[1], a[0] * b[1] + a[1] * b[0]


def _csq(a):
    t = a[0] * a[1]
    return a[0] * a[0] - a[1] * a[1], t + t


def _twiddle(a, k, n):
    if k == 0:
        return a
    h = float(np.sqrt(0.5))
    if 8 * k == n:
        return (a[0] + a[1]) * h, (a[1] - a[0]) * h
    if 8 * k == 3 * n:
        return (a[1] - a[0]) * h, (a[0] + a[1]) * (-h)
    w = (float(np.cos(2 * np.pi * k / n)), float(-np.sin(2 * np.pi * k / n)))
    return _cmul(a, w)


def _fft(x):
    n = len(x)
    if n == 1:
        return x
    if n == 2:
        return [(x[0][0] + x[1][0], x[0][1] + x[1][1]), (x[0][0] - x[1][0], x[0][1] - x[1][1])]
    e, o1, o3 = _fft(x[0::2]), _fft(x[1::4]), _fft(x[3::4])
    out = [None] * n
    q = n // 4
    for k in range(q):
        a, b = _twiddle(o1[k], k, n), _twiddle(o3[k], 3 * k, n)
        s = (a[0] + b[0], a[1] + b[1])
        d = (a[0] - b[0], a[1] - b[1])
        out[k] = (e[k][0] + s[0], e[k][1] + s[1])
        out[k + 2 * q] = (e[k][0] - s[0], e[k][1] - s[1])
        out[k + q] = (e[k + q][0] + d[1], e[k + q][1] - d[0])
        out[k + 3 * q] = (e[k + q][0] - d[1], e[k + q][1] + d[0])
    return out


def _ifft(x):
    return [(b, a) for a, b in _fft([(b, a) for a, b in x])]


def _layernorm(x):
    m = jnp.sum(x, axis=0, keepdims=True) * (1.0 / D)
    xc = x - m
    v = jnp.sum(xc * xc, axis=0, keepdims=True) * (1.0 / D)
    return (xc * lax.rsqrt(v + EPS)).astype(BF16)


def _kernel(x_hbm, are_hbm, aim_hbm, bre_hbm, bim_hbm, cre_hbm, cim_hbm, ldt_ref, dsk_ref,
            wqkv_hbm, wo_hbm, ff_hbm, fk_hbm, fi_hbm, out_hbm,
            io_v, par_v, wqkv_v, wo_v, ff_v, fk_v, fi_v, dt_v, dk_v, wt_v, wot_v, tmp_v,
            x_v, u_v, kt_v, kh_v, s_v, z_v, kv_v, q_v, o_v, sems):
    srcs = (are_hbm, aim_hbm, bre_hbm, bim_hbm, cre_hbm, cim_hbm)
    par_cp = [pltpu.make_async_copy(s, par_v.at[i], sems.at[i]) for i, s in enumerate(srcs)]
    x_w, out_w = x_hbm.bitcast(U32), out_hbm.bitcast(U32)
    x_cp = [pltpu.make_async_copy(x_w.at[:, i, :], io_v.at[i], sems.at[12 + i])
            for i in range(R // 2)]
    fk_cp = pltpu.make_async_copy(fk_hbm, fk_v, sems.at[7])
    ff_cp = pltpu.make_async_copy(ff_hbm, ff_v, sems.at[8])
    fi_cp = pltpu.make_async_copy(fi_hbm, fi_v, sems.at[9])
    wqkv_cp = pltpu.make_async_copy(wqkv_hbm, wqkv_v, sems.at[10])
    wo_cp = pltpu.make_async_copy(wo_hbm, wo_v, sems.at[11])
    for cp in par_cp + x_cp + [fk_cp, ff_cp, fi_cp, wqkv_cp, wo_cp]:
        cp.start()

    lane = lax.broadcasted_iota(jnp.int32, (8, C), 1)
    rho = _tap_offsets()

    dt_row = jnp.exp(ldt_ref[...].astype(F32)).astype(BF16).astype(F32)
    dk_row = dsk_ref[...].astype(F32)
    for b in range(D // C):
        cols = slice(b * C, (b + 1) * C)
        dt_v[cols, :] = jnp.broadcast_to(dt_row[:, cols], (C, C)).T
        dk_v[cols, :] = jnp.broadcast_to(dk_row[:, cols], (C, C)).T

    sub = lax.broadcasted_iota(jnp.int32, (8, C), 0)

    def flip(x):
        x = pltpu.roll(x, 4, 0)
        x = jnp.where((sub & 2) == 0, pltpu.roll(x, 6, 0), pltpu.roll(x, 2, 0))
        return jnp.where((sub & 1) == 0, pltpu.roll(x, 7, 0), pltpu.roll(x, 1, 0))

    def filter_taps(a_re, a_im, b_re, b_im, c_re, c_im, dt, dskip):
        mag = jnp.exp(dt * a_re)
        ph = dt * a_im
        a1 = (mag * jnp.cos(ph), mag * jnp.sin(ph))
        w = _cmul((c_re, c_im), (dt * b_re, dt * b_im))
        a2 = _csq(a1)
        a4 = _csq(a2)
        a8 = _csq(a4)
        a16 = _csq(a8)
        right = [(jnp.ones_like(mag), jnp.zeros_like(mag)), (flip(a16[0]), -flip(a16[1]))]
        for j in range(2, 17):
            right.append(_csq(right[j // 2]) if j % 2 == 0 else _cmul(right[j - 1], right[1]))
        a256 = (flip(right[16][0]), -flip(right[16][1]))
        left = {(0, 0): w}
        for step, a in ((16, a16), (8, a8), (4, a4), (2, a2), (1, a1)):
            for p in range(step, 17, 2 * step):
                left[0, p] = _cmul(left[0, p - step], a)
        keys = [(s, p) for s in range(8) for p in sorted(set(rho[s]) | {16}) if p]
        for s, p in keys:
            if s:
                left[s, p] = _cmul(left[s - 1, p], a256)
        lhs = jnp.concatenate([jnp.concatenate(left[k], axis=1) for k in keys], axis=0)
        rhs = jnp.concatenate([jnp.concatenate(right[j], axis=1) for j in range(16)], axis=0)
        res = lax.dot_general(lhs.astype(BF16), rhs.astype(BF16), _NT, preferred_element_type=F32)
        part = {k: pltpu.roll(res[8 * n:8 * n + 8], k[0], 1, stride=1, stride_axis=0)
                for n, k in enumerate(keys)}
        pos = (lane - 7) & (C - 1)
        seg = pos & 7
        memo = {}

        def merge(ps):
            s = 8 - len(ps)
            if len(ps) == 1 or not any(ps):
                return part[s, ps[0]]
            if ps not in memo:
                memo[ps] = jnp.where(seg == s, part[s, ps[0]], merge(ps[1:]))
            return memo[ps]

        t16 = merge((16,) * 8)
        tap0 = jnp.sum(w[0], axis=1, keepdims=True) + dskip
        t0 = jnp.where(pos < 8, pltpu.roll(t16, 9, 1), pltpu.roll(t16, 8, 1))
        t0 = jnp.where(pos == 0, tap0, t0)
        for s in range(8):
            part[s, 0] = t0
        return [merge(tuple(rho[s][r] for s in range(8))) for r in range(R)]

    def filter_step(i, carry):
        rows = pl.ds(pl.multiple_of(i * 16, 16), 16)
        args = [par_v[n, rows, :].astype(F32) for n in range(6)] + [dt_v[rows, :], dk_v[rows, :]]
        lo = filter_taps(*[a[:8] for a in args])
        hi = filter_taps(*[a[8:] for a in args])
        for r in range(R):
            kt_v[r, rows, :] = jnp.concatenate([lo[r], hi[r]], axis=0).astype(BF16)
        return carry

    def spectrum_dft(r, carry):
        kh_v[r] = jnp.dot(kt_v[r], fk_v[r], preferred_element_type=F32)
        return carry

    def spectrum_fft(i, carry):
        rows = pl.ds(pl.multiple_of(i * 8, 8), 8)
        out = _fft([(kh_v[r, rows, :C], kh_v[r, rows, C:]) for r in range(R)])
        for r in range(R):
            kh_v[r, rows, :C] = out[r][0]
            kh_v[r, rows, C:] = out[r][1]
        return carry

    for cp in par_cp:
        cp.wait()
    with jax.named_scope("filter"):
        lax.fori_loop(0, D // 16, filter_step, 0)
    fk_cp.wait()
    with jax.named_scope("spectrum"):
        lax.fori_loop(0, R, spectrum_dft, 0)
        lax.fori_loop(0, D // 8, spectrum_fft, 0)

    def load_step(i, carry):
        for b in range(D // C):
            cols = slice(b * C, (b + 1) * C)
            wd = io_v[i, :, cols].T
            x_v[2 * i, cols, :] = pltpu.bitcast(wd << 16, F32)
            x_v[2 * i + 1, cols, :] = pltpu.bitcast(wd & jnp.uint32(0xFFFF0000), F32)
        for r in (2 * i, 2 * i + 1):
            u_v[r] = _layernorm(x_v[r])
        return carry

    for cp in x_cp:
        cp.wait()
    with jax.named_scope("load"):
        lax.fori_loop(0, R // 2, load_step, 0)

    def head_order(b, tile):
        tmp_v[b] = tile
        return jnp.concatenate([tmp_v[b, pl.ds(dh, 8, stride=DH), :] for dh in range(DH)], axis=0)

    wqkv_cp.wait()
    wo_cp.wait()
    with jax.named_scope("weights"):
        for j in range(3 * D // C):
            for b in range(D // C):
                hd, ch = slice(j * C, (j + 1) * C), slice(b * C, (b + 1) * C)
                wt = head_order(b, wqkv_v[ch, hd].astype(F32).T)
                wt_v[hd, ch] = (wt * DH ** -0.5 if j < D // C else wt).astype(BF16)
                if j < D // C:
                    wot_v[ch, hd] = head_order(4 + b, wo_v[hd, ch].astype(F32)).T.astype(BF16)
    ff_cp.wait()
    fi_cp.wait()

    def conv_block(b, carry):
        base = pl.multiple_of(b * CB, CB)
        rows = pl.ds(base, CB)
        for r in range(R):
            s_v[r] = jnp.dot(u_v[r, rows, :], ff_v[r], preferred_element_type=F32)

        def mix(i, carry):
            halves = []
            for h in range(2):
                off = pl.multiple_of(i * 16 + 8 * h, 8)
                sr, kr = pl.ds(off, 8), pl.ds(base + off, 8)
                uf = _fft([(s_v[r, sr, :C], s_v[r, sr, C:]) for r in range(R)])
                halves.append(_ifft([_cmul(uf[r], (kh_v[r, kr, :C], kh_v[r, kr, C:]))
                                     for r in range(R)]))
            zr = pl.ds(pl.multiple_of(i * 16, 16), 16)
            for r in range(R):
                for c in range(2):
                    z_v[r, zr, c * C:(c + 1) * C] = jnp.concatenate(
                        [halves[0][r][c], halves[1][r][c]], axis=0).astype(BF16)
            return carry

        lax.fori_loop(0, CB // 16, mix, 0)
        for r in range(R):
            x_v[r, rows, :] += jnp.dot(z_v[r], fi_v[r], preferred_element_type=F32)
        return carry

    def kv_step(r, carry):
        xn = _layernorm(x_v[r])
        u_v[r] = xn
        kv = jnp.dot(wt_v[D:, :], xn, preferred_element_type=F32)
        slot = 16 * (r & 1) + (r >> 1)
        kv_v[slot + 8] = kv
        kv_v[slot] = pltpu.roll(kv, 1, 1)
        return carry

    def attend(r):
        slot = 16 * (r & 1) + 8 + (r >> 1)
        for g in range(D // C):
            logits = []
            for w in range(WIN):
                acc = None
                for dh in range(DH):
                    rows = pl.ds(g * C + dh * 8, 8)
                    t = q_v[rows, :] * kv_v[slot - w, rows, :]
                    acc = t if acc is None else acc + t
                if w:
                    acc = jnp.where(lane < jnp.where((r >> 1) < w, 1, 0), -1e9, acc)
                logits.append(acc)
            m = logits[0]
            for t in logits[1:]:
                m = jnp.maximum(m, t)
            e = [jnp.exp(t - m) for t in logits]
            den = e[0]
            for t in e[1:]:
                den = den + t
            inv = 1.0 / den
            p = [t * inv for t in e]
            for dh in range(0, DH, 2):
                pair = []
                for k in range(2):
                    rows = pl.ds(D + g * C + (dh + k) * 8, 8)
                    acc = None
                    for w in range(WIN):
                        t = p[w] * kv_v[slot - w, rows, :]
                        acc = t if acc is None else acc + t
                    pair.append(acc)
                o_v[pl.ds(g * C + dh * 8, 16), :] = jnp.concatenate(pair, axis=0).astype(BF16)

    def attn_step(last, r, carry):
        q_v[...] = jnp.dot(wt_v[:D, :], u_v[r], preferred_element_type=F32)
        attend(r)
        x = x_v[r] + jnp.dot(wot_v[...], o_v[...], preferred_element_type=F32)
        x_v[r] = x
        if not last:
            u_v[r] = _layernorm(x)
        return carry

    for last in (False, True):
        with jax.named_scope("conv"):
            lax.fori_loop(0, D // CB, conv_block, 0)
        with jax.named_scope("kv"):
            lax.fori_loop(0, R, kv_step, 0)
        with jax.named_scope("attn"):
            lax.fori_loop(0, R, lambda r, c, last=last: attn_step(last, r, c), 0)

    def store_step(i, carry):
        for b in range(D // C):
            cols = slice(b * C, (b + 1) * C)
            lo = pltpu.bitcast(x_v[2 * i, cols, :].astype(BF16).astype(F32), U32)
            hi = pltpu.bitcast(x_v[2 * i + 1, cols, :].astype(BF16).astype(F32), U32)
            io_v[i, :, cols] = (hi | (lo >> 16)).T
        return carry

    with jax.named_scope("store"):
        lax.fori_loop(0, R // 2, store_step, 0)
    out_cp = [pltpu.make_async_copy(io_v.at[i], out_w.at[:, i, :], sems.at[12 + i])
              for i in range(R // 2)]
    for cp in out_cp:
        cp.start()
    for cp in out_cp:
        cp.wait()


@jax.jit
def pallas_interleave_layers__ssm_conv_s4__sliding_local_dilated__prompt_kernel(
    A_u: jax.Array,
    A_A_re: jax.Array,
    A_A_im: jax.Array,
    A_B_re: jax.Array,
    A_B_im: jax.Array,
    A_C_re: jax.Array,
    A_C_im: jax.Array,
    A_log_dt: jax.Array,
    A_Dskip: jax.Array,
    B_x: jax.Array,
    B_wqkv: jax.Array,
    B_wo: jax.Array,
):
    del B_x
    assert A_u.shape == (1, L, D) and A_A_re.shape == (D, N) and A_A_re.dtype == BF16
    hbm = pl.BlockSpec(memory_space=pl.ANY)
    vmem = pl.BlockSpec(memory_space=pltpu.VMEM)
    out = pl.pallas_call(
        _kernel,
        in_specs=[hbm] * 7 + [vmem] * 2 + [hbm] * 5,
        out_specs=hbm,
        out_shape=jax.ShapeDtypeStruct((C, R, D), BF16),
        scratch_shapes=[
            pltpu.VMEM((R // 2, C, D), U32),
            pltpu.VMEM((6, D, N), BF16),
            pltpu.VMEM((D, 3 * D), BF16),
            pltpu.VMEM((D, D), BF16),
            pltpu.VMEM((R, C, 2 * C), BF16),
            pltpu.VMEM((R, C, 2 * C), BF16),
            pltpu.VMEM((R, 2 * C, C), BF16),
            pltpu.VMEM((D, C), F32),
            pltpu.VMEM((D, C), F32),
            pltpu.VMEM((3 * D, D), BF16),
            pltpu.VMEM((D, D), BF16),
            pltpu.VMEM((8, C, C), F32),
            pltpu.VMEM((R, D, C), F32),
            pltpu.VMEM((R, D, C), BF16),
            pltpu.VMEM((R, D, C), BF16),
            pltpu.VMEM((R, D, 2 * C), F32),
            pltpu.VMEM((R, CB, 2 * C), F32),
            pltpu.VMEM((R, CB, 2 * C), BF16),
            pltpu.VMEM((2 * R, 2 * D, C), F32),
            pltpu.VMEM((D, C), F32),
            pltpu.VMEM((D, C), BF16),
            pltpu.SemaphoreType.DMA((20,)),
        ],
        compiler_params=pltpu.CompilerParams(vmem_limit_bytes=100 * 1024 * 1024),
    )(A_u.reshape(C, R, D), A_A_re, A_A_im, A_B_re, A_B_im, A_C_re, A_C_im,
      A_log_dt.reshape(1, D), A_Dskip.reshape(1, D), B_wqkv, B_wo, *_dft_tables())
    return out.reshape(1, L, D)
```

```python
import ml_dtypes
import numpy as np

import jax
import jax.numpy as jnp
from jax import lax
import jax.experimental.pallas as pl
import jax.experimental.pallas.tpu as pltpu

L, D, N = 2048, 512, 128
R, C = 16, 128
DH, WIN = 16, 8
CB = 64
LV = 1
PH, NP = 2 ** LV, 7 ** LV
QKV_CHUNKS, OUT_CHUNKS = ((1,), (2,), (0,)), ((0,), (1,), (2,), (3,))
LAG = 7
EPS = 1e-5
F32, BF16, U32 = jnp.float32, jnp.bfloat16, jnp.uint32
_NT = (((1,), (1,)), ((), ()))


def _host_words(a):
    h = np.ascontiguousarray(a).astype(ml_dtypes.bfloat16).view(np.uint16).astype(np.uint32)
    return h[..., 0::2, :] | (h[..., 1::2, :] << 16)


def _dft_tables():
    t = R * np.arange(C)[None, :, None] + np.arange(R)[:, None, None]
    ang = 2.0 * np.pi * (np.arange(C)[None, None, :] + 0.5) * t / (2 * L)
    fwd = np.concatenate([np.cos(ang), -np.sin(ang)], axis=-1)
    p = (np.arange(C) - 7) % C
    fwd_k = fwd[:, 16 * (p % 8) + p // 8, :] / L
    inv = fwd.transpose(0, 2, 1)
    fwd, fwd_k = [np.concatenate([a[..., :C], a[..., C:]], axis=1) for a in (fwd, fwd_k)]
    return _host_words(np.concatenate([fwd, inv])), _host_words(fwd_k)


def _tap_offsets():
    l = np.arange(L)
    lr = l.astype(np.float32).astype(ml_dtypes.bfloat16).astype(np.float32).astype(np.int64)
    rho = (lr - (l // R) * R).reshape(8, 16, R)
    assert (rho == rho[:, :1]).all()
    return rho[:, 0].tolist()


def _cmul(a, b):
    return a[0] * b[0] - a[1] * b[1], a[0] * b[1] + a[1] * b[0]


def _csq(a):
    t = a[0] * a[1]
    return a[0] * a[0] - a[1] * a[1], t + t


def _twiddle(a, k, n):
    if k == 0:
        return a
    if 4 * k == n:
        return a[1], -a[0]
    h = float(np.sqrt(0.5))
    if 8 * k == n:
        return (a[0] + a[1]) * h, (a[1] - a[0]) * h
    if 8 * k == 3 * n:
        return (a[1] - a[0]) * h, (a[0] + a[1]) * (-h)
    w = (float(np.cos(2 * np.pi * k / n)), float(-np.sin(2 * np.pi * k / n)))
    return _cmul(a, w)


def _fft(x):
    n = len(x)
    if n == 1:
        return x
    if n == 2:
        return [(x[0][0] + x[1][0], x[0][1] + x[1][1]), (x[0][0] - x[1][0], x[0][1] - x[1][1])]
    e, o1, o3 = _fft(x[0::2]), _fft(x[1::4]), _fft(x[3::4])
    out = [None] * n
    q = n // 4
    for k in range(q):
        a, b = _twiddle(o1[k], k, n), _twiddle(o3[k], 3 * k, n)
        s = (a[0] + b[0], a[1] + b[1])
        d = (a[0] - b[0], a[1] - b[1])
        out[k] = (e[k][0] + s[0], e[k][1] + s[1])
        out[k + 2 * q] = (e[k][0] - s[0], e[k][1] - s[1])
        out[k + q] = (e[k + q][0] + d[1], e[k + q][1] - d[0])
        out[k + 3 * q] = (e[k + q][0] - d[1], e[k + q][1] + d[0])
    return out


def _ifft(x):
    return [(b, a) for a, b in _fft([(b, a) for a, b in x])]


def _tree(op, xs):
    while len(xs) > 1:
        xs = [op(*xs[i:i + 2]) if i + 1 < len(xs) else xs[i] for i in range(0, len(xs), 2)]
    return xs[0]


def _sums(x, acc=None):
    parts = [x[i:i + 8] for i in range(0, x.shape[0], 8)]
    new = _tree(jnp.add, parts), _tree(jnp.add, [t * t for t in parts])
    return new if acc is None else (acc[0] + new[0], acc[1] + new[1])


def _stats(acc):
    m, sq = [jnp.sum(t, axis=0, keepdims=True) * (1.0 / D) for t in acc]
    return m, lax.rsqrt(jnp.maximum(sq - m * m, 0.0) + EPS)


def _words(x):
    return pltpu.bitcast(x.astype(BF16), U32)


def _pairs(x):
    b = pltpu.bitcast(x.astype(BF16).astype(F32), U32)
    return b[x.shape[0] // 2:] | (b[:x.shape[0] // 2] >> 16)


def _halves(w):
    return pltpu.bitcast(w, BF16)


def _dot(a, b, dims=(((1,), (0,)), ((), ()))):
    return lax.dot_general(a.astype(BF16), b.astype(BF16), dims, preferred_element_type=F32)


def _split(src, table, r, rows):
    lo, hi = [_dot(src[n, rows, :], _halves(jnp.concatenate(
        [table[n, :C // 2], table[n, C // 2:]], axis=1))) for n in (r, r + 8)]
    d = lo - hi
    return lo + hi, jnp.concatenate(_twiddle((d[:, :C], d[:, C:]), r, R), axis=1)


def _run(*jobs):
    order = []
    for k, (_, n, *span) in enumerate(jobs):
        lo, hi = span or (0.0, 1.0)
        order += [(lo + (hi - lo) * i / n, k) for i in range(n)]
    for _, k in sorted(order):
        next(jobs[k][0])
    for job in jobs:
        for _ in job[0]:
            pass


def _chain(gens):
    for g in gens:
        yield from g


def _lhs_terms(a, levels):
    if not levels:
        return [jnp.concatenate(a, axis=0)]
    m, k = a[0].shape[0] // 2, a[0].shape[1] // 2
    terms = []
    for t in a:
        a11, a12, a21, a22 = t[:m, :k], t[:m, k:], t[m:, :k], t[m:, k:]
        terms.append((a11 + a22, a21 + a22, a22, a12 - a22, a21 - a11, a11, a11 + a12))
    return [x for ts in zip(*terms) for x in _lhs_terms(list(ts), levels - 1)]


def _rhs_terms(b, levels):
    if not levels:
        return [b]
    k, n = b.shape[0] // 2, b.shape[1] // 2
    b11, b12, b21, b22 = b[:k, :n], b[:k, n:], b[k:, :n], b[k:, n:]
    terms = (b11 + b22, b11, b21 - b11, b21 + b22, b11 + b12, b12 - b22, b22)
    return [x for t in terms for x in _rhs_terms(t, levels - 1)]


def _strassen(product, levels, emit=None, base=0):
    if not levels:
        out = {(0, 0): product(base)}
        if emit:
            emit(out)
        yield
        return out
    half, out = 2 ** (levels - 1), {}

    def term(i):
        return _strassen(product, levels - 1, None, base + i * 7 ** (levels - 1))

    def done(i, j, x):
        x = {(i * half + a, j * half + b): v for (a, b), v in x.items()}
        out.update(x)
        if emit:
            emit(x)

    def add(x, y):
        return {k: x[k] + y[k] for k in x}

    def sub(x, y):
        return {k: x[k] - y[k] for k in x}

    m1 = yield from term(0)
    m2 = yield from term(1)
    c22 = sub(m1, m2)
    m4 = yield from term(2)
    c11 = add(m1, m4)
    done(1, 0, add(m2, m4))
    c11 = add(c11, (yield from term(3)))
    c22 = add(c22, (yield from term(4)))
    m3 = yield from term(5)
    done(1, 1, add(c22, m3))
    m5 = yield from term(6)
    done(0, 0, sub(c11, m5))
    done(0, 1, add(m3, m5))
    return out


def _ds(start, size):
    return pl.ds(start if isinstance(start, int) else pl.multiple_of(start, size), size)


def _loop(lo, hi, body):
    lax.fori_loop(lo, hi, lambda i, c: (body(i), c)[1], 0)


def _kernel(x_hbm, are_hbm, aim_hbm, bre_hbm, bim_hbm, cre_hbm, cim_hbm, ldt_ref, dsk_ref,
            wqkv_hbm, wo_hbm, tab_hbm, fk_hbm, zero_s, out_hbm,
            io_v, par_v, wqkv_v, wo_v, tab_v, fk_v, dt_v, dk_v, wt_v, wot_v,
            x_v, u_v, kt_v, kh_v, op_v, ga_v, gb_v, sa_v, sb_v, za_v, zb_v,
            qa_v, qb_v, ya_v, yb_v, sems):
    srcs = (are_hbm, aim_hbm, bre_hbm, bim_hbm, cre_hbm, cim_hbm)
    par_cp = [pltpu.make_async_copy(s.bitcast(U32), par_v.at[i], sems.at[i])
              for i, s in enumerate(srcs)]
    x_w, out_w = x_hbm.bitcast(U32), out_hbm.bitcast(U32)
    x_cp = [pltpu.make_async_copy(x_w.at[:, i, :], io_v.at[i], sems.at[12 + i])
            for i in range(R // 2)]
    fk_cp = pltpu.make_async_copy(fk_hbm, fk_v, sems.at[7])
    tab_cp = pltpu.make_async_copy(tab_hbm, tab_v, sems.at[8])
    wqkv_cp = pltpu.make_async_copy(wqkv_hbm.bitcast(U32), wqkv_v, sems.at[10])
    wo_cp = [pltpu.make_async_copy(wo_hbm.bitcast(U32).at[:, pl.ds(t * C, C)], wo_v.at[t],
                                   sems.at[20 + t]) for t in range(D // C)]
    for cp in par_cp:
        cp.start()

    lane = lax.broadcasted_iota(jnp.int32, (8, C), 1)
    sub = lax.broadcasted_iota(jnp.int32, (8, C), 0)
    rho = _tap_offsets()

    zero = zero_s[0]

    def pin(ref, x):
        ref[ref.shape[0] - 1 + zero, :8, :C] = pltpu.bitcast(x[:8, :C], ref.dtype)

    def pacer(lag, ref):
        queue = []

        def pace(x):
            queue.append(x)
            if len(queue) > lag:
                pin(ref, queue.pop(0))
            return x
        return pace

    dt_row = jnp.exp(ldt_ref[...].astype(F32).reshape(1, D)).astype(BF16).astype(F32)
    dk_row = dsk_ref[...].astype(F32).reshape(1, D)
    for b in range(D // C):
        cols = slice(b * C, (b + 1) * C)
        dt_v[cols, :] = jnp.broadcast_to(dt_row[:, cols], (C, C)).T
        dk_v[cols, :] = jnp.broadcast_to(dk_row[:, cols], (C, C)).T

    keys = [(s, p) for s in range(8) for p in sorted(set(rho[s]) | {16}) if p]
    nk = 8 * len(keys)

    def flip(x):
        x = pltpu.roll(x, 4, 0)
        x = jnp.where((sub & 2) == 0, pltpu.roll(x, 6, 0), pltpu.roll(x, 2, 0))
        return jnp.where((sub & 1) == 0, pltpu.roll(x, 7, 0), pltpu.roll(x, 1, 0))

    def powers(i, g_v):
        par = [_halves(par_v[n, _ds(i * 8, 8), :]).astype(F32) for n in range(6)]
        for h in range(2):
            a_re, a_im, b_re, b_im, c_re, c_im = [a[8 * h:8 * h + 8] for a in par]
            rows = _ds(i * 16 + 8 * h, 8)
            dt = dt_v[rows, :]
            mag = jnp.exp(dt * a_re)
            ph = dt * a_im
            a1 = (mag * jnp.cos(ph), mag * jnp.sin(ph))
            w = _cmul((c_re, c_im), (dt * b_re, dt * b_im))
            dk_v[rows, :] += jnp.sum(w[0], axis=1, keepdims=True)
            a2 = _csq(a1)
            a4 = _csq(a2)
            a8 = _csq(a4)
            a16 = _csq(a8)
            right = [(jnp.ones_like(mag), jnp.zeros_like(mag)), (flip(a16[0]), -flip(a16[1]))]
            for j in range(2, 16):
                right.append(_csq(right[j // 2]) if j % 2 == 0 else _cmul(right[j - 1], right[1]))
            a256 = _csq(_csq(_csq(_csq(a16))))
            left = {(0, 0): w}
            for step, a in ((16, a16), (8, a8), (4, a4), (2, a2), (1, a1)):
                for p in range(step, 17, 2 * step):
                    left[0, p] = _cmul(left[0, p - step], a)
            for s, p in keys:
                if s:
                    left[s, p] = _cmul(left[s - 1, p], a256)
            vals = [left[k] for k in keys] + right
            for n, val in enumerate(vals):
                g_v[h, 8 * n:8 * n + 8, :C], g_v[h, 8 * n:8 * n + 8, C:] = val

    def taps(i, g_v):
        pos = (lane - 7) & (C - 1)
        for h in range(2):
            res = _dot(g_v[h, :nk, :], g_v[h, nk:, :], _NT)
            part = {k: pltpu.roll(res[8 * n:8 * n + 8], k[0], 1, stride=1, stride_axis=0)
                    for n, k in enumerate(keys)}
            memo = {}

            def merge(ps):
                s = 8 - len(ps)
                if len(ps) == 1 or not any(ps):
                    return part[s, ps[0]]
                if ps not in memo:
                    memo[ps] = jnp.where((pos & 7) == s, part[s, ps[0]], merge(ps[1:]))
                return memo[ps]

            t16 = merge((16,) * 8)
            t0 = jnp.where(pos < 8, pltpu.roll(t16, 9, 1), pltpu.roll(t16, 8, 1))
            t0 = jnp.where(pos == 0, dk_v[_ds(i * 16 + 8 * h, 8), :], t0)
            for s in range(8):
                part[s, 0] = t0
            for r in range(R):
                kt_v[r, _ds(i * 16 + 8 * h, 8), :] = merge(tuple(rho[s][r] for s in range(8)))

    def filter_step(i):
        taps(2 * i, ga_v)
        powers(2 * i + 1, gb_v)
        taps(2 * i + 1, gb_v)
        powers(2 * i + 2, ga_v)

    for cp in par_cp:
        cp.wait()
    for cp in x_cp + [fk_cp, tab_cp, wqkv_cp] + wo_cp:
        cp.start()
    with jax.named_scope("filter"):
        n = D // 16
        powers(0, ga_v)
        _loop(0, n // 2 - 1, filter_step)
        taps(n - 2, ga_v)
        powers(n - 1, gb_v)
        taps(n - 1, gb_v)

    def load_step(i):
        kh_v[i], kh_v[i + 8] = _split(kt_v, fk_v, i, slice(None))
        wd = jnp.concatenate([io_v[i, :, b * C:(b + 1) * C].T for b in range(D // C)], axis=0)
        for r, w in ((2 * i, wd << 16), (2 * i + 1, wd & jnp.uint32(0xFFFF0000))):
            x = pltpu.bitcast(w, F32)
            x_v[r] = x
            m, s = _stats(_sums(x))
            u_v[r] = (x - m) * s

    for cp in x_cp + [fk_cp]:
        cp.wait()
    with jax.named_scope("load"):
        for i in range(R // 2):
            load_step(i)

    hp = DH // 2 // PH

    def weights():
        row = lax.broadcasted_iota(jnp.int32, (C, C), 0)
        col = lax.broadcasted_iota(jnp.int32, (C, C), 1)
        pick = jnp.where(col == (row & 7) * DH + (row >> 3), 1.0, 0.0)
        for g in range(D // C):
            for n, chunk in enumerate(QKV_CHUNKS):
                tiles = [_dot(pick * (DH ** -0.5 if t == 0 else 1.0),
                              _halves(wqkv_v[:, pl.ds(t * D + g * C, C)]), _NT) for t in chunk]
                for i, a in enumerate(_lhs_terms(tiles, LV)):
                    wt_v[g, n, i] = _words(a)
        for n, chunk in enumerate(OUT_CHUNKS):
            tiles = [_halves(jnp.concatenate(
                [wo_v[t, pl.ds(g * C // 2 + h * hp + i, 8, stride=DH // 2), :]
                 for h in range(PH) for g in range(D // C) for i in range(hp)],
                axis=0)).T.astype(F32) for t in chunk]
            for i, a in enumerate(_lhs_terms(tiles, LV)):
                wot_v[n, i] = _words(a)

    for cp in [tab_cp, wqkv_cp] + wo_cp:
        cp.wait()
    with jax.named_scope("weights"):
        weights()

    def forward(b):
        s_v = (sa_v, sb_v)[b % 2]
        for r in range(8):
            s_v[r], s_v[r + 8] = _split(u_v, tab_v, r, pl.ds(b * CB, CB))
            yield

    def inverse(b, shift=0):
        z_v = (za_v, zb_v)[b % 2]
        for r in range(8):
            ev = z_v[r]
            od = _twiddle((z_v[r + 8, :, C:], z_v[r + 8, :, :C]), r, R)
            od = jnp.concatenate(od[::-1], axis=1)
            for n, z in ((r, ev + od), (r + 8, ev - od)):
                rows = pl.ds(b * CB, CB)
                x_v[n + shift, rows, :] = x_v[n, rows, :] + _dot(z, _halves(tab_v[R + n]))
            yield

    def mix(first, b):
        s_v, z_v = (sa_v, sb_v)[b % 2], (za_v, zb_v)[b % 2]
        for i in range(CB // 4):
            sr, kr = pl.ds(i // 2 * 8, 8), pl.ds(b * CB + i // 2 * 8, 8)
            rs = range(i % 2 * 8, i % 2 * 8 + 8)
            kf = [(kh_v[r, kr, :C], kh_v[r, kr, C:]) for r in rs]
            if first:
                kf = _fft(kf)
                for r, k in zip(rs, kf):
                    kh_v[r, kr, :C], kh_v[r, kr, C:] = k
            uf = _fft([(s_v[r, sr, :C], s_v[r, sr, C:]) for r in rs])
            for r, z in zip(rs, _ifft([_cmul(*t) for t in zip(uf, kf)])):
                z_v[r, sr, :C], z_v[r, sr, C:] = z
            yield

    def conv(first, b):
        _run(*[(forward(b + 1), 8)] * (b + 1 < D // CB),
             *[(inverse(b - 1), 8, 0.0625, 1.0625)] * (b > 0), (mix(first, b), CB // 4))

    sz, kw, groups = C // PH, D // PH // 2, R // PH

    def moments(p, stats):
        for r in range(PH * p, PH * p + PH):
            acc = None
            for b in range(D // C):
                for row in range(b * C, b * C + C, 32):
                    acc = _sums(x_v[r, pl.ds(row, 32), :], acc)
                pin(op_v, acc[1])
                stats[r] = acc if b + 1 < D // C else _stats(acc)
                yield

    def terms(tile, i):
        return _rhs_terms(jnp.concatenate([jnp.concatenate(
            [tile(j, h * 2 * kw + 32 * i) for j in range(PH)], axis=1) for h in range(PH)],
            axis=0), LV)

    def norm(p, stats):
        for i in range(kw // 16):
            for n, b in enumerate(terms(lambda j, row: (
                    x_v[PH * p + j, pl.ds(row, 32), :] - stats[PH * p + j][0]) * stats[PH * p + j][1], i)):
                op_v[p + zero, pl.ds(n * kw + 16 * i, 16), :] = _words(b)
            yield

    def qkv(g, n, p, pace):
        buf = (qa_v, qb_v)[g % 2]

        def emit(blocks):
            for (i, j), val in blocks.items():
                slot = 16 * (j % 2) + PH // 2 * p + j // 2
                for k, t in enumerate(QKV_CHUNKS[n]):
                    part, rows = val[k * sz:(k + 1) * sz], pl.ds(t * C + i * sz, sz)
                    buf[8 + slot + (zero if t else 0), rows, :] = part
                    if t and slot % 16:
                        buf[slot + zero, rows, :] = pltpu.roll(part, 1, 1)

        return _strassen(lambda i: pace(_dot(
            _halves(wt_v[g, n, i]), _halves(op_v[p, pl.ds(i * kw, kw), :]))), LV, emit)

    def attend(g, p):
        buf, probs = (qa_v, qb_v)[g % 2], []
        for j in range(PH):
            n = PH // 2 * p + j // 2
            slot = 16 * (j % 2) + 8 + n
            logits = [None] * WIN
            for dh in range(DH):
                q = buf[slot, pl.ds(dh * 8, 8), :]
                for w in range(WIN):
                    t = q * buf[slot - w, pl.ds(C + dh * 8, 8), :]
                    logits[w] = t if dh == 0 else logits[w] + t
                if dh % 4 == 3:
                    pin(op_v, logits[dh // 2])
                    yield
            for w in range(n + 1, WIN):
                logits[w] = jnp.where(lane == 0, -1e9, logits[w])
            m = _tree(jnp.maximum, logits)
            ex = [jnp.exp(t - m) for t in logits]
            inv = 1.0 / _tree(jnp.add, ex)
            probs.append((slot, [t * inv for t in ex]))
            yield
        for i in range(hp):
            cols = []
            for slot, pr in probs:
                cols.append(jnp.concatenate([_tree(jnp.add, [
                    pr[w] * buf[slot - w, pl.ds(2 * C + (2 * (h * hp + i) + e) * 8, 8), :]
                    for w in range(WIN)]) for h in range(PH) for e in range(2)], axis=0))
                if len(cols) < PH:
                    pin(op_v, cols[-1])
                    yield
            for n, b in enumerate(_rhs_terms(jnp.concatenate(cols, axis=1), LV)):
                op_v[p + zero, pl.ds((NP + n) * kw + (g * hp + i) * 8, 8), :] = _pairs(b)
            yield

    sums = {}

    def project(last, n, p, pace):
        def emit(blocks):
            for (i, j), val in blocks.items():
                for k, t in enumerate(OUT_CHUNKS[n]):
                    rows = pl.ds(t * C + i * sz, sz)
                    x = x_v[PH * p + j, rows, :] + val[k * sz:(k + 1) * sz]
                    (ya_v, yb_v)[p % 2][j + zero, rows, :] = x
                    if not last:
                        x_v[PH * p + j, rows, :] = x
                        sums[PH * p + j] = _sums(x, sums.get(PH * p + j))

        return _strassen(lambda i: pace(_dot(
            _halves(wot_v[n, i]), _halves(op_v[p, pl.ds((NP + i) * kw, kw), :]))), LV, emit)

    def out_copy(n):
        return pltpu.make_async_copy(io_v.at[n], out_w.at[:, n, :], sems.at[12 + n])

    def finish(last, p):
        y_v = (ya_v, yb_v)[p % 2]
        if last:
            for j in range(0, PH, 2):
                for b in range(D // C):
                    wd = _pairs(y_v[j:j + 2, pl.ds(b * C, C), :].reshape(2 * C, C))
                    io_v[(PH * p + j) // 2, :, b * C:(b + 1) * C] = wd.T
                    pin(op_v, wd)
                    yield
        else:
            for j, (m, s) in enumerate([_stats(sums[PH * p + j]) for j in range(PH)]):
                for b in range(D // C):
                    u = (y_v[j, pl.ds(b * C, C), :] - m) * s
                    u_v[PH * p + j + zero, pl.ds(b * C, C), :] = u
                    pin(op_v, u)
                    yield

    heads, chunks = D // C, range(len(QKV_CHUNKS))
    n_qkv, n_att, n_term = NP * len(chunks), 5 * PH + 8, kw // 16

    def first_heads():
        pace, stats = pacer(LAG, x_v), {}
        _run((inverse(D // CB - 1, zero), 8), (moments(0, stats), 4 * PH, 0.4, 0.7),
             (moments(1, stats), 4 * PH, 0.7, 1.0), (norm(0, stats), n_term, 0.8, 1.0))
        for p in range(groups):
            _run((_chain(qkv(0, n, p, pace) for n in chunks), n_qkv),
                 *[(norm(p + 1, stats), n_term)] * (p + 1 < groups),
                 *[(moments(p + 2, stats), 4 * PH)] * (p + 2 < groups))

    def next_heads(g):
        pace = pacer(LAG, (qa_v, qb_v)[1 - g % 2])
        early = [(attend(g, 0), n_att, 0.88, 1.0)] * (g == heads - 1)
        _run((_chain(qkv(g, n, p, pace) for n in chunks for p in range(groups)), n_qkv * groups),
             (_chain(attend(g - 1, p) for p in range(groups)), n_att * groups,
              0.0, 0.88 if early else 1.0), *early)

    def output(last):
        pace, n_fin = pacer(LAG, qb_v), 2 * PH if last else 4 * PH
        for p in range(groups):
            _run((_chain(project(last, n, p, pace) for n in range(len(OUT_CHUNKS))),
                  NP * len(OUT_CHUNKS)),
                 *[(attend(heads - 1, p + 1), n_att)] * (p + 1 < groups),
                 *[(finish(last, p - 1), n_fin, 0.3, 1.0)] * (p > 0))
        _run((finish(last, groups - 1), n_fin, 0.0, 0.5),
             *[(forward(0), 8)] * (not last))

    def layer(i):
        with jax.named_scope("conv"):
            for b in range(D // CB):
                pl.when(i == 0)(lambda: conv(True, b))
                pl.when(i == 1)(lambda: conv(False, b))
        with jax.named_scope("kv"):
            pl.when(zero == 0)(first_heads)
        with jax.named_scope("mid"):
            for g in range(1, heads):
                pl.when(zero < g)(lambda: next_heads(g))
        with jax.named_scope("attn"):
            pl.when(i == 0)(lambda: output(False))
            pl.when(i == 1)(lambda: output(True))

    _run((forward(0), 8))
    _loop(0, 2, layer)

    for p in range(R // 2):
        out_copy(p).start()
    for p in range(R // 2):
        out_copy(p).wait()


@jax.jit
def pallas_interleave_layers__ssm_conv_s4__sliding_local_dilated__prompt_kernel(
    A_u: jax.Array,
    A_A_re: jax.Array,
    A_A_im: jax.Array,
    A_B_re: jax.Array,
    A_B_im: jax.Array,
    A_C_re: jax.Array,
    A_C_im: jax.Array,
    A_log_dt: jax.Array,
    A_Dskip: jax.Array,
    B_x: jax.Array,
    B_wqkv: jax.Array,
    B_wo: jax.Array,
):
    del B_x
    assert A_u.shape == (1, L, D) and A_A_re.shape == (D, N) and A_A_re.dtype == BF16
    hbm = pl.BlockSpec(memory_space=pl.ANY)
    vmem = pl.BlockSpec(memory_space=pltpu.VMEM)
    out = pl.pallas_call(
        _kernel,
        in_specs=[hbm] * 7 + [vmem] * 2 + [hbm] * 4 + [pl.BlockSpec(memory_space=pltpu.SMEM)],
        out_specs=hbm,
        out_shape=jax.ShapeDtypeStruct((C, R, D), BF16),
        scratch_shapes=[
            pltpu.VMEM((R // 2, C, D), U32),
            pltpu.VMEM((6, D // 2, N), U32),
            pltpu.VMEM((D // 2, 3 * D), U32),
            pltpu.VMEM((D // C, D // 2, C), U32),
            pltpu.VMEM((2 * R, C, C), U32),
            pltpu.VMEM((R, C, C), U32),
            pltpu.VMEM((D, C), F32),
            pltpu.VMEM((D, C), F32),
            pltpu.VMEM((D // C, len(QKV_CHUNKS), NP, len(QKV_CHUNKS[0]) * C // PH // 2, D // PH),
                       U32),
            pltpu.VMEM((len(OUT_CHUNKS), NP, len(OUT_CHUNKS[0]) * C // PH // 2, D // PH),
                       U32),
            pltpu.VMEM((R + 1, D, C), F32),
            pltpu.VMEM((R, D, C), F32),
            pltpu.VMEM((R, D, C), F32),
            pltpu.VMEM((R, D, 2 * C), F32),
            pltpu.VMEM((R // PH + 1, NP * D // PH, C), U32),
            *[pltpu.VMEM((2, 448, 2 * C), F32)] * 2,
            *[pltpu.VMEM((R, CB, 2 * C), F32)] * 2,
            *[pltpu.VMEM((R, CB, 2 * C), F32)] * 2,
            *[pltpu.VMEM((2 * R + 1, 3 * C, C), F32)] * 2,
            *[pltpu.VMEM((PH, D, C), F32)] * 2,
            pltpu.SemaphoreType.DMA((24,)),
        ],
        compiler_params=pltpu.CompilerParams(vmem_limit_bytes=100 * 1024 * 1024),
    )(A_u.reshape(C, R, D), A_A_re, A_A_im, A_B_re, A_B_im, A_C_re, A_C_im,
      A_log_dt, A_Dskip, B_wqkv, B_wo, *_dft_tables(),
      np.zeros((1,), np.int32))
    return out.reshape(1, L, D)
```

```python
import ml_dtypes
import numpy as np

import jax
import jax.numpy as jnp
from jax import lax
import jax.experimental.pallas as pl
import jax.experimental.pallas.tpu as pltpu

L, D, N = 2048, 512, 128
R, C = 16, 128
DH, WIN = 16, 8
CB = 64
LV = 1
PH, NP = 2 ** LV, 7 ** LV
QKV_CHUNKS, OUT_CHUNKS = ((1,), (2,), (0,)), ((0,), (1,), (2,), (3,))
LAG = 7
EPS = 1e-5
F32, BF16, U32 = jnp.float32, jnp.bfloat16, jnp.uint32
_NT = (((1,), (1,)), ((), ()))


def _host_words(a):
    h = np.ascontiguousarray(a).astype(ml_dtypes.bfloat16).view(np.uint16).astype(np.uint32)
    return h[..., 0::2, :] | (h[..., 1::2, :] << 16)


def _dft_tables():
    t = R * np.arange(C)[None, :, None] + np.arange(R)[:, None, None]
    ang = 2.0 * np.pi * (np.arange(C)[None, None, :] + 0.5) * t / (2 * L)
    fwd = np.concatenate([np.cos(ang), -np.sin(ang)], axis=-1)
    p = (np.arange(C) - 7) % C
    fwd_k = fwd[:, 16 * (p % 8) + p // 8, :] / L
    inv = fwd.transpose(0, 2, 1)
    fwd, fwd_k = [np.concatenate([a[..., :C], a[..., C:]], axis=1) for a in (fwd, fwd_k)]
    return _host_words(np.concatenate([fwd, inv])), _host_words(fwd_k)


def _tap_offsets():
    l = np.arange(L)
    lr = l.astype(np.float32).astype(ml_dtypes.bfloat16).astype(np.float32).astype(np.int64)
    rho = (lr - (l // R) * R).reshape(8, 16, R)
    assert (rho == rho[:, :1]).all()
    return rho[:, 0].tolist()


def _cmul(a, b):
    return a[0] * b[0] - a[1] * b[1], a[0] * b[1] + a[1] * b[0]


def _csq(a):
    t = a[0] * a[1]
    return a[0] * a[0] - a[1] * a[1], t + t


def _twiddle(a, k, n):
    if k == 0:
        return a
    if 4 * k == n:
        return a[1], -a[0]
    h = float(np.sqrt(0.5))
    if 8 * k == n:
        return (a[0] + a[1]) * h, (a[1] - a[0]) * h
    if 8 * k == 3 * n:
        return (a[1] - a[0]) * h, (a[0] + a[1]) * (-h)
    w = (float(np.cos(2 * np.pi * k / n)), float(-np.sin(2 * np.pi * k / n)))
    return _cmul(a, w)


def _fft(x):
    n = len(x)
    if n == 1:
        return x
    if n == 2:
        return [(x[0][0] + x[1][0], x[0][1] + x[1][1]), (x[0][0] - x[1][0], x[0][1] - x[1][1])]
    e, o1, o3 = _fft(x[0::2]), _fft(x[1::4]), _fft(x[3::4])
    out = [None] * n
    q = n // 4
    for k in range(q):
        a, b = _twiddle(o1[k], k, n), _twiddle(o3[k], 3 * k, n)
        s = (a[0] + b[0], a[1] + b[1])
        d = (a[0] - b[0], a[1] - b[1])
        out[k] = (e[k][0] + s[0], e[k][1] + s[1])
        out[k + 2 * q] = (e[k][0] - s[0], e[k][1] - s[1])
        out[k + q] = (e[k + q][0] + d[1], e[k + q][1] - d[0])
        out[k + 3 * q] = (e[k + q][0] - d[1], e[k + q][1] + d[0])
    return out


def _ifft(x):
    return [(b, a) for a, b in _fft([(b, a) for a, b in x])]


def _tree(op, xs):
    while len(xs) > 1:
        xs = [op(*xs[i:i + 2]) if i + 1 < len(xs) else xs[i] for i in range(0, len(xs), 2)]
    return xs[0]


def _sums(x, acc=None):
    parts = [x[i:i + 8] for i in range(0, x.shape[0], 8)]
    new = _tree(jnp.add, parts), _tree(jnp.add, [t * t for t in parts])
    return new if acc is None else (acc[0] + new[0], acc[1] + new[1])


def _stats(acc):
    m, sq = [jnp.sum(t, axis=0, keepdims=True) * (1.0 / D) for t in acc]
    return m, lax.rsqrt(jnp.maximum(sq - m * m, 0.0) + EPS)


def _words(x):
    return pltpu.bitcast(x.astype(BF16), U32)


def _pairs(x):
    b = pltpu.bitcast(x.astype(BF16).astype(F32), U32)
    return b[x.shape[0] // 2:] | (b[:x.shape[0] // 2] >> 16)


def _halves(w):
    return pltpu.bitcast(w, BF16)


def _dot(a, b, dims=(((1,), (0,)), ((), ()))):
    return lax.dot_general(a.astype(BF16), b.astype(BF16), dims, preferred_element_type=F32)


def _split(src, table, r, rows):
    lo, hi = [_dot(src[n, rows, :], _halves(jnp.concatenate(
        [table[n, :C // 2], table[n, C // 2:]], axis=1))) for n in (r, r + 8)]
    d = lo - hi
    return lo + hi, jnp.concatenate(_twiddle((d[:, :C], d[:, C:]), r, R), axis=1)


def _run(*jobs):
    order = []
    for k, (_, n, *span) in enumerate(jobs):
        lo, hi = span or (0.0, 1.0)
        order += [(lo + (hi - lo) * i / n, k) for i in range(n)]
    for _, k in sorted(order):
        next(jobs[k][0])
    for job in jobs:
        for _ in job[0]:
            pass


def _chain(gens):
    for g in gens:
        yield from g


def _lhs_terms(a, levels):
    if not levels:
        return [jnp.concatenate(a, axis=0)]
    m, k = a[0].shape[0] // 2, a[0].shape[1] // 2
    terms = []
    for t in a:
        a11, a12, a21, a22 = t[:m, :k], t[:m, k:], t[m:, :k], t[m:, k:]
        terms.append((a11 + a22, a21 + a22, a22, a12 - a22, a21 - a11, a11, a11 + a12))
    return [x for ts in zip(*terms) for x in _lhs_terms(list(ts), levels - 1)]


def _rhs_terms(b, levels):
    if not levels:
        return [b]
    k, n = b.shape[0] // 2, b.shape[1] // 2
    b11, b12, b21, b22 = b[:k, :n], b[:k, n:], b[k:, :n], b[k:, n:]
    terms = (b11 + b22, b11, b21 - b11, b21 + b22, b11 + b12, b12 - b22, b22)
    return [x for t in terms for x in _rhs_terms(t, levels - 1)]


def _strassen(product, levels, emit=None, base=0):
    if not levels:
        out = {(0, 0): product(base)}
        if emit:
            emit(out)
        yield
        return out
    half, out = 2 ** (levels - 1), {}

    def term(i):
        return _strassen(product, levels - 1, None, base + i * 7 ** (levels - 1))

    def done(i, j, x):
        x = {(i * half + a, j * half + b): v for (a, b), v in x.items()}
        out.update(x)
        if emit:
            emit(x)

    def add(x, y):
        return {k: x[k] + y[k] for k in x}

    def sub(x, y):
        return {k: x[k] - y[k] for k in x}

    m1 = yield from term(0)
    m2 = yield from term(1)
    c22 = sub(m1, m2)
    m4 = yield from term(2)
    c11 = add(m1, m4)
    done(1, 0, add(m2, m4))
    c11 = add(c11, (yield from term(3)))
    c22 = add(c22, (yield from term(4)))
    m3 = yield from term(5)
    done(1, 1, add(c22, m3))
    m5 = yield from term(6)
    done(0, 0, sub(c11, m5))
    done(0, 1, add(m3, m5))
    return out


def _ds(start, size):
    return pl.ds(start if isinstance(start, int) else pl.multiple_of(start, size), size)


def _loop(lo, hi, body):
    lax.fori_loop(lo, hi, lambda i, c: (body(i), c)[1], 0)


def _kernel(x_hbm, are_hbm, aim_hbm, bre_hbm, bim_hbm, cre_hbm, cim_hbm, ldt_ref, dsk_ref,
            wqkv_hbm, wo_hbm, tab_hbm, fk_hbm, zero_s, out_hbm,
            io_v, par_v, wqkv_v, wo_v, tab_v, fk_v, dt_v, dk_v, wt_v, wot_v,
            x_v, u_v, kt_v, kh_v, op_v, sa_v, sb_v, za_v, zb_v,
            qa_v, qb_v, ya_v, yb_v, sems):
    srcs = (are_hbm, aim_hbm, bre_hbm, bim_hbm, cre_hbm, cim_hbm)
    par_cp = [pltpu.make_async_copy(s.bitcast(U32), par_v.at[i], sems.at[i])
              for i, s in enumerate(srcs)]
    x_w, out_w = x_hbm.bitcast(U32), out_hbm.bitcast(U32)
    x_cp = [pltpu.make_async_copy(x_w.at[:, i, :], io_v.at[i], sems.at[12 + i])
            for i in range(R // 2)]
    fk_cp = pltpu.make_async_copy(fk_hbm, fk_v, sems.at[7])
    tab_cp = pltpu.make_async_copy(tab_hbm, tab_v, sems.at[8])
    wqkv_cp = pltpu.make_async_copy(wqkv_hbm.bitcast(U32), wqkv_v, sems.at[10])
    wo_cp = [pltpu.make_async_copy(wo_hbm.bitcast(U32).at[:, pl.ds(t * C, C)], wo_v.at[t],
                                   sems.at[20 + t]) for t in range(D // C)]
    for cp in par_cp:
        cp.start()

    lane = lax.broadcasted_iota(jnp.int32, (8, C), 1)
    sub = lax.broadcasted_iota(jnp.int32, (8, C), 0)
    rho = _tap_offsets()

    zero = zero_s[0]

    def pin(ref, x):
        ref[ref.shape[0] - 1 + zero, :8, :C] = pltpu.bitcast(x[:8, :C], ref.dtype)

    regions = []

    def region(fn, *args):
        regions.append(fn)
        pl.when(zero < len(regions))(lambda: fn(*args))

    def pacer(lag, ref):
        queue = []

        def pace(x):
            queue.append(x)
            if len(queue) > lag:
                pin(ref, queue.pop(0))
            return x
        return pace

    dt_row = jnp.exp(ldt_ref[...].astype(F32).reshape(1, D)).astype(BF16).astype(F32)
    dk_row = dsk_ref[...].astype(F32).reshape(1, D)
    for b in range(D // C):
        cols = slice(b * C, (b + 1) * C)
        dt_v[cols, :] = jnp.broadcast_to(dt_row[:, cols], (C, C)).T
        dk_v[cols, :] = jnp.broadcast_to(dk_row[:, cols], (C, C)).T

    keys = [(s, p) for p in (16, *range(1, 16)) for s in range(8) if p == 16 or p in rho[s]]

    def flip(x):
        x = pltpu.roll(x, 4, 0)
        x = jnp.where((sub & 2) == 0, pltpu.roll(x, 6, 0), pltpu.roll(x, 2, 0))
        return jnp.where((sub & 1) == 0, pltpu.roll(x, 7, 0), pltpu.roll(x, 1, 0))

    def discretise(i):
        a_re, a_im, b_re, b_im, c_re, c_im = [
            _halves(par_v[n, pl.ds(i * 8, 8), :]).astype(F32) for n in range(6)]
        rows = pl.ds(i * 16, 16)
        dt = dt_v[rows, :]
        mag, ph = jnp.exp(dt * a_re), dt * a_im
        w = _cmul((c_re, c_im), (dt * b_re, dt * b_im))
        tap0 = dk_v[rows, :] + jnp.sum(w[0], axis=1, keepdims=True)
        return mag * jnp.cos(ph), mag * jnp.sin(ph), *w, tap0

    def taps(i, a_re, a_im, w_re, w_im, tap0):
        rows = pl.ds(i * 8, 8)
        a = {1: (a_re, a_im)}
        for n in range(8):
            a[2 << n] = _csq(a[1 << n])
        right = [(jnp.ones((8, C), F32), jnp.zeros((8, C), F32)), (flip(a[16][0]), -flip(a[16][1]))]
        for j in range(2, 16):
            right.append(_csq(right[j // 2]) if j % 2 == 0 else _cmul(right[j - 1], right[1]))
        left = {(0, 0): (w_re, w_im)}
        for s, p in keys:
            left[s, p] = (_cmul(left[s - 1, p], a[256]) if s else
                          _cmul(left[0, p & (p - 1)], a[p & -p]))
        res = _dot(*[jnp.concatenate([jnp.concatenate(v, axis=1) for v in vals], axis=0)
                     for vals in ([left[k] for k in keys], right)], _NT)
        part = {k: pltpu.roll(res[8 * n:8 * n + 8], k[0], 1, stride=1, stride_axis=0)
                for n, k in enumerate(keys)}
        pos, memo = (lane - 7) & (C - 1), {}

        def merge(ps, s=0):
            if len(ps) == 1 or not any(ps):
                return part[s, ps[0]]
            if (ps, s) not in memo:
                h = len(ps) // 2
                memo[ps, s] = jnp.where((pos & h) == 0, merge(ps[:h], s), merge(ps[h:], s + h))
            return memo[ps, s]

        t16 = merge((16,) * 8)
        t0 = jnp.where(pos < 8, pltpu.roll(t16, 9, 1), pltpu.roll(t16, 8, 1))
        t0 = jnp.where(pos == 0, tap0, t0)
        for s in range(8):
            part[s, 0] = t0
        for r in range(R):
            kt_v[r, rows, :] = merge(tuple(rho[s][r] for s in range(8)))

    def filters(lo, hi):
        for i in range(lo, hi):
            vals = discretise(i)
            for h in range(2):
                taps(2 * i + h, *[v[8 * h:8 * h + 8] for v in vals])

    for cp in par_cp:
        cp.wait()
    for cp in x_cp + [fk_cp, wqkv_cp] + wo_cp + [tab_cp]:
        cp.start()
    with jax.named_scope("filter"):
        filters(0, D // 16)

    def spectra():
        for r in range(8):
            for b in range(D // C):
                rows = pl.ds(b * C, C)
                kh_v[r, rows, :], kh_v[r + 8, rows, :] = _split(kt_v, fk_v, r, rows)
                yield

    def load():
        for i in range(R // 2):
            acc = [None, None]
            for b in range(D // C):
                wd = io_v[i, :, b * C:(b + 1) * C].T
                for e, w in enumerate((wd << 16, wd & jnp.uint32(0xFFFF0000))):
                    x = pltpu.bitcast(w, F32)
                    x_v[2 * i + e + zero, pl.ds(b * C, C), :] = x
                    acc[e] = _sums(x, acc[e])
                yield
            for e in range(2):
                m, s = _stats(acc[e])
                for b in range(D // C):
                    u_v[2 * i + e, pl.ds(b * C, C), :] = (x_v[2 * i + e, pl.ds(b * C, C), :] - m) * s
                yield

    hp = DH // 2 // PH

    def weights():
        row = lax.broadcasted_iota(jnp.int32, (C, C), 0)
        col = lax.broadcasted_iota(jnp.int32, (C, C), 1)
        pick = jnp.where(col == (row & 7) * DH + (row >> 3), 1.0, 0.0)
        for g in range(D // C):
            for n, chunk in enumerate(QKV_CHUNKS):
                tiles = [_dot(pick * (DH ** -0.5 if t == 0 else 1.0),
                              _halves(wqkv_v[:, pl.ds(t * D + g * C, C)]), _NT) for t in chunk]
                for i, a in enumerate(_lhs_terms(tiles, LV)):
                    wt_v[g, n, i] = _words(a)
                yield
        for n, chunk in enumerate(OUT_CHUNKS):
            tiles = [_halves(jnp.concatenate(
                [wo_v[t, pl.ds(g * C // 2 + h * hp + i, 8, stride=DH // 2), :]
                 for h in range(PH) for g in range(D // C) for i in range(hp)],
                axis=0)).T.astype(F32) for t in chunk]
            for i, a in enumerate(_lhs_terms(tiles, LV)):
                wot_v[n, i] = _words(a)
            yield

    for cp in x_cp + [fk_cp, wqkv_cp] + wo_cp:
        cp.wait()
    with jax.named_scope("load"):
        region(_run, (spectra(), 32), (load(), 48),
               (weights(), 4 * len(QKV_CHUNKS) + len(OUT_CHUNKS)))
    tab_cp.wait()

    def forward(b):
        s_v = (sa_v, sb_v)[b % 2]
        for r in range(8):
            s_v[r], s_v[r + 8] = _split(u_v, tab_v, r, pl.ds(b * CB, CB))
            yield

    def inverse(b, shift=0):
        z_v = (za_v, zb_v)[b % 2]
        for r in range(8):
            ev = z_v[r]
            od = _twiddle((z_v[r + 8, :, C:], z_v[r + 8, :, :C]), r, R)
            od = jnp.concatenate(od[::-1], axis=1)
            for n, z in ((r, ev + od), (r + 8, ev - od)):
                rows = pl.ds(b * CB, CB)
                x_v[n + shift, rows, :] = x_v[n, rows, :] + _dot(z, _halves(tab_v[R + n]))
            yield

    def mix(first, b):
        s_v, z_v = (sa_v, sb_v)[b % 2], (za_v, zb_v)[b % 2]
        for i in range(CB // 4):
            sr, kr = pl.ds(i // 2 * 8, 8), pl.ds(b * CB + i // 2 * 8, 8)
            rs = range(i % 2 * 8, i % 2 * 8 + 8)
            kf = [(kh_v[r, kr, :C], kh_v[r, kr, C:]) for r in rs]
            if first:
                kf = _fft(kf)
                for r, k in zip(rs, kf):
                    kh_v[r, kr, :C], kh_v[r, kr, C:] = k
            uf = _fft([(s_v[r, sr, :C], s_v[r, sr, C:]) for r in rs])
            for r, z in zip(rs, _ifft([_cmul(*t) for t in zip(uf, kf)])):
                z_v[r, sr, :C], z_v[r, sr, C:] = z
            yield

    def conv(first, b):
        _run(*[(forward(b + 1), 8)] * (b + 1 < D // CB),
             *[(inverse(b - 1), 8, 0.0625, 1.0625)] * (b > 0), (mix(first, b), CB // 4))

    sz, kw, groups = C // PH, D // PH // 2, R // PH

    def moments(p, stats):
        for r in range(PH * p, PH * p + PH):
            acc = None
            for b in range(D // C):
                for row in range(b * C, b * C + C, 32):
                    acc = _sums(x_v[r, pl.ds(row, 32), :], acc)
                pin(op_v, acc[1])
                stats[r] = acc if b + 1 < D // C else _stats(acc)
                yield

    def terms(tile, i):
        return _rhs_terms(jnp.concatenate([jnp.concatenate(
            [tile(j, h * 2 * kw + 32 * i) for j in range(PH)], axis=1) for h in range(PH)],
            axis=0), LV)

    def norm(p, stats):
        for i in range(kw // 16):
            for n, b in enumerate(terms(lambda j, row: (
                    x_v[PH * p + j, pl.ds(row, 32), :] - stats[PH * p + j][0]) * stats[PH * p + j][1], i)):
                op_v[p + zero, pl.ds(n * kw + 16 * i, 16), :] = _words(b)
            yield

    def qkv(g, n, p, pace):
        buf = (qa_v, qb_v)[g % 2]

        def emit(blocks):
            for (i, j), val in blocks.items():
                slot = 16 * (j % 2) + PH // 2 * p + j // 2
                for k, t in enumerate(QKV_CHUNKS[n]):
                    part, rows = val[k * sz:(k + 1) * sz], pl.ds(t * C + i * sz, sz)
                    buf[8 + slot + (zero if t else 0), rows, :] = part
                    if t and slot % 16:
                        buf[slot + zero, rows, :] = pltpu.roll(part, 1, 1)

        return _strassen(lambda i: pace(_dot(
            _halves(wt_v[g, n, i]), _halves(op_v[p, pl.ds(i * kw, kw), :]))), LV, emit)

    def attend(g, p):
        buf, probs = (qa_v, qb_v)[g % 2], []
        for j in range(PH):
            n = PH // 2 * p + j // 2
            slot = 16 * (j % 2) + 8 + n
            logits = [None] * WIN
            for dh in range(DH):
                q = buf[slot, pl.ds(dh * 8, 8), :]
                for w in range(WIN):
                    t = q * buf[slot - w, pl.ds(C + dh * 8, 8), :]
                    logits[w] = t if dh == 0 else logits[w] + t
                if dh % 4 == 3:
                    pin(op_v, logits[dh // 2])
                    yield
            for w in range(n + 1, WIN):
                logits[w] = jnp.where(lane == 0, -1e9, logits[w])
            m = _tree(jnp.maximum, logits)
            ex = [jnp.exp(t - m) for t in logits]
            inv = 1.0 / _tree(jnp.add, ex)
            probs.append((slot, [t * inv for t in ex]))
            yield
        for i in range(hp):
            cols = []
            for slot, pr in probs:
                cols.append(jnp.concatenate([_tree(jnp.add, [
                    pr[w] * buf[slot - w, pl.ds(2 * C + (2 * (h * hp + i) + e) * 8, 8), :]
                    for w in range(WIN)]) for h in range(PH) for e in range(2)], axis=0))
                if len(cols) < PH:
                    pin(op_v, cols[-1])
                    yield
            for n, b in enumerate(_rhs_terms(jnp.concatenate(cols, axis=1), LV)):
                op_v[p + zero, pl.ds((NP + n) * kw + (g * hp + i) * 8, 8), :] = _pairs(b)
            yield

    sums = {}

    def project(last, n, p, pace):
        def emit(blocks):
            for (i, j), val in blocks.items():
                for k, t in enumerate(OUT_CHUNKS[n]):
                    rows = pl.ds(t * C + i * sz, sz)
                    x = x_v[PH * p + j, rows, :] + val[k * sz:(k + 1) * sz]
                    (ya_v, yb_v)[p % 2][j + zero, rows, :] = x
                    if not last:
                        x_v[PH * p + j, rows, :] = x
                        sums[PH * p + j] = _sums(x, sums.get(PH * p + j))

        return _strassen(lambda i: pace(_dot(
            _halves(wot_v[n, i]), _halves(op_v[p, pl.ds((NP + i) * kw, kw), :]))), LV, emit)

    def out_copy(n):
        return pltpu.make_async_copy(io_v.at[n], out_w.at[:, n, :], sems.at[12 + n])

    def finish(last, p):
        y_v = (ya_v, yb_v)[p % 2]
        if last:
            for j in range(0, PH, 2):
                for b in range(D // C):
                    wd = _pairs(y_v[j:j + 2, pl.ds(b * C, C), :].reshape(2 * C, C))
                    io_v[(PH * p + j) // 2, :, b * C:(b + 1) * C] = wd.T
                    pin(op_v, wd)
                    yield
        else:
            for j, (m, s) in enumerate([_stats(sums[PH * p + j]) for j in range(PH)]):
                for b in range(D // C):
                    u = (y_v[j, pl.ds(b * C, C), :] - m) * s
                    u_v[PH * p + j + zero, pl.ds(b * C, C), :] = u
                    pin(op_v, u)
                    yield

    heads, chunks = D // C, range(len(QKV_CHUNKS))
    n_qkv, n_att, n_term = NP * len(chunks), 5 * PH + 8, kw // 16

    def first_heads():
        pace, stats = pacer(LAG, x_v), {}
        _run((inverse(D // CB - 1, zero), 8), (moments(0, stats), 4 * PH, 0.4, 0.7),
             (moments(1, stats), 4 * PH, 0.7, 1.0), (norm(0, stats), n_term, 0.8, 1.0))
        for p in range(groups):
            _run((_chain(qkv(0, n, p, pace) for n in chunks), n_qkv),
                 *[(norm(p + 1, stats), n_term)] * (p + 1 < groups),
                 *[(moments(p + 2, stats), 4 * PH)] * (p + 2 < groups))

    def next_heads(g):
        pace = pacer(LAG, (qa_v, qb_v)[1 - g % 2])
        early = [(attend(g, 0), n_att, 0.88, 1.0)] * (g == heads - 1)
        _run((_chain(qkv(g, n, p, pace) for n in chunks for p in range(groups)), n_qkv * groups),
             (_chain(attend(g - 1, p) for p in range(groups)), n_att * groups,
              0.0, 0.88 if early else 1.0), *early)

    def output(last):
        pace, n_fin = pacer(LAG, qb_v), 2 * PH if last else 4 * PH
        for p in range(groups):
            if last and p > 1:
                for n in range(PH // 2):
                    out_copy(PH // 2 * (p - 2) + n).start()
            _run((_chain(project(last, n, p, pace) for n in range(len(OUT_CHUNKS))),
                  NP * len(OUT_CHUNKS)),
                 *[(attend(heads - 1, p + 1), n_att)] * (p + 1 < groups),
                 *[(finish(last, p - 1), n_fin, 0.3, 1.0)] * (p > 0))
        _run((finish(last, groups - 1), n_fin, 0.0, 0.5),
             *[(forward(0), 8)] * (not last))

    _run((forward(0), 8))
    for last in (False, True):
        with jax.named_scope("conv"):
            for b in range(D // CB):
                region(conv, not last, b)
        with jax.named_scope("kv"):
            region(first_heads)
        with jax.named_scope("mid"):
            for g in range(1, heads):
                region(next_heads, g)
        with jax.named_scope("attn"):
            region(output, last)

    for p in range(R // 2 - PH, R // 2):
        out_copy(p).start()
    for p in range(R // 2):
        out_copy(p).wait()


@jax.jit
def pallas_interleave_layers__ssm_conv_s4__sliding_local_dilated__prompt_kernel(
    A_u: jax.Array,
    A_A_re: jax.Array,
    A_A_im: jax.Array,
    A_B_re: jax.Array,
    A_B_im: jax.Array,
    A_C_re: jax.Array,
    A_C_im: jax.Array,
    A_log_dt: jax.Array,
    A_Dskip: jax.Array,
    B_x: jax.Array,
    B_wqkv: jax.Array,
    B_wo: jax.Array,
):
    del B_x
    assert A_u.shape == (1, L, D) and A_A_re.shape == (D, N) and A_A_re.dtype == BF16
    hbm = pl.BlockSpec(memory_space=pl.ANY)
    vmem = pl.BlockSpec(memory_space=pltpu.VMEM)
    out = pl.pallas_call(
        _kernel,
        in_specs=[hbm] * 7 + [vmem] * 2 + [hbm] * 4 + [pl.BlockSpec(memory_space=pltpu.SMEM)],
        out_specs=hbm,
        out_shape=jax.ShapeDtypeStruct((C, R, D), BF16),
        scratch_shapes=[
            pltpu.VMEM((R // 2, C, D), U32),
            pltpu.VMEM((6, D // 2, N), U32),
            pltpu.VMEM((D // 2, 3 * D), U32),
            pltpu.VMEM((D // C, D // 2, C), U32),
            pltpu.VMEM((2 * R, C, C), U32),
            pltpu.VMEM((R, C, C), U32),
            pltpu.VMEM((D, C), F32),
            pltpu.VMEM((D, C), F32),
            pltpu.VMEM((D // C, len(QKV_CHUNKS), NP, len(QKV_CHUNKS[0]) * C // PH // 2, D // PH),
                       U32),
            pltpu.VMEM((len(OUT_CHUNKS), NP, len(OUT_CHUNKS[0]) * C // PH // 2, D // PH),
                       U32),
            pltpu.VMEM((R + 1, D, C), F32),
            pltpu.VMEM((R, D, C), F32),
            pltpu.VMEM((R, D, C), F32),
            pltpu.VMEM((R, D, 2 * C), F32),
            pltpu.VMEM((R // PH + 1, NP * D // PH, C), U32),
            *[pltpu.VMEM((R, CB, 2 * C), F32)] * 2,
            *[pltpu.VMEM((R, CB, 2 * C), F32)] * 2,
            *[pltpu.VMEM((2 * R + 1, 3 * C, C), F32)] * 2,
            *[pltpu.VMEM((PH, D, C), F32)] * 2,
            pltpu.SemaphoreType.DMA((24,)),
        ],
        compiler_params=pltpu.CompilerParams(vmem_limit_bytes=100 * 1024 * 1024),
    )(A_u.reshape(C, R, D), A_A_re, A_A_im, A_B_re, A_B_im, A_C_re, A_C_im,
      A_log_dt, A_Dskip, B_wqkv, B_wo, *_dft_tables(),
      np.zeros((1,), np.int32))
    return out.reshape(1, L, D)
```

```python
import ml_dtypes
import numpy as np

import jax
import jax.numpy as jnp
from jax import lax
import jax.experimental.pallas as pl
import jax.experimental.pallas.tpu as pltpu

L, D, N = 2048, 512, 128
R, C = 16, 128
DH, WIN = 16, 8
CB = 64
LV = 1
PH, NP = 2 ** LV, 7 ** LV
QKV_CHUNKS, OUT_CHUNKS = ((1,), (2,), (0,)), ((0,), (1,), (2,), (3,))
PLAN = ((1, 0, 0), (3, 1, 0), (6, 3, 1), (8, 5, 3), (8, 7, 5), (8, 8, 7))
LAG = 7
HEAD = 3
EPS = 1e-5
F32, BF16, U32 = jnp.float32, jnp.bfloat16, jnp.uint32
_NT = (((1,), (1,)), ((), ()))


def _host_words(a):
    h = np.ascontiguousarray(a).astype(ml_dtypes.bfloat16).view(np.uint16).astype(np.uint32)
    return h[..., 0::2, :] | (h[..., 1::2, :] << 16)


def _dft_tables():
    t = R * np.arange(C)[None, :, None] + np.arange(R)[:, None, None]
    ang = 2.0 * np.pi * (np.arange(C)[None, None, :] + 0.5) * t / (2 * L)
    fwd = np.concatenate([np.cos(ang), -np.sin(ang)], axis=-1)
    p = (np.arange(C) - 7) % C
    fwd_k = fwd[:, 16 * (p % 8) + p // 8, :] / L
    inv = fwd.transpose(0, 2, 1)
    fwd, fwd_k = [np.concatenate([a[..., :C], a[..., C:]], axis=1) for a in (fwd, fwd_k)]
    return _host_words(np.concatenate([fwd, inv])), _host_words(fwd_k)


def _tap_offsets():
    l = np.arange(L)
    lr = l.astype(np.float32).astype(ml_dtypes.bfloat16).astype(np.float32).astype(np.int64)
    rho = (lr - (l // R) * R).reshape(8, 16, R)
    assert (rho == rho[:, :1]).all()
    return rho[:, 0].tolist()


def _cmul(a, b):
    return a[0] * b[0] - a[1] * b[1], a[0] * b[1] + a[1] * b[0]


def _csq(a):
    t = a[0] * a[1]
    return a[0] * a[0] - a[1] * a[1], t + t


def _twiddle(a, k, n):
    if k == 0:
        return a
    if 4 * k == n:
        return a[1], -a[0]
    h = float(np.sqrt(0.5))
    if 8 * k == n:
        return (a[0] + a[1]) * h, (a[1] - a[0]) * h
    if 8 * k == 3 * n:
        return (a[1] - a[0]) * h, (a[0] + a[1]) * (-h)
    w = (float(np.cos(2 * np.pi * k / n)), float(-np.sin(2 * np.pi * k / n)))
    return _cmul(a, w)


def _fft(x):
    n = len(x)
    if n == 1:
        return x
    if n == 2:
        return [(x[0][0] + x[1][0], x[0][1] + x[1][1]), (x[0][0] - x[1][0], x[0][1] - x[1][1])]
    e, o1, o3 = _fft(x[0::2]), _fft(x[1::4]), _fft(x[3::4])
    out = [None] * n
    q = n // 4
    for k in range(q):
        a, b = _twiddle(o1[k], k, n), _twiddle(o3[k], 3 * k, n)
        s = (a[0] + b[0], a[1] + b[1])
        d = (a[0] - b[0], a[1] - b[1])
        out[k] = (e[k][0] + s[0], e[k][1] + s[1])
        out[k + 2 * q] = (e[k][0] - s[0], e[k][1] - s[1])
        out[k + q] = (e[k + q][0] + d[1], e[k + q][1] - d[0])
        out[k + 3 * q] = (e[k + q][0] - d[1], e[k + q][1] + d[0])
    return out


def _ifft(x):
    return [(b, a) for a, b in _fft([(b, a) for a, b in x])]


def _tree(op, xs):
    while len(xs) > 1:
        xs = [op(*xs[i:i + 2]) if i + 1 < len(xs) else xs[i] for i in range(0, len(xs), 2)]
    return xs[0]


def _sums(x, acc=None):
    parts = [x[i:i + 8] for i in range(0, x.shape[0], 8)]
    new = _tree(jnp.add, parts), _tree(jnp.add, [t * t for t in parts])
    return new if acc is None else (acc[0] + new[0], acc[1] + new[1])


def _stats(acc):
    m, sq = [jnp.sum(t, axis=0, keepdims=True) * (1.0 / D) for t in acc]
    return m, lax.rsqrt(jnp.maximum(sq - m * m, 0.0) + EPS)


def _words(x):
    return pltpu.bitcast(x.astype(BF16), U32)


def _pairs(x):
    b = pltpu.bitcast(x, U32) + jnp.uint32(0x8000)
    return (b[x.shape[0] // 2:] & jnp.uint32(0xFFFF0000)) | (b[:x.shape[0] // 2] >> 16)


def _halves(w):
    return pltpu.bitcast(w, BF16)


def _dot(a, b, dims=(((1,), (0,)), ((), ()))):
    return lax.dot_general(a.astype(BF16), b.astype(BF16), dims, preferred_element_type=F32)


def _split(src, table, r, rows):
    lo, hi = [_dot(src[n, rows, :], _halves(jnp.concatenate(
        [table[n, :C // 2], table[n, C // 2:]], axis=1))) for n in (r, r + 8)]
    d = lo - hi
    return lo + hi, jnp.concatenate(_twiddle((d[:, :C], d[:, C:]), r, R), axis=1)


def _run(*jobs):
    order = []
    for k, (_, n, *span) in enumerate(jobs):
        lo, hi = span or (0.0, 1.0)
        order += [(lo + (hi - lo) * i / n, k) for i in range(n)]
    for _, k in sorted(order):
        next(jobs[k][0])
    for job in jobs:
        for _ in job[0]:
            pass


def _chain(gens):
    for g in gens:
        yield from g


def _lhs_terms(a, levels):
    if not levels:
        return [jnp.concatenate(a, axis=0)]
    m, k = a[0].shape[0] // 2, a[0].shape[1] // 2
    terms = []
    for t in a:
        a11, a12, a21, a22 = t[:m, :k], t[:m, k:], t[m:, :k], t[m:, k:]
        terms.append((a11 + a22, a21 + a22, a22, a12 - a22, a21 - a11, a11, a11 + a12))
    return [x for ts in zip(*terms) for x in _lhs_terms(list(ts), levels - 1)]


def _rhs_terms(b, levels):
    if not levels:
        return [b]
    k, n = b.shape[0] // 2, b.shape[1] // 2
    b11, b12, b21, b22 = b[:k, :n], b[:k, n:], b[k:, :n], b[k:, n:]
    terms = (b11 + b22, b11, b21 - b11, b21 + b22, b11 + b12, b12 - b22, b22)
    return [x for t in terms for x in _rhs_terms(t, levels - 1)]


def _strassen(product, levels, emit=None, base=0):
    if not levels:
        out = {(0, 0): product(base)}
        if emit:
            emit(out)
        yield
        return out
    half, out = 2 ** (levels - 1), {}

    def term(i):
        return _strassen(product, levels - 1, None, base + i * 7 ** (levels - 1))

    def done(i, j, x):
        x = {(i * half + a, j * half + b): v for (a, b), v in x.items()}
        out.update(x)
        if emit:
            emit(x)

    def add(x, y):
        return {k: x[k] + y[k] for k in x}

    def sub(x, y):
        return {k: x[k] - y[k] for k in x}

    m1 = yield from term(0)
    m2 = yield from term(1)
    c22 = sub(m1, m2)
    m4 = yield from term(2)
    c11 = add(m1, m4)
    done(1, 0, add(m2, m4))
    c11 = add(c11, (yield from term(3)))
    c22 = add(c22, (yield from term(4)))
    m3 = yield from term(5)
    done(1, 1, add(c22, m3))
    m5 = yield from term(6)
    done(0, 0, sub(c11, m5))
    done(0, 1, add(m3, m5))
    return out


def _ds(start, size):
    return pl.ds(start if isinstance(start, int) else pl.multiple_of(start, size), size)


def _loop(lo, hi, body):
    lax.fori_loop(lo, hi, lambda i, c: (body(i), c)[1], 0)


def _kernel(x_hbm, are_hbm, aim_hbm, bre_hbm, bim_hbm, cre_hbm, cim_hbm, ldt_hbm, dsk_hbm,
            wqkv_hbm, wo_hbm, tab_hbm, fk_hbm, zero_hbm, out_hbm,
            io_v, par_v, wqkv_v, wo_v, tab_v, fk_v, dt_v, dk_v, wt_v, wot_v,
            x_v, u_v, kt_v, kh_v, op_v, s_v,
            qa_v, qb_v, ya_v, yb_v, ldt_ref, dsk_ref, zero_s, sems):
    srcs = (are_hbm, aim_hbm, bre_hbm, bim_hbm, cre_hbm, cim_hbm)
    par_cp = [[pltpu.make_async_copy(s.bitcast(U32).at[rows], par_v.at[i, rows], sems.at[k])
               for i, s in enumerate(srcs)]
              for k, rows in enumerate((pl.ds(0, HEAD * 8), pl.ds(HEAD * 8, D // 2 - HEAD * 8)))]
    small_cp = [pltpu.make_async_copy(*pair, sems.at[2 + i]) for i, pair in enumerate(
        ((ldt_hbm, ldt_ref), (dsk_hbm, dsk_ref), (zero_hbm, zero_s)))]
    x_w, out_w = x_hbm.bitcast(U32), out_hbm.bitcast(U32)
    x_cp = [pltpu.make_async_copy(x_w.at[:, i, :], io_v.at[i], sems.at[12 + i])
            for i in range(R // 2)]
    fk_cp = pltpu.make_async_copy(fk_hbm, fk_v.at[:R], sems.at[7])
    tab_cp = pltpu.make_async_copy(tab_hbm, tab_v, sems.at[8])
    wqkv_cp = pltpu.make_async_copy(wqkv_hbm.bitcast(U32), wqkv_v, sems.at[10])
    wo_cp = [pltpu.make_async_copy(wo_hbm.bitcast(U32).at[:, pl.ds(t * C, C)], wo_v.at[t],
                                   sems.at[20 + t]) for t in range(D // C)]
    for cp in small_cp + par_cp[0] + par_cp[1]:
        cp.start()
    for cp in small_cp + par_cp[0]:
        cp.wait()

    lane = lax.broadcasted_iota(jnp.int32, (8, C), 1)
    sub = lax.broadcasted_iota(jnp.int32, (8, C), 0)
    rho = _tap_offsets()

    zero = zero_s[0]

    def pin(ref, x):
        ref[ref.shape[0] - 1 + zero, :8, :C] = pltpu.bitcast(x[:8, :C], ref.dtype)

    regions = []

    def region(fn, *args):
        regions.append(fn)
        pl.when(zero < len(regions))(lambda: fn(*args))

    def pacer(lag, ref):
        queue = []

        def pace(x):
            queue.append(x)
            if len(queue) > lag:
                pin(ref, queue.pop(0))
            return x
        return pace

    dt_row = jnp.exp(ldt_ref[...].astype(F32).reshape(1, D)).astype(BF16).astype(F32)
    dk_row = dsk_ref[...].astype(F32).reshape(1, D)
    for b in range(D // C):
        cols = slice(b * C, (b + 1) * C)
        dt_v[cols, :] = jnp.broadcast_to(dt_row[:, cols], (C, C)).T
        dk_v[cols, :] = jnp.broadcast_to(dk_row[:, cols], (C, C)).T

    keys = [(s, p) for p in (16, *range(1, 16)) for s in range(8) if p == 16 or p in rho[s]]

    def flip(x):
        x = pltpu.roll(x, 4, 0)
        x = jnp.where((sub & 2) == 0, pltpu.roll(x, 6, 0), pltpu.roll(x, 2, 0))
        return jnp.where((sub & 1) == 0, pltpu.roll(x, 7, 0), pltpu.roll(x, 1, 0))

    def discretise(i):
        a_re, a_im, b_re, b_im, c_re, c_im = [
            _halves(par_v[n, pl.ds(i * 8, 8), :]).astype(F32) for n in range(6)]
        rows = pl.ds(i * 16, 16)
        dt = dt_v[rows, :]
        mag, ph = jnp.exp(dt * a_re), dt * a_im
        w = _cmul((c_re, c_im), (dt * b_re, dt * b_im))
        tap0 = dk_v[rows, :] + jnp.sum(w[0], axis=1, keepdims=True)
        return mag * jnp.cos(ph), mag * jnp.sin(ph), *w, tap0

    def taps(i, a_re, a_im, w_re, w_im, tap0):
        rows = pl.ds(i * 8, 8)
        a = {1: (a_re, a_im)}
        for n in range(8):
            a[2 << n] = _csq(a[1 << n])
        right = [(jnp.ones((8, C), F32), jnp.zeros((8, C), F32)), (flip(a[16][0]), -flip(a[16][1]))]
        for j in range(2, 16):
            right.append(_csq(right[j // 2]) if j % 2 == 0 else _cmul(right[j - 1], right[1]))
        left = {(0, 0): (w_re, w_im)}
        for s, p in keys:
            left[s, p] = (_cmul(left[s - 1, p], a[256]) if s else
                          _cmul(left[0, p & (p - 1)], a[p & -p]))
        res = _dot(*[jnp.concatenate([jnp.concatenate(v, axis=1) for v in vals], axis=0)
                     for vals in ([left[k] for k in keys], right)], _NT)
        part = {k: pltpu.roll(res[8 * n:8 * n + 8], k[0], 1, stride=1, stride_axis=0)
                for n, k in enumerate(keys)}
        pos, memo = (lane - 7) & (C - 1), {}

        def merge(ps, s=0):
            if len(ps) == 1 or not any(ps):
                return part[s, ps[0]]
            if (ps, s) not in memo:
                h = len(ps) // 2
                memo[ps, s] = jnp.where((pos & h) == 0, merge(ps[:h], s), merge(ps[h:], s + h))
            return memo[ps, s]

        t16 = merge((16,) * 8)
        t0 = jnp.where(pos < 8, pltpu.roll(t16, 9, 1), pltpu.roll(t16, 8, 1))
        t0 = jnp.where(pos == 0, tap0, t0)
        for s in range(8):
            part[s, 0] = t0
        for r in range(R):
            kt_v[r, rows, :] = merge(tuple(rho[s][r] for s in range(8)))

    def filters(lo, hi):
        for i in range(lo, hi):
            vals = discretise(i)
            for h in range(2):
                taps(2 * i + h, *[v[8 * h:8 * h + 8] for v in vals])

    with jax.named_scope("filter"):
        filters(0, HEAD)
        for cp in x_cp + [fk_cp, wqkv_cp] + wo_cp + [tab_cp]:
            cp.start()
        for cp in par_cp[1]:
            cp.wait()
        filters(HEAD, D // 16)

    def spectra():
        pace = pacer(2, io_v)
        for r in range(8):
            for b in range(D // C):
                rows = pl.ds(b * C, C)
                ev, od = _split(kt_v, fk_v, r, rows)
                kh_v[r, rows, :], kh_v[r + 8, rows, :] = pace(ev), od
                yield

    def load():
        stats = []
        for i in range(R // 2 + 1):
            acc = [None, None]
            for b in range(D // C):
                rows = pl.ds(b * C, C)
                for e, (m, s) in enumerate(stats):
                    u_v[2 * i - 2 + e, rows, :] = u = (x_v[2 * i - 2 + e, rows, :] - m) * s
                    pin(fk_v, u)
                if i < R // 2:
                    wd = io_v[i, :, rows].T
                    for e, w in enumerate((wd << 16, wd & jnp.uint32(0xFFFF0000))):
                        x = pltpu.bitcast(w, F32)
                        x_v[2 * i + e + zero, rows, :] = x
                        acc[e] = _sums(x, acc[e])
                yield
            stats = [_stats(t) for t in acc if t]

    hp = DH // 2 // PH

    def weights():
        row = lax.broadcasted_iota(jnp.int32, (C, C), 0)
        col = lax.broadcasted_iota(jnp.int32, (C, C), 1)
        pick = jnp.where(col == (row & 7) * DH + (row >> 3), 1.0, 0.0)
        for g in range(D // C):
            for n, chunk in enumerate(QKV_CHUNKS):
                tiles = [_dot(pick * (DH ** -0.5 if t == 0 else 1.0),
                              _halves(wqkv_v[:, pl.ds(t * D + g * C, C)]), _NT) for t in chunk]
                for i, a in enumerate(_lhs_terms(tiles, LV)):
                    wt_v[g, n, i] = _words(a)
                yield
        for n, chunk in enumerate(OUT_CHUNKS):
            tiles = [_halves(jnp.concatenate(
                [wo_v[t, pl.ds(g * C // 2 + h * hp + i, 8, stride=DH // 2), :]
                 for h in range(PH) for g in range(D // C) for i in range(hp)],
                axis=0)).T.astype(F32) for t in chunk]
            for i, a in enumerate(_lhs_terms(tiles, LV)):
                wot_v[n, i] = _words(a)
            yield

    for cp in x_cp + [fk_cp, wqkv_cp] + wo_cp:
        cp.wait()
    with jax.named_scope("load"):
        region(_run, (spectra(), 32), (load(), 36),
               (weights(), 4 * len(QKV_CHUNKS) + len(OUT_CHUNKS)))
    tab_cp.wait()

    def forward(b):
        rows = pl.ds(b * CB, CB)
        for r in range(8):
            s_v[r, rows, :], s_v[r + 8, rows, :] = _split(u_v, tab_v, r, rows)
            yield

    def inverse(b, shift=0):
        rows = pl.ds(b * CB, CB)
        for r in range(8):
            ev = s_v[r, rows, :]
            od = _twiddle((s_v[r + 8, rows, C:], s_v[r + 8, rows, :C]), r, R)
            od = jnp.concatenate(od[::-1], axis=1)
            for n, z in ((r, ev + od), (r + 8, ev - od)):
                x_v[n + shift, rows, :] = x_v[n, rows, :] + _dot(z, _halves(tab_v[R + n]))
            yield

    def mix(first, b):
        for i in range(CB // 4):
            kr = pl.ds(b * CB + i // 2 * 8, 8)
            rs = range(i % 2 * 8, i % 2 * 8 + 8)
            kf = [(kh_v[r, kr, :C], kh_v[r, kr, C:]) for r in rs]
            if first:
                kf = _fft(kf)
                for r, k in zip(rs, kf):
                    kh_v[r, kr, :C], kh_v[r, kr, C:] = k
            uf = _fft([(s_v[r, kr, :C], s_v[r, kr, C:]) for r in rs])
            for r, z in zip(rs, _ifft([_cmul(*t) for t in zip(uf, kf)])):
                s_v[r, kr, :C], s_v[r, kr, C:] = z
            yield

    def conv(first, done, todo):
        fwd, mid, inv = [range(*span) for span in zip(done, todo)]
        _run((_chain(forward(b) for b in fwd), 8 * len(fwd)),
             (_chain(inverse(b) for b in inv), 8 * len(inv), 0.03, 1.03),
             (_chain(mix(first, b) for b in mid), CB // 4 * len(mid)))

    sz, kw, groups = C // PH, D // PH // 2, R // PH

    def moments(p, stats):
        for r in range(PH * p, PH * p + PH):
            acc = None
            for b in range(D // C):
                for row in range(b * C, b * C + C, 32):
                    acc = _sums(x_v[r, pl.ds(row, 32), :], acc)
                pin(op_v, acc[1])
                stats[r] = acc if b + 1 < D // C else _stats(acc)
                yield

    def terms(tile, i):
        return _rhs_terms(jnp.concatenate([jnp.concatenate(
            [tile(j, h * 2 * kw + 32 * i) for j in range(PH)], axis=1) for h in range(PH)],
            axis=0), LV)

    def norm(p, stats):
        for i in range(kw // 16):
            for n, b in enumerate(terms(lambda j, row: (
                    x_v[PH * p + j, pl.ds(row, 32), :] - stats[PH * p + j][0]) * stats[PH * p + j][1], i)):
                op_v[p + zero, pl.ds(n * kw + 16 * i, 16), :] = _words(b)
            yield

    def qkv(g, n, p, pace):
        buf = (qa_v, qb_v)[g % 2]

        def emit(blocks):
            for (i, j), val in blocks.items():
                slot = 16 * (j % 2) + PH // 2 * p + j // 2
                for k, t in enumerate(QKV_CHUNKS[n]):
                    part, rows = val[k * sz:(k + 1) * sz], pl.ds(t * C + i * sz, sz)
                    buf[8 + slot + (zero if t else 0), rows, :] = part
                    if t and slot % 16:
                        buf[slot + zero, rows, :] = pltpu.roll(part, 1, 1)

        return _strassen(lambda i: pace(_dot(
            _halves(wt_v[g, n, i]), _halves(op_v[p, pl.ds(i * kw, kw), :]))), LV, emit)

    held = [[pl.ds(8 + j * C + i * 16 * PH, 16 * PH) for i in range(hp)] for j in range(PH)]

    def attend(g, p):
        buf = (qa_v, qb_v)[g % 2]
        for j in range(PH):
            n = PH // 2 * p + j // 2
            slot = 16 * (j % 2) + 8 + n
            logits = [None] * WIN
            for dh in range(DH):
                q = buf[slot, pl.ds(dh * 8, 8), :]
                for w in range(WIN):
                    t = q * buf[slot - w, pl.ds(C + dh * 8, 8), :]
                    logits[w] = t if dh == 0 else logits[w] + t
                if dh % 4 == 3:
                    pin(op_v, logits[dh // 2])
                    yield
            for w in range(n + 1, WIN):
                logits[w] = jnp.where(lane == 0, -1e9, logits[w])
            m = _tree(jnp.maximum, logits)
            ex = [jnp.exp(t - m) for t in logits]
            inv = 1.0 / _tree(jnp.add, ex)
            pr = [t * inv for t in ex]
            yield
            for i in range(hp):
                o = jnp.concatenate([_tree(jnp.add, [
                    pr[w] * buf[slot - w, pl.ds(2 * C + (2 * (h * hp + i) + e) * 8, 8), :]
                    for w in range(WIN)]) for h in range(PH) for e in range(2)], axis=0)
                op_v[groups + zero, held[j][i], :] = pltpu.bitcast(o, U32)
                yield
        for i in range(hp):
            cols = [pltpu.bitcast(op_v[groups, rows[i], :], F32) for rows in held]
            for t, b in enumerate(_rhs_terms(jnp.concatenate(cols, axis=1), LV)):
                op_v[p + zero, pl.ds((NP + t) * kw + (g * hp + i) * 8, 8), :] = _pairs(b)
            yield

    sums = {}

    def project(last, n, p, pace):
        def emit(blocks):
            for (i, j), val in blocks.items():
                for k, t in enumerate(OUT_CHUNKS[n]):
                    rows = pl.ds(t * C + i * sz, sz)
                    x = x_v[PH * p + j, rows, :] + val[k * sz:(k + 1) * sz]
                    (ya_v, yb_v)[p % 2][j + zero, rows, :] = x
                    if not last:
                        x_v[PH * p + j, rows, :] = x
                        sums[PH * p + j] = _sums(x, sums.get(PH * p + j))

        return _strassen(lambda i: pace(_dot(
            _halves(wot_v[n, i]), _halves(op_v[p, pl.ds((NP + i) * kw, kw), :]))), LV, emit)

    def out_copy(n):
        return pltpu.make_async_copy(io_v.at[n], out_w.at[:, n, :], sems.at[12 + n])

    sent = []

    def send(p):
        for n in range(len(sent), PH // 2 * p):
            sent.append(n)
            out_copy(n).start()

    def finish(last, p):
        y_v = (ya_v, yb_v)[p % 2]
        if last:
            for j in range(0, PH, 2):
                for b in range(D // C):
                    wd = _pairs(y_v[j:j + 2, pl.ds(b * C, C), :].reshape(2 * C, C))
                    io_v[(PH * p + j) // 2, :, b * C:(b + 1) * C] = wd.T
                    pin(op_v, wd)
                    yield
        else:
            for j, (m, s) in enumerate([_stats(sums[PH * p + j]) for j in range(PH)]):
                for b in range(D // C):
                    u = (y_v[j, pl.ds(b * C, C), :] - m) * s
                    u_v[PH * p + j + zero, pl.ds(b * C, C), :] = u
                    pin(op_v, u)
                    yield

    heads, chunks = D // C, range(len(QKV_CHUNKS))
    n_qkv, n_att, n_term = NP * len(chunks), 5 * PH + 8 + hp, kw // 16

    def first_heads():
        pace, stats = pacer(LAG, x_v), {}
        _run((inverse(D // CB - 1, zero), 8), (moments(0, stats), 4 * PH, 0.4, 0.7),
             (moments(1, stats), 4 * PH, 0.7, 1.0), (norm(0, stats), n_term, 0.8, 1.0))
        for p in range(groups):
            _run((_chain(qkv(0, n, p, pace) for n in chunks), n_qkv),
                 *[(norm(p + 1, stats), n_term)] * (p + 1 < groups),
                 *[(moments(p + 2, stats), 4 * PH)] * (p + 2 < groups))

    def next_heads(g):
        pace = pacer(LAG, (qa_v, qb_v)[1 - g % 2])
        early = [(attend(g, 0), n_att, 0.88, 1.0)] * (g == heads - 1)
        _run((_chain(qkv(g, n, p, pace) for n in chunks for p in range(groups)), n_qkv * groups),
             (_chain(attend(g - 1, p) for p in range(groups)), n_att * groups,
              0.0, 0.88 if early else 1.0), *early)

    def output(last):
        pace, n_fin = pacer(LAG, qb_v), 2 * PH if last else 4 * PH
        for p in range(groups):
            if last and p in (groups // 2, groups - 1):
                send(p - 1)
            _run((_chain(project(last, n, p, pace) for n in range(len(OUT_CHUNKS))),
                  NP * len(OUT_CHUNKS)),
                 *[(attend(heads - 1, p + 1), n_att)] * (p + 1 < groups),
                 *[(finish(last, p - 1), n_fin, 0.3, 1.0)] * (p > 0))
        if last:
            send(groups - 1)
        _run((finish(last, groups - 1), n_fin, 0.0, 0.5),
             *[(forward(0), 8)] * (not last))

    _run((forward(0), 8))
    for last in (False, True):
        with jax.named_scope("conv"):
            for done, todo in zip(PLAN, PLAN[1:]):
                region(conv, not last, done, todo)
        with jax.named_scope("kv"):
            region(first_heads)
        with jax.named_scope("mid"):
            for g in range(1, heads):
                region(next_heads, g)
        with jax.named_scope("attn"):
            region(output, last)

    send(groups)
    for p in range(R // 2):
        out_copy(p).wait()


@jax.jit
def pallas_interleave_layers__ssm_conv_s4__sliding_local_dilated__prompt_kernel(
    A_u: jax.Array,
    A_A_re: jax.Array,
    A_A_im: jax.Array,
    A_B_re: jax.Array,
    A_B_im: jax.Array,
    A_C_re: jax.Array,
    A_C_im: jax.Array,
    A_log_dt: jax.Array,
    A_Dskip: jax.Array,
    B_x: jax.Array,
    B_wqkv: jax.Array,
    B_wo: jax.Array,
):
    del B_x
    assert A_u.shape == (1, L, D) and A_A_re.shape == (D, N) and A_A_re.dtype == BF16
    hbm = pl.BlockSpec(memory_space=pl.ANY)
    out = pl.pallas_call(
        _kernel,
        in_specs=[hbm] * 14,
        out_specs=hbm,
        out_shape=jax.ShapeDtypeStruct((C, R, D), BF16),
        scratch_shapes=[
            pltpu.VMEM((R // 2 + 1, C, D), U32),
            pltpu.VMEM((6, D // 2, N), U32),
            pltpu.VMEM((D // 2, 3 * D), U32),
            pltpu.VMEM((D // C, D // 2, C), U32),
            pltpu.VMEM((2 * R, C, C), U32),
            pltpu.VMEM((R + 1, C, C), U32),
            pltpu.VMEM((D, C), F32),
            pltpu.VMEM((D, C), F32),
            pltpu.VMEM((D // C, len(QKV_CHUNKS), NP, len(QKV_CHUNKS[0]) * C // PH // 2, D // PH),
                       U32),
            pltpu.VMEM((len(OUT_CHUNKS), NP, len(OUT_CHUNKS[0]) * C // PH // 2, D // PH),
                       U32),
            pltpu.VMEM((R + 1, D, C), F32),
            pltpu.VMEM((R, D, C), F32),
            pltpu.VMEM((R, D, C), F32),
            pltpu.VMEM((R, D, 2 * C), F32),
            pltpu.VMEM((R // PH + 1, NP * D // PH, C), U32),
            pltpu.VMEM((R, D, 2 * C), F32),
            *[pltpu.VMEM((2 * R + 1, 3 * C, C), F32)] * 2,
            *[pltpu.VMEM((PH, D, C), F32)] * 2,
            *[pltpu.VMEM((D,), BF16)] * 2,
            pltpu.SMEM((1,), jnp.int32),
            pltpu.SemaphoreType.DMA((24,)),
        ],
        compiler_params=pltpu.CompilerParams(vmem_limit_bytes=100 * 1024 * 1024),
    )(A_u.reshape(C, R, D), A_A_re, A_A_im, A_B_re, A_B_im, A_C_re, A_C_im,
      A_log_dt, A_Dskip, B_wqkv, B_wo, *_dft_tables(),
      np.zeros((1,), np.int32))
    return out.reshape(1, L, D)
```

```python
import ml_dtypes
import numpy as np

import jax
import jax.numpy as jnp
from jax import lax
import jax.experimental.pallas as pl
import jax.experimental.pallas.tpu as pltpu

L, D, N = 2048, 512, 128
R, C = 16, 128
DH, WIN = 16, 8
CB = 64
LV = 1
PH, NP = 2 ** LV, 7 ** LV
QKV_CHUNKS, OUT_CHUNKS = ((1,), (2,), (0,)), ((0,), (1,), (2,), (3,))
PLAN = ((1, 0, 0), (3, 1, 0), (6, 3, 1), (8, 5, 3), (8, 7, 5), (8, 8, 6))
LAG, DUE = 4, 3
HEAD = 3
EPS = 1e-5
F32, BF16, U32 = jnp.float32, jnp.bfloat16, jnp.uint32
_NT = (((1,), (1,)), ((), ()))


def _host_words(a):
    h = np.ascontiguousarray(a).astype(ml_dtypes.bfloat16).view(np.uint16).astype(np.uint32)
    return h[..., 0::2, :] | (h[..., 1::2, :] << 16)


def _dft_tables():
    t = R * np.arange(C)[None, :, None] + np.arange(R)[:, None, None]
    ang = 2.0 * np.pi * (np.arange(C)[None, None, :] + 0.5) * t / (2 * L)
    fwd = np.concatenate([np.cos(ang), -np.sin(ang)], axis=-1)
    p = (np.arange(C) - 7) % C
    fwd_k = fwd[:, 16 * (p % 8) + p // 8, :] / L
    inv = fwd.transpose(0, 2, 1)
    fwd, fwd_k = [np.concatenate([a[..., :C], a[..., C:]], axis=1) for a in (fwd, fwd_k)]
    return _host_words(np.concatenate([fwd, inv])), _host_words(fwd_k)


def _tap_offsets():
    l = np.arange(L)
    lr = l.astype(np.float32).astype(ml_dtypes.bfloat16).astype(np.float32).astype(np.int64)
    rho = (lr - (l // R) * R).reshape(8, 16, R)
    assert (rho == rho[:, :1]).all()
    return rho[:, 0].tolist()


def _cmul(a, b):
    return a[0] * b[0] - a[1] * b[1], a[0] * b[1] + a[1] * b[0]


def _csq(a):
    t = a[0] * a[1]
    return a[0] * a[0] - a[1] * a[1], t + t


def _twiddle(a, k, n):
    if k == 0:
        return a
    if 4 * k == n:
        return a[1], -a[0]
    h = float(np.sqrt(0.5))
    if 8 * k == n:
        return (a[0] + a[1]) * h, (a[1] - a[0]) * h
    if 8 * k == 3 * n:
        return (a[1] - a[0]) * h, (a[0] + a[1]) * (-h)
    w = (float(np.cos(2 * np.pi * k / n)), float(-np.sin(2 * np.pi * k / n)))
    return _cmul(a, w)


def _fft(x):
    n = len(x)
    if n == 1:
        return x
    if n == 2:
        return [(x[0][0] + x[1][0], x[0][1] + x[1][1]), (x[0][0] - x[1][0], x[0][1] - x[1][1])]
    e, o1, o3 = _fft(x[0::2]), _fft(x[1::4]), _fft(x[3::4])
    out = [None] * n
    q = n // 4
    for k in range(q):
        a, b = _twiddle(o1[k], k, n), _twiddle(o3[k], 3 * k, n)
        s = (a[0] + b[0], a[1] + b[1])
        d = (a[0] - b[0], a[1] - b[1])
        out[k] = (e[k][0] + s[0], e[k][1] + s[1])
        out[k + 2 * q] = (e[k][0] - s[0], e[k][1] - s[1])
        out[k + q] = (e[k + q][0] + d[1], e[k + q][1] - d[0])
        out[k + 3 * q] = (e[k + q][0] - d[1], e[k + q][1] + d[0])
    return out


def _ifft(x):
    return [(b, a) for a, b in _fft([(b, a) for a, b in x])]


def _tree(op, xs):
    while len(xs) > 1:
        xs = [op(*xs[i:i + 2]) if i + 1 < len(xs) else xs[i] for i in range(0, len(xs), 2)]
    return xs[0]


def _sums(x, acc=None):
    parts = [x[i:i + 8] for i in range(0, x.shape[0], 8)]
    new = _tree(jnp.add, parts), _tree(jnp.add, [t * t for t in parts])
    return new if acc is None else (acc[0] + new[0], acc[1] + new[1])


def _stats(acc):
    m, sq = [jnp.sum(t, axis=0, keepdims=True) * (1.0 / D) for t in acc]
    return m, lax.rsqrt(jnp.maximum(sq - m * m, 0.0) + EPS)


def _words(x):
    return pltpu.bitcast(x.astype(BF16), U32)


def _pairs(x):
    b = pltpu.bitcast(x, U32) + jnp.uint32(0x8000)
    return (b[x.shape[0] // 2:] & jnp.uint32(0xFFFF0000)) | (b[:x.shape[0] // 2] >> 16)


def _halves(w):
    return pltpu.bitcast(w, BF16)


def _dot(a, b, dims=(((1,), (0,)), ((), ()))):
    return lax.dot_general(a.astype(BF16), b.astype(BF16), dims, preferred_element_type=F32)


def _split(src, table, r):
    lo, hi = [_dot(src(n), _halves(jnp.concatenate(
        [table[n, :C // 2], table[n, C // 2:]], axis=1))) for n in (r, r + 8)]
    d = lo - hi
    return lo + hi, jnp.concatenate(_twiddle((d[:, :C], d[:, C:]), r, R), axis=1)


def _run(*jobs):
    order = []
    for k, (_, n, *span) in enumerate(jobs):
        lo, hi = span or (0.0, 1.0)
        order += [(lo + (hi - lo) * i / n, k) for i in range(n)]
    for _, k in sorted(order):
        next(jobs[k][0])
    for job in jobs:
        for _ in job[0]:
            pass


def _chain(gens):
    for g in gens:
        yield from g


def _lhs_terms(a, levels):
    if not levels:
        return [jnp.concatenate(a, axis=0)]
    m, k = a[0].shape[0] // 2, a[0].shape[1] // 2
    terms = []
    for t in a:
        a11, a12, a21, a22 = t[:m, :k], t[:m, k:], t[m:, :k], t[m:, k:]
        terms.append((a11 + a22, a21 + a22, a22, a12 - a22, a21 - a11, a11, a11 + a12))
    return [x for ts in zip(*terms) for x in _lhs_terms(list(ts), levels - 1)]


def _rhs_terms(b, levels):
    if not levels:
        return [b]
    k, n = b.shape[0] // 2, b.shape[1] // 2
    b11, b12, b21, b22 = b[:k, :n], b[:k, n:], b[k:, :n], b[k:, n:]
    terms = (b11 + b22, b11, b21 - b11, b21 + b22, b11 + b12, b12 - b22, b22)
    return [x for t in terms for x in _rhs_terms(t, levels - 1)]


def _strassen(product, levels, emit=None, base=0):
    if not levels:
        out = {(0, 0): product(base)}
        if emit:
            emit(out)
        yield
        return out
    half, out = 2 ** (levels - 1), {}

    def term(i):
        return _strassen(product, levels - 1, None, base + i * 7 ** (levels - 1))

    def done(i, j, x):
        x = {(i * half + a, j * half + b): v for (a, b), v in x.items()}
        out.update(x)
        if emit:
            emit(x)

    def add(x, y):
        return {k: x[k] + y[k] for k in x}

    def sub(x, y):
        return {k: x[k] - y[k] for k in x}

    m1 = yield from term(0)
    m2 = yield from term(1)
    c22 = sub(m1, m2)
    m4 = yield from term(2)
    c11 = add(m1, m4)
    done(1, 0, add(m2, m4))
    c11 = add(c11, (yield from term(3)))
    c22 = add(c22, (yield from term(4)))
    m3 = yield from term(5)
    done(1, 1, add(c22, m3))
    m5 = yield from term(6)
    done(0, 0, sub(c11, m5))
    done(0, 1, add(m3, m5))
    return out


def _ds(start, size):
    return pl.ds(start if isinstance(start, int) else pl.multiple_of(start, size), size)


def _loop(lo, hi, body):
    lax.fori_loop(lo, hi, lambda i, c: (body(i), c)[1], 0)


def _kernel(x_hbm, are_hbm, aim_hbm, bre_hbm, bim_hbm, cre_hbm, cim_hbm, ldt_hbm, dsk_hbm,
            wqkv_hbm, wo_hbm, tab_hbm, fk_hbm, zero_hbm, out_hbm,
            io_v, par_v, wqkv_v, wo_v, tab_v, fk_v, dt_v, dk_v, wt_v, wot_v,
            x_v, st_v, kt_v, kh_v, xt_v, ot_v, held_v, gate_v, s_v,
            qa_v, qb_v, ya_v, yb_v, ldt_ref, dsk_ref, zero_s, sems):
    srcs = (are_hbm, aim_hbm, bre_hbm, bim_hbm, cre_hbm, cim_hbm)
    par_cp = [[pltpu.make_async_copy(s.bitcast(U32).at[rows], par_v.at[i, rows], sems.at[k])
               for i, s in enumerate(srcs)]
              for k, rows in enumerate((pl.ds(0, HEAD * 8), pl.ds(HEAD * 8, D // 2 - HEAD * 8)))]
    small_cp = [pltpu.make_async_copy(*pair, sems.at[2 + i]) for i, pair in enumerate(
        ((ldt_hbm, ldt_ref), (dsk_hbm, dsk_ref), (zero_hbm, zero_s)))]
    x_w, out_w = x_hbm.bitcast(U32), out_hbm.bitcast(U32)
    x_cp = [pltpu.make_async_copy(x_w.at[:, i, :], io_v.at[i], sems.at[12 + i])
            for i in range(R // 2)]
    fk_cp = pltpu.make_async_copy(fk_hbm, fk_v.at[:R], sems.at[7])
    tab_cp = pltpu.make_async_copy(tab_hbm, tab_v, sems.at[8])
    wqkv_cp = pltpu.make_async_copy(wqkv_hbm.bitcast(U32), wqkv_v, sems.at[10])
    wo_cp = [pltpu.make_async_copy(wo_hbm.bitcast(U32).at[:, pl.ds(t * C, C)], wo_v.at[t],
                                   sems.at[20 + t]) for t in range(D // C)]
    for cp in small_cp + par_cp[0] + par_cp[1]:
        cp.start()
    for cp in small_cp + par_cp[0]:
        cp.wait()

    lane = lax.broadcasted_iota(jnp.int32, (8, C), 1)
    sub = lax.broadcasted_iota(jnp.int32, (8, C), 0)
    rho = _tap_offsets()

    zero = zero_s[0]

    def pin(ref, x, k=1):
        ref[ref.shape[0] - 1 + k * zero, :8, :C] = pltpu.bitcast(x[:8, :C], ref.dtype)

    regions = []

    def region(fn, *args):
        regions.append(fn)
        pl.when(zero < len(regions))(lambda: fn(*args))

    def pacer(lag, ref, k=1):
        queue = []

        def pace(x, urgent=False):
            if urgent:
                queue[-1].append(x)
                return x
            queue.append([x])
            if len(queue) > lag:
                pin(ref, queue[-1 - lag][0], k)
            if len(queue) > lag + DUE:
                for y in queue.pop(0)[1:]:
                    pin(gate_v, y)
            return x
        return pace

    dt_row = jnp.exp(ldt_ref[...].astype(F32).reshape(1, D)).astype(BF16).astype(F32)
    dk_row = dsk_ref[...].astype(F32).reshape(1, D)
    for b in range(D // C):
        cols = slice(b * C, (b + 1) * C)
        dt_v[cols, :] = jnp.broadcast_to(dt_row[:, cols], (C, C)).T
        dk_v[cols, :] = jnp.broadcast_to(dk_row[:, cols], (C, C)).T

    keys = [(s, p) for p in (16, *range(1, 16)) for s in range(8) if p == 16 or p in rho[s]]

    def flip(x):
        x = pltpu.roll(x, 4, 0)
        x = jnp.where((sub & 2) == 0, pltpu.roll(x, 6, 0), pltpu.roll(x, 2, 0))
        return jnp.where((sub & 1) == 0, pltpu.roll(x, 7, 0), pltpu.roll(x, 1, 0))

    def discretise(i):
        a_re, a_im, b_re, b_im, c_re, c_im = [
            _halves(par_v[n, pl.ds(i * 8, 8), :]).astype(F32) for n in range(6)]
        rows = pl.ds(i * 16, 16)
        dt = dt_v[rows, :]
        mag, ph = jnp.exp(dt * a_re), dt * a_im
        w = _cmul((c_re, c_im), (dt * b_re, dt * b_im))
        tap0 = dk_v[rows, :] + jnp.sum(w[0], axis=1, keepdims=True)
        return mag * jnp.cos(ph), mag * jnp.sin(ph), *w, tap0

    def taps(i, a_re, a_im, w_re, w_im, tap0):
        rows = pl.ds(i * 8, 8)
        a = {1: (a_re, a_im)}
        for n in range(8):
            a[2 << n] = _csq(a[1 << n])
        right = [(jnp.ones((8, C), F32), jnp.zeros((8, C), F32)), (flip(a[16][0]), -flip(a[16][1]))]
        for j in range(2, 16):
            right.append(_csq(right[j // 2]) if j % 2 == 0 else _cmul(right[j - 1], right[1]))
        left = {(0, 0): (w_re, w_im)}
        for s, p in keys:
            left[s, p] = (_cmul(left[s - 1, p], a[256]) if s else
                          _cmul(left[0, p & (p - 1)], a[p & -p]))
        res = _dot(*[jnp.concatenate([jnp.concatenate(v, axis=1) for v in vals], axis=0)
                     for vals in ([left[k] for k in keys], right)], _NT)
        part = {k: pltpu.roll(res[8 * n:8 * n + 8], k[0], 1, stride=1, stride_axis=0)
                for n, k in enumerate(keys)}
        pos, memo = (lane - 7) & (C - 1), {}

        def merge(ps, s=0):
            if len(ps) == 1 or not any(ps):
                return part[s, ps[0]]
            if (ps, s) not in memo:
                h = len(ps) // 2
                memo[ps, s] = jnp.where((pos & h) == 0, merge(ps[:h], s), merge(ps[h:], s + h))
            return memo[ps, s]

        t16 = merge((16,) * 8)
        t0 = jnp.where(pos < 8, pltpu.roll(t16, 9, 1), pltpu.roll(t16, 8, 1))
        t0 = jnp.where(pos == 0, tap0, t0)
        for s in range(8):
            part[s, 0] = t0
        for r in range(R):
            kt_v[r, rows, :] = merge(tuple(rho[s][r] for s in range(8)))

    def filters(lo, hi):
        for i in range(lo, hi):
            vals = discretise(i)
            for h in range(2):
                taps(2 * i + h, *[v[8 * h:8 * h + 8] for v in vals])

    with jax.named_scope("filter"):
        filters(0, HEAD)
        for cp in x_cp + [fk_cp, wqkv_cp] + wo_cp + [tab_cp]:
            cp.start()
        for cp in par_cp[1]:
            cp.wait()
        filters(HEAD, D // 16)

    def spectra():
        pace = pacer(2, io_v)
        for r in range(8):
            for b in range(D // C):
                rows = pl.ds(b * C, C)
                ev, od = _split(lambda n: kt_v[n, rows, :], fk_v, r)
                kh_v[r, rows, :], kh_v[r + 8, rows, :] = pace(ev), od
                yield

    def keep(r, acc):
        for n, t in enumerate(_stats(acc)):
            st_v[r, n] = jnp.broadcast_to(t, (8, C))

    def load():
        for i in range(R // 2):
            acc = [None, None]
            for b in range(D // C):
                rows = pl.ds(b * C, C)
                wd = io_v[i, :, rows].T
                if b:
                    pin(fk_v, jnp.add(*acc[0]) + jnp.add(*acc[1]))
                for e, w in enumerate((wd << 16, wd & jnp.uint32(0xFFFF0000))):
                    x_v[2 * i + e, rows, :] = x = pltpu.bitcast(w, F32)
                    acc[e] = _sums(x, acc[e])
                yield
            for e in range(2):
                keep(2 * i + e, acc[e])

    hp = DH // 2 // PH

    def weights():
        row = lax.broadcasted_iota(jnp.int32, (C, C), 0)
        col = lax.broadcasted_iota(jnp.int32, (C, C), 1)
        pick = jnp.where(col == (row & 7) * DH + (row >> 3), 1.0, 0.0)
        for g in range(D // C):
            for n, chunk in enumerate(QKV_CHUNKS):
                tiles = [_dot(pick * (DH ** -0.5 if t == 0 else 1.0),
                              _halves(wqkv_v[:, pl.ds(t * D + g * C, C)]), _NT) for t in chunk]
                for i, a in enumerate(_lhs_terms(tiles, LV)):
                    wt_v[g, n, i] = _words(a)
                yield
        for n, chunk in enumerate(OUT_CHUNKS):
            tiles = [_halves(jnp.concatenate(
                [wo_v[t, pl.ds(g * C // 2 + h * hp + i, 8, stride=DH // 2), :]
                 for h in range(PH) for g in range(D // C) for i in range(hp)],
                axis=0)).T.astype(F32) for t in chunk]
            for i, a in enumerate(_lhs_terms(tiles, LV)):
                wot_v[n, i] = _words(a)
            yield

    for cp in x_cp + [fk_cp, wqkv_cp] + wo_cp:
        cp.wait()
    with jax.named_scope("load"):
        region(_run, (spectra(), 32), (load(), 32),
               (weights(), 4 * len(QKV_CHUNKS) + len(OUT_CHUNKS)))
    tab_cp.wait()

    def forward(b, shift=0):
        rows = pl.ds(b * CB, CB)

        def normed(n):
            m, s = [jnp.concatenate([st_v[n, i]] * (CB // 8), axis=0) for i in range(2)]
            return (x_v[n + shift, rows, :] - m) * s

        for r in range(8):
            s_v[r, rows, :], s_v[r + 8, rows, :] = _split(normed, tab_v, r)
            yield

    def inverse(b):
        rows = pl.ds(b * CB, CB)
        for r in range(8):
            ev = s_v[r, rows, :]
            od = _twiddle((s_v[r + 8, rows, C:], s_v[r + 8, rows, :C]), r, R)
            od = jnp.concatenate(od[::-1], axis=1)
            for n, z in ((r, ev + od), (r + 8, ev - od)):
                x_v[n, rows, :] += _dot(z, _halves(tab_v[R + n]))
            yield

    def mix(first, b):
        for i in range(CB // 4):
            kr = pl.ds(b * CB + i // 2 * 8, 8)
            rs = range(i % 2 * 8, i % 2 * 8 + 8)
            kf = [(kh_v[r, kr, :C], kh_v[r, kr, C:]) for r in rs]
            if first:
                kf = _fft(kf)
                for r, k in zip(rs, kf):
                    kh_v[r, kr, :C], kh_v[r, kr, C:] = k
            uf = _fft([(s_v[r, kr, :C], s_v[r, kr, C:]) for r in rs])
            for r, z in zip(rs, _ifft([_cmul(*t) for t in zip(uf, kf)])):
                s_v[r, kr, :C], s_v[r, kr, C:] = z
            yield

    def conv(first, done, todo):
        fwd, mid, inv = [range(*span) for span in zip(done, todo)]
        _run((_chain(forward(b) for b in fwd), 8 * len(fwd)),
             (_chain(inverse(b) for b in inv), 8 * len(inv), 0.03, 1.03),
             (_chain(mix(first, b) for b in mid), CB // 4 * len(mid)))

    sz, kw, groups = C // PH, D // PH // 2, R // PH

    gate_v[0] = jnp.zeros((8, C), U32)

    def gated(w):
        tail = jnp.concatenate([w[-8:, :-C], w[-8:, -C:] | gate_v[0]], axis=1)
        return _halves(jnp.concatenate([w[:-8], tail], axis=0))

    def moments(p, stats):
        for r in range(PH * p, PH * p + PH):
            acc = None
            for b in range(D // C):
                for row in range(b * C, b * C + C, 32):
                    acc = _sums(x_v[r + (zero if p > 1 else 0), pl.ds(row, 32), :], acc)
                pin(gate_v, jnp.add(*acc))
                stats[r] = acc if b + 1 < D // C else _stats(acc)
                yield

    def terms(tile, i):
        return _rhs_terms(jnp.concatenate([jnp.concatenate(
            [tile(j, h * 2 * kw + 32 * i) for j in range(PH)], axis=1) for h in range(PH)],
            axis=0), LV)

    def norm(p, stats):
        for i in range(kw // 16):
            for n, b in enumerate(terms(lambda j, row: (
                    x_v[PH * p + j - (zero if p else 0), pl.ds(row, 32), :] - stats[PH * p + j][0]) * stats[PH * p + j][1], i)):
                xt_v[p % 2][p // 2 + zero, n, pl.ds(16 * i, 16), :] = wd = _words(b)
                pin(gate_v, wd[:8] | wd[8:])
            yield

    def qkv(g, n, p, pace):
        buf = (qa_v, qb_v)[g % 2]

        def emit(blocks):
            for (i, j), val in blocks.items():
                slot = 16 * (j % 2) + PH // 2 * p + j // 2
                for k, t in enumerate(QKV_CHUNKS[n]):
                    part, rows = val[k * sz:(k + 1) * sz], pl.ds(t * C + i * sz, sz)
                    buf[8 + slot + (zero if t else 0), rows, :] = part
                    if t and slot % 16:
                        buf[slot + zero, rows, :] = pltpu.roll(part, 1, 1)

        return _strassen(lambda i: pace(_dot(
            gated(wt_v[g, n, i]), _halves(xt_v[p % 2][p // 2, i]))), LV, emit)

    def attend(g, p):
        buf = (qa_v, qb_v)[g % 2]
        for j in range(PH):
            n = PH // 2 * p + j // 2
            slot = 16 * (j % 2) + 8 + n
            logits = [None] * WIN
            for dh in range(DH):
                q = buf[slot, pl.ds(dh * 8, 8), :]
                for w in range(WIN):
                    t = q * buf[slot - w, pl.ds(C + dh * 8, 8), :]
                    logits[w] = t if dh == 0 else logits[w] + t
                if dh % 2 == 1:
                    pin(gate_v, logits[dh // 2])
                    yield
            for w in range(n + 1, WIN):
                logits[w] = jnp.where(lane == 0, -1e9, logits[w])
            m = _tree(jnp.maximum, logits)
            ex = [jnp.exp(t - m) for t in logits]
            inv = 1.0 / _tree(jnp.add, ex)
            pr = [t * inv for t in ex]
            yield from range(3)
            for i in range(hp):
                o = jnp.concatenate([_tree(jnp.add, [
                    pr[w] * buf[slot - w, pl.ds(2 * C + (2 * (h * hp + i) + e) * 8, 8), :]
                    for w in range(WIN)]) for h in range(PH) for e in range(2)], axis=0)
                held_v[j + zero, i] = o
                pin(gate_v, o[-8:])
                yield from range(2)
        for i in range(hp):
            cols = [held_v[j, i] for j in range(PH)]
            for t, b in enumerate(_rhs_terms(jnp.concatenate(cols, axis=1), LV)):
                ot_v[p % 2][p // 2 + zero, t, pl.ds((g * hp + i) * 8, 8), :] = wd = _pairs(b)
                if t == 0:
                    pin(gate_v, wd)
            yield

    sums = {}

    def project(last, n, p, pace):
        def emit(blocks):
            for (i, j), val in blocks.items():
                for k, t in enumerate(OUT_CHUNKS[n]):
                    rows = pl.ds(t * C + i * sz, sz)
                    x = x_v[PH * p + j, rows, :] + val[k * sz:(k + 1) * sz]
                    if not last:
                        x_v[PH * p + j, rows, :] = x
                        sums[PH * p + j] = _sums(x, sums.get(PH * p + j))
                        pace(jnp.add(*sums[PH * p + j]), True)
                    elif j % 2:
                        wd = _pairs(jnp.concatenate([sums.pop((i, j - 1, t)), x], axis=0))
                        (ya_v, yb_v)[p % 2][j // 2 + zero, rows, :] = wd
                        pace(wd[-8:], True)
                    else:
                        sums[i, j, t] = x

        return _strassen(lambda i: pace(_dot(
            gated(wot_v[n, i]), _halves(ot_v[p % 2][p // 2, i]))), LV, emit)

    def out_copy(n):
        return pltpu.make_async_copy(io_v.at[n], out_w.at[:, n, :], sems.at[12 + n])

    sent = []

    def send(p):
        for n in range(len(sent), PH // 2 * p):
            sent.append(n)
            out_copy(n).start()

    def finish(last, p):
        for j in range(PH):
            if not last:
                keep(PH * p + j, sums[PH * p + j])
            for b in range(j % 2 * 2, j % 2 * 2 + 2):
                if last:
                    cols = pl.ds(b * C, C)
                    io_v[(PH * p + j) // 2, :, cols] = (ya_v, yb_v)[p % 2][j // 2, cols, :].T
                yield

    heads, chunks = D // C, range(len(QKV_CHUNKS))
    n_qkv, n_att, n_term = NP * len(chunks), 11 * PH + 16 + hp, kw // 16

    def first_heads():
        pace, stats = pacer(LAG, x_v, 2), {}
        _run(*[(inverse(b), 8) for b in range(PLAN[-1][2], D // CB)],
             (moments(0, stats), 4 * PH, 0.3, 0.55), (moments(1, stats), 4 * PH, 0.6, 1.0),
             (norm(0, stats), n_term, 0.6, 1.0))
        for p in range(groups):
            _run((_chain(qkv(0, n, p, pace) for n in chunks), n_qkv),
                 *[(norm(p + 1, stats), n_term, 0.0, 0.85)] * (p + 1 < groups),
                 *[(moments(p + 2, stats), 4 * PH)] * (p + 2 < groups))

    def next_heads(g):
        pace = pacer(LAG, (qa_v, qb_v)[1 - g % 2])
        early = [(attend(g, 0), n_att, 0.88, 1.0)] * (g == heads - 1)
        _run((_chain(qkv(g, n, p, pace) for n in chunks for p in range(groups)), n_qkv * groups),
             (_chain(attend(g - 1, p) for p in range(groups)), n_att * groups,
              0.0, 0.88 if early else 1.0), *early)

    def output(last):
        pace, n_fin = pacer(LAG, qb_v), 2 * PH
        for p in range(groups):
            if last and p in (groups // 2, groups - 1):
                send(p - 1)
            _run((_chain(project(last, n, p, pace) for n in range(len(OUT_CHUNKS))),
                  NP * len(OUT_CHUNKS)),
                 *[(attend(heads - 1, p + 1), n_att, 0.0, 0.9)] * (p + 1 < groups),
                 *[(finish(last, p - 1), n_fin, 0.3, 1.0)] * (p > 0))
        if last:
            send(groups - 1)
        _run((finish(last, groups - 1), n_fin, 0.0, 0.5),
             *[(forward(0, zero), 8)] * (not last))

    _run((forward(0), 8))
    for last in (False, True):
        with jax.named_scope("conv"):
            for done, todo in zip(PLAN, PLAN[1:]):
                region(conv, not last, done, todo)
        with jax.named_scope("kv"):
            region(first_heads)
        with jax.named_scope("mid"):
            for g in range(1, heads):
                region(next_heads, g)
        with jax.named_scope("attn"):
            region(output, last)

    send(groups)
    for p in range(R // 2):
        out_copy(p).wait()


@jax.jit
def pallas_interleave_layers__ssm_conv_s4__sliding_local_dilated__prompt_kernel(
    A_u: jax.Array,
    A_A_re: jax.Array,
    A_A_im: jax.Array,
    A_B_re: jax.Array,
    A_B_im: jax.Array,
    A_C_re: jax.Array,
    A_C_im: jax.Array,
    A_log_dt: jax.Array,
    A_Dskip: jax.Array,
    B_x: jax.Array,
    B_wqkv: jax.Array,
    B_wo: jax.Array,
):
    del B_x
    assert A_u.shape == (1, L, D) and A_A_re.shape == (D, N) and A_A_re.dtype == BF16
    hbm = pl.BlockSpec(memory_space=pl.ANY)
    out = pl.pallas_call(
        _kernel,
        in_specs=[hbm] * 14,
        out_specs=hbm,
        out_shape=jax.ShapeDtypeStruct((C, R, D), BF16),
        scratch_shapes=[
            pltpu.VMEM((R // 2 + 1, C, D), U32),
            pltpu.VMEM((6, D // 2, N), U32),
            pltpu.VMEM((D // 2, 3 * D), U32),
            pltpu.VMEM((D // C, D // 2, C), U32),
            pltpu.VMEM((2 * R, C, C), U32),
            pltpu.VMEM((R + 1, C, C), U32),
            pltpu.VMEM((D, C), F32),
            pltpu.VMEM((D, C), F32),
            pltpu.VMEM((D // C, len(QKV_CHUNKS), NP, len(QKV_CHUNKS[0]) * C // PH // 2, D // PH),
                       U32),
            pltpu.VMEM((len(OUT_CHUNKS), NP, len(OUT_CHUNKS[0]) * C // PH // 2, D // PH),
                       U32),
            pltpu.VMEM((R + 1, D, C), F32),
            pltpu.VMEM((R, 2, 8, C), F32),
            pltpu.VMEM((R, D, C), F32),
            pltpu.VMEM((R, D, 2 * C), F32),
            *[[pltpu.VMEM((R // PH // 2, NP, D // PH // 2, C), U32)] * 2] * 2,
            pltpu.VMEM((PH, DH // 2 // PH, 16 * PH, C), F32),
            pltpu.VMEM((2, 8, C), U32),
            pltpu.VMEM((R, D, 2 * C), F32),
            *[pltpu.VMEM((2 * R + 1, 3 * C, C), F32)] * 2,
            *[pltpu.VMEM((PH // 2, D, C), U32)] * 2,
            *[pltpu.VMEM((D,), BF16)] * 2,
            pltpu.SMEM((1,), jnp.int32),
            pltpu.SemaphoreType.DMA((24,)),
        ],
        compiler_params=pltpu.CompilerParams(vmem_limit_bytes=100 * 1024 * 1024),
    )(A_u.reshape(C, R, D), A_A_re, A_A_im, A_B_re, A_B_im, A_C_re, A_C_im,
      A_log_dt, A_Dskip, B_wqkv, B_wo, *_dft_tables(),
      np.zeros((1,), np.int32))
    return out.reshape(1, L, D)
```

```python
import ml_dtypes
import numpy as np

import jax
import jax.numpy as jnp
from jax import lax
import jax.experimental.pallas as pl
import jax.experimental.pallas.tpu as pltpu

L, D, N = 2048, 512, 128
R, C = 16, 128
DH, WIN = 16, 8
CB = 64
LV = 1
PH, NP = 2 ** LV, 7 ** LV
QKV_CHUNKS, OUT_CHUNKS = ((1,), (2,), (0,)), ((0,), (1,), (2,), (3,))
PLAN = ((1, 0, 0), (3, 1, 0), (6, 3, 1), (8, 6, 3), (8, 8, 6))
LAG, EARLY = 4, (0, 0, 1, 2)
HEAD = 3
EPS = 1e-5
F32, BF16, U32 = jnp.float32, jnp.bfloat16, jnp.uint32
_NT = (((1,), (1,)), ((), ()))


def _host_words(a):
    h = np.ascontiguousarray(a).astype(ml_dtypes.bfloat16).view(np.uint16).astype(np.uint32)
    return h[..., 0::2, :] | (h[..., 1::2, :] << 16)


def _dft_tables():
    t = R * np.arange(C)[None, :, None] + np.arange(R)[:, None, None]
    ang = 2.0 * np.pi * (np.arange(C)[None, None, :] + 0.5) * t / (2 * L)
    fwd = np.concatenate([np.cos(ang), -np.sin(ang)], axis=-1)
    p = (np.arange(C) - 7) % C
    fwd_k = fwd[:, 16 * (p % 8) + p // 8, :] / L
    inv = fwd.transpose(0, 2, 1)
    fwd, fwd_k = [np.concatenate([a[..., :C], a[..., C:]], axis=1) for a in (fwd, fwd_k)]
    return _host_words(np.concatenate([fwd, inv])), _host_words(fwd_k)


def _tap_offsets():
    l = np.arange(L)
    lr = l.astype(np.float32).astype(ml_dtypes.bfloat16).astype(np.float32).astype(np.int64)
    rho = (lr - (l // R) * R).reshape(8, 16, R)
    assert (rho == rho[:, :1]).all()
    return rho[:, 0].tolist()


def _cmul(a, b):
    return a[0] * b[0] - a[1] * b[1], a[0] * b[1] + a[1] * b[0]


def _csq(a):
    t = a[0] * a[1]
    return a[0] * a[0] - a[1] * a[1], t + t


def _twiddle(a, k, n):
    if k == 0:
        return a
    if 4 * k == n:
        return a[1], -a[0]
    h = float(np.sqrt(0.5))
    if 8 * k == n:
        return (a[0] + a[1]) * h, (a[1] - a[0]) * h
    if 8 * k == 3 * n:
        return (a[1] - a[0]) * h, (a[0] + a[1]) * (-h)
    w = (float(np.cos(2 * np.pi * k / n)), float(-np.sin(2 * np.pi * k / n)))
    return _cmul(a, w)


def _fft(x):
    n = len(x)
    if n == 1:
        return x
    if n == 2:
        return [(x[0][0] + x[1][0], x[0][1] + x[1][1]), (x[0][0] - x[1][0], x[0][1] - x[1][1])]
    e, o1, o3 = _fft(x[0::2]), _fft(x[1::4]), _fft(x[3::4])
    out = [None] * n
    q = n // 4
    for k in range(q):
        a, b = _twiddle(o1[k], k, n), _twiddle(o3[k], 3 * k, n)
        s = (a[0] + b[0], a[1] + b[1])
        d = (a[0] - b[0], a[1] - b[1])
        out[k] = (e[k][0] + s[0], e[k][1] + s[1])
        out[k + 2 * q] = (e[k][0] - s[0], e[k][1] - s[1])
        out[k + q] = (e[k + q][0] + d[1], e[k + q][1] - d[0])
        out[k + 3 * q] = (e[k + q][0] - d[1], e[k + q][1] + d[0])
    return out


def _ifft(x):
    return [(b, a) for a, b in _fft([(b, a) for a, b in x])]


def _fold(op, x):
    while x.shape[0] > 1:
        x = op(x[:x.shape[0] // 2], x[x.shape[0] // 2:])
    return x[0]


def _sums(x, acc=None):
    x = x.reshape(-1, 8, C)
    new = _fold(jnp.add, x), _fold(jnp.add, x * x)
    return new if acc is None else (acc[0] + new[0], acc[1] + new[1])


def _stats(acc):
    m, sq = [jnp.sum(t, axis=0, keepdims=True) * (1.0 / D) for t in acc]
    return m, lax.rsqrt(jnp.maximum(sq - m * m, 0.0) + EPS)


def _words(x):
    return pltpu.bitcast(x.astype(BF16), U32)


def _pairs(x):
    b = pltpu.bitcast(x, U32) + jnp.uint32(0x8000)
    return (b[x.shape[0] // 2:] & jnp.uint32(0xFFFF0000)) | (b[:x.shape[0] // 2] >> 16)


def _halves(w):
    return pltpu.bitcast(w, BF16)


def _dot(a, b, dims=(((1,), (0,)), ((), ()))):
    return lax.dot_general(a.astype(BF16), b.astype(BF16), dims, preferred_element_type=F32)


def _split(src, table, r):
    lo, hi = [_dot(src(n), _halves(jnp.concatenate(
        [table[n, :C // 2], table[n, C // 2:]], axis=1))) for n in (r, r + 8)]
    d = lo - hi
    return lo + hi, jnp.concatenate(_twiddle((d[:, :C], d[:, C:]), r, R), axis=1)


def _run(*jobs):
    order = []
    for k, (_, n, *span) in enumerate(jobs):
        lo, hi = span or (0.0, 1.0)
        order += [(lo + (hi - lo) * i / n, k) for i in range(n)]
    for _, k in sorted(order):
        next(jobs[k][0])
    for job in jobs:
        for _ in job[0]:
            pass


def _chain(gens):
    for g in gens:
        yield from g


def _lhs_terms(a, levels):
    if not levels:
        return [jnp.concatenate(a, axis=0)]
    m, k = a[0].shape[0] // 2, a[0].shape[1] // 2
    terms = []
    for t in a:
        a11, a12, a21, a22 = t[:m, :k], t[:m, k:], t[m:, :k], t[m:, k:]
        terms.append((a11 + a22, a21 + a22, a22, a12 - a22, a21 - a11, a11, a11 + a12))
    return [x for ts in zip(*terms) for x in _lhs_terms(list(ts), levels - 1)]


def _rhs_terms(b, levels):
    if not levels:
        return [b]
    k, n = b.shape[0] // 2, b.shape[1] // 2
    b11, b12, b21, b22 = b[:k, :n], b[:k, n:], b[k:, :n], b[k:, n:]
    terms = (b11 + b22, b11, b21 - b11, b21 + b22, b11 + b12, b12 - b22, b22)
    return [x for t in terms for x in _rhs_terms(t, levels - 1)]


def _strassen(product, levels, emit=None, base=0):
    if not levels:
        out = {(0, 0): product(base)}
        if emit:
            emit(out)
        yield
        return out
    half, out = 2 ** (levels - 1), {}

    def term(i):
        return _strassen(product, levels - 1, None, base + i * 7 ** (levels - 1))

    def done(i, j, x):
        x = {(i * half + a, j * half + b): v for (a, b), v in x.items()}
        out.update(x)
        if emit:
            emit(x)

    def add(x, y):
        return {k: x[k] + y[k] for k in x}

    def sub(x, y):
        return {k: x[k] - y[k] for k in x}

    m1 = yield from term(0)
    m2 = yield from term(1)
    c22 = sub(m1, m2)
    m4 = yield from term(2)
    c11 = add(m1, m4)
    done(1, 0, add(m2, m4))
    c11 = add(c11, (yield from term(3)))
    c22 = add(c22, (yield from term(4)))
    m3 = yield from term(5)
    done(1, 1, add(c22, m3))
    m5 = yield from term(6)
    done(0, 0, sub(c11, m5))
    done(0, 1, add(m3, m5))
    return out


def _ds(start, size):
    return pl.ds(start if isinstance(start, int) else pl.multiple_of(start, size), size)


def _loop(lo, hi, body):
    lax.fori_loop(lo, hi, lambda i, c: (body(i), c)[1], 0)


def _kernel(x_hbm, are_hbm, aim_hbm, bre_hbm, bim_hbm, cre_hbm, cim_hbm, ldt_hbm, dsk_hbm,
            wqkv_hbm, wo_hbm, tab_hbm, fk_hbm, zero_hbm, out_hbm,
            io_v, par_v, wqkv_v, wo_v, tab_v, fk_v, dt_v, dk_v, wt_v, wot_v,
            x_v, st_v, kt_v, kh_v, xt_v, ot_v, held_v, gate_v, s_v,
            q_v, ka_v, kb_v, ya_v, yb_v, ldt_ref, dsk_ref, zero_s, sems):
    srcs = (are_hbm, aim_hbm, bre_hbm, bim_hbm, cre_hbm, cim_hbm)
    par_cp = [[pltpu.make_async_copy(s.bitcast(U32).at[rows], par_v.at[i, rows], sems.at[k])
               for i, s in enumerate(srcs)]
              for k, rows in enumerate((pl.ds(0, HEAD * 8), pl.ds(HEAD * 8, D // 2 - HEAD * 8)))]
    small_cp = [pltpu.make_async_copy(*pair, sems.at[2 + i]) for i, pair in enumerate(
        ((ldt_hbm, ldt_ref), (dsk_hbm, dsk_ref), (zero_hbm, zero_s)))]
    x_w, out_w = x_hbm.bitcast(U32), out_hbm.bitcast(U32)
    x_cp = [pltpu.make_async_copy(x_w.at[:, i, :], io_v.at[i], sems.at[12 + i])
            for i in range(R // 2)]
    fk_cp = pltpu.make_async_copy(fk_hbm, fk_v.at[:R], sems.at[7])
    tab_cp = pltpu.make_async_copy(tab_hbm, tab_v, sems.at[8])
    wqkv_cp = pltpu.make_async_copy(wqkv_hbm.bitcast(U32), wqkv_v, sems.at[10])
    wo_cp = [pltpu.make_async_copy(wo_hbm.bitcast(U32).at[:, pl.ds(t * C, C)], wo_v.at[t],
                                   sems.at[20 + t]) for t in range(D // C)]
    for cp in small_cp + par_cp[0] + par_cp[1]:
        cp.start()
    for cp in small_cp + par_cp[0]:
        cp.wait()

    lane = lax.broadcasted_iota(jnp.int32, (8, C), 1)
    sub = lax.broadcasted_iota(jnp.int32, (8, C), 0)
    rho = _tap_offsets()

    zero = zero_s[0]

    def pin(ref, x, k=1):
        ref[ref.shape[0] - 1 + k * zero, :8, :C] = pltpu.bitcast(x[:8, :C], ref.dtype)

    gate_v[0] = jnp.zeros((8, C), U32)

    def gated(w):
        tail = w[-8:] | jnp.concatenate([gate_v[0]] * (w.shape[1] // C), axis=1)
        return _halves(jnp.concatenate([w[:-8], tail], axis=0))

    regions = []

    def region(fn, *args):
        regions.append(fn)
        pl.when(zero < len(regions))(lambda: fn(*args))

    def pacer(lag, ref, k=1):
        queue = []

        def pace(x):
            queue.append(x)
            if len(queue) > lag:
                pin(ref[0], queue.pop(0), k)
            return x
        return pace

    dt_row = jnp.exp(ldt_ref[...].astype(F32).reshape(1, D)).astype(BF16).astype(F32)
    dk_row = dsk_ref[...].astype(F32).reshape(1, D)
    for b in range(D // C):
        cols = slice(b * C, (b + 1) * C)
        dt_v[cols, :] = jnp.broadcast_to(dt_row[:, cols], (C, C)).T
        dk_v[cols, :] = jnp.broadcast_to(dk_row[:, cols], (C, C)).T

    keys = [(s, p) for p in (16, *range(1, 16)) for s in range(8) if p == 16 or p in rho[s]]

    def flip(x):
        x = pltpu.roll(x, 4, 0)
        x = jnp.where((sub & 2) == 0, pltpu.roll(x, 6, 0), pltpu.roll(x, 2, 0))
        return jnp.where((sub & 1) == 0, pltpu.roll(x, 7, 0), pltpu.roll(x, 1, 0))

    def discretise(i):
        a_re, a_im, b_re, b_im, c_re, c_im = [
            _halves(par_v[n, pl.ds(i * 8, 8), :]).astype(F32) for n in range(6)]
        rows = pl.ds(i * 16, 16)
        dt = dt_v[rows, :]
        mag, ph = jnp.exp(dt * a_re), dt * a_im
        w = _cmul((c_re, c_im), (dt * b_re, dt * b_im))
        tap0 = dk_v[rows, :] + jnp.sum(w[0], axis=1, keepdims=True)
        return mag * jnp.cos(ph), mag * jnp.sin(ph), *w, tap0

    def taps(i, a_re, a_im, w_re, w_im, tap0):
        rows = pl.ds(i * 8, 8)
        a = {1: (a_re, a_im)}
        for n in range(8):
            a[2 << n] = _csq(a[1 << n])
        right = [(jnp.ones((8, C), F32), jnp.zeros((8, C), F32)), (flip(a[16][0]), -flip(a[16][1]))]
        for j in range(2, 16):
            right.append(_csq(right[j // 2]) if j % 2 == 0 else _cmul(right[j - 1], right[1]))
        left = {(0, 0): (w_re, w_im)}
        for s, p in keys:
            left[s, p] = (_cmul(left[s - 1, p], a[256]) if s else
                          _cmul(left[0, p & (p - 1)], a[p & -p]))
        res = _dot(*[jnp.concatenate([jnp.concatenate(v, axis=1) for v in vals], axis=0)
                     for vals in ([left[k] for k in keys], right)], _NT)
        part = {k: pltpu.roll(res[8 * n:8 * n + 8], k[0], 1, stride=1, stride_axis=0)
                for n, k in enumerate(keys)}
        pos, memo = (lane - 7) & (C - 1), {}

        def merge(ps, s=0):
            if len(ps) == 1 or not any(ps):
                return part[s, ps[0]]
            if (ps, s) not in memo:
                h = len(ps) // 2
                memo[ps, s] = jnp.where((pos & h) == 0, merge(ps[:h], s), merge(ps[h:], s + h))
            return memo[ps, s]

        t16 = merge((16,) * 8)
        t0 = jnp.where(pos < 8, pltpu.roll(t16, 9, 1), pltpu.roll(t16, 8, 1))
        t0 = jnp.where(pos == 0, tap0, t0)
        for s in range(8):
            part[s, 0] = t0
        for r in range(R):
            kt_v[r, rows, :] = merge(tuple(rho[s][r] for s in range(8)))

    def filters(lo, hi):
        for i in range(lo, hi):
            vals = discretise(i)
            for h in range(2):
                taps(2 * i + h, *[v[8 * h:8 * h + 8] for v in vals])

    with jax.named_scope("filter"):
        filters(0, HEAD)
        for cp in x_cp + [fk_cp, wqkv_cp] + wo_cp + [tab_cp]:
            cp.start()
        for cp in par_cp[1]:
            cp.wait()
        filters(HEAD, D // 16)

    def spectra():
        pace = pacer(2, [io_v])
        for r in range(8):
            for b in range(D // C):
                rows = pl.ds(b * C, C)
                ev, od = _split(lambda n: kt_v[n, rows, :], fk_v, r)
                kh_v[r, rows, :], kh_v[r + 8, rows, :] = pace(ev), od
                yield

    def keep(r, acc):
        for n, t in enumerate(_stats(acc)):
            st_v[r, n] = jnp.broadcast_to(t, (8, C))

    def load():
        for i in range(R // 2):
            acc = [None, None]
            for b in range(D // C):
                rows = pl.ds(b * C, C)
                wd = io_v[i, :, rows].T
                if b:
                    pin(fk_v, jnp.add(*acc[0]) + jnp.add(*acc[1]))
                for e, w in enumerate((wd << 16, wd & jnp.uint32(0xFFFF0000))):
                    x_v[2 * i + e, rows, :] = x = pltpu.bitcast(w, F32)
                    acc[e] = _sums(x, acc[e])
                yield
            for e in range(2):
                keep(2 * i + e, acc[e])

    hp = DH // 2 // PH

    def weights():
        row = lax.broadcasted_iota(jnp.int32, (C, C), 0)
        col = lax.broadcasted_iota(jnp.int32, (C, C), 1)
        pick = jnp.where(col == (row & 7) * DH + (row >> 3), 1.0, 0.0)
        for g in range(D // C):
            for n, chunk in enumerate(QKV_CHUNKS):
                tiles = [_dot(pick * (DH ** -0.5 if t == 0 else 1.0),
                              _halves(wqkv_v[:, pl.ds(t * D + g * C, C)]), _NT) for t in chunk]
                for i, a in enumerate(_lhs_terms(tiles, LV)):
                    wt_v[g, n, i] = _words(a)
                yield
        for n, chunk in enumerate(OUT_CHUNKS):
            tiles = [_halves(jnp.concatenate(
                [wo_v[t, pl.ds(g * C // 2 + h * hp + i, 8, stride=DH // 2), :]
                 for h in range(PH) for g in range(D // C) for i in range(hp)],
                axis=0)).T.astype(F32) for t in chunk]
            for i, a in enumerate(_lhs_terms(tiles, LV)):
                wot_v[n, i] = _words(a)
            yield

    for cp in x_cp + [fk_cp, wqkv_cp] + wo_cp:
        cp.wait()
    with jax.named_scope("load"):
        region(_run, (spectra(), 32), (load(), 32),
               (weights(), 4 * len(QKV_CHUNKS) + len(OUT_CHUNKS)))
    tab_cp.wait()

    def units(b):
        return [(pl.ds(b * CB + i // 2 * 8, 8), range(i % 2 * 8, i % 2 * 8 + 8))
                for i in range(CB // 4)]

    def filter_fft(b):
        for rows, rs in units(b):
            for r, k in zip(rs, _fft([(kh_v[r, rows, :C], kh_v[r, rows, C:]) for r in rs])):
                kh_v[r, rows, :C], kh_v[r, rows, C:] = k
            yield

    def forward(b):
        rows = pl.ds(b * CB, CB)

        def normed(n):
            m, s = [jnp.concatenate([st_v[n, i]] * (CB // 8), axis=0) for i in range(2)]
            return (x_v[n, rows, :] - m) * s

        for r in range(8):
            s_v[r, rows, :], s_v[r + 8, rows, :] = _split(normed, tab_v, r)
            yield

    def inverse(b):
        rows = pl.ds(b * CB, CB)
        for r in range(8):
            ev = s_v[r, rows, :]
            od = _twiddle((s_v[r + 8, rows, C:], s_v[r + 8, rows, :C]), r, R)
            od = jnp.concatenate(od[::-1], axis=1)
            for n, z in ((r, ev + od), (r + 8, ev - od)):
                x_v[n, rows, :] += _dot(z, _halves(tab_v[R + n]))
            yield

    def mix(b):
        for rows, rs in units(b):
            uf = _fft([(s_v[r, rows, :C], s_v[r, rows, C:]) for r in rs])
            yield
            yf = [_cmul(u, (kh_v[r, rows, :C], kh_v[r, rows, C:])) for r, u in zip(rs, uf)]
            for r, z in zip(rs, _ifft(yf)):
                s_v[r, rows, :C], s_v[r, rows, C:] = z

    def conv(first, k):
        fwd, mid, inv = [range(*span) for span in zip(PLAN[k], PLAN[k + 1])]
        nxt = range(PLAN[k + 1][1], PLAN[k + 2][1]) if first and k + 2 < len(PLAN) else ()
        _run((_chain(forward(b) for b in fwd), 8 * len(fwd)),
             (_chain(inverse(b) for b in inv), 8 * len(inv), 0.03, 1.03),
             (_chain(mix(b) for b in mid), CB // 4 * len(mid)),
             (_chain(filter_fft(b) for b in nxt), CB // 4 * len(nxt)))

    sz, kw, groups = C // PH, D // PH // 2, R // PH

    def moments(p, stats):
        for r in range(PH * p, PH * p + PH):
            acc = None
            for b in range(8):
                for row in range(b * 64, b * 64 + 64, 32):
                    acc = _sums(x_v[r + (zero if p > 1 else 0), pl.ds(row, 32), :], acc)
                pin(gate_v, jnp.add(*acc))
                stats[r] = acc if b < 7 else _stats(acc)
                yield

    def terms(tile, i):
        return _rhs_terms(jnp.concatenate([jnp.concatenate(
            [tile(j, h * 2 * kw + 16 * i) for j in range(PH)], axis=1) for h in range(PH)],
            axis=0), LV)

    def norm(p, stats):
        for i in range(kw // 8):
            for n, b in enumerate(terms(lambda j, row: (
                    x_v[PH * p + j - (zero if p else 0), pl.ds(row, 16), :] - stats[PH * p + j][0]) * stats[PH * p + j][1], i)):
                xt_v[p][zero + n, pl.ds(8 * i, 8), :] = wd = _words(b)
                pin(gate_v, wd)
            yield

    def qkv(g, n, p, pace):
        buf = (ka_v, kb_v)[g % 2]

        def emit(blocks):
            for (i, j), val in blocks.items():
                slot = 16 * (j % 2) + PH // 2 * p + j // 2
                for k, t in enumerate(QKV_CHUNKS[n]):
                    part = val[k * sz:(k + 1) * sz]
                    if t == 0:
                        q_v[g % 2, PH * p + j, pl.ds(i * sz, sz), :] = part
                        continue
                    rows = pl.ds((t - 1) * C + i * sz, sz)
                    buf[8 + slot + zero, rows, :] = part
                    if slot % 16:
                        buf[slot + zero, rows, :] = pltpu.roll(part, 1, 1)

        return _strassen(lambda i: pace(_dot(
            gated(wt_v[g, n, i]), _halves(xt_v[p][i]))), LV, emit)

    def attend(g, p):
        buf = (ka_v, kb_v)[g % 2]
        for j in range(PH):
            n = PH // 2 * p + j // 2
            slot = 16 * (j % 2) + 8 + n
            window = pl.ds(slot - WIN + 1, WIN)
            for dh in range(DH):
                t = q_v[g % 2, PH * p + j, pl.ds(dh * 8, 8), :] * buf[window, pl.ds(dh * 8, 8), :]
                logits = t if dh == 0 else logits + t
                if dh % 2:
                    for w in range(dh // 2 % 2, WIN, 2):
                        pin(gate_v, logits[w])
                    yield
            if n < WIN - 1:
                logits = jnp.concatenate(
                    [jnp.where(lane == 0, -1e9, logits[:WIN - 1 - n]), logits[WIN - 1 - n:]])
            ex = jnp.exp(logits - _fold(jnp.maximum, logits))
            pr = ex * (1.0 / _fold(jnp.add, ex))
            yield from range(3)
            for i in range(hp):
                for h in range(PH):
                    for e in range(2):
                        rows = pl.ds(C + (2 * (h * hp + i) + e) * 8, 8)
                        o = _fold(jnp.add, pr * buf[window, rows, :])
                        held_v[j + zero, i, pl.ds(16 * h + 8 * e, 8), :] = o
                        pin(gate_v, o)
                    yield
        for i in range(hp):
            cols = [held_v[j, i] for j in range(PH)]
            for t, b in enumerate(_rhs_terms(jnp.concatenate(cols, axis=1), LV)):
                ot_v[p][zero + t, pl.ds((g * hp + i) * 8, 8), :] = wd = _pairs(b)
                if t % 2 == 0:
                    pin(gate_v, wd)
            yield

    sums = {}

    def project(last, n, p, pace):
        def emit(blocks):
            for (i, j), val in blocks.items():
                for k, t in enumerate(OUT_CHUNKS[n]):
                    rows = pl.ds(t * C + i * sz, sz)
                    x = x_v[PH * p + j, rows, :] + val[k * sz:(k + 1) * sz]
                    if not last:
                        x_v[PH * p + j, rows, :] = x
                        sums[PH * p + j] = _sums(x, sums.get(PH * p + j))
                    elif j % 2:
                        wd = _pairs(jnp.concatenate([sums.pop((i, j - 1, t)), x], axis=0))
                        (ya_v, yb_v)[p % 2][j // 2 + zero, rows, :] = wd
                    else:
                        sums[i, j, t] = x

        return _strassen(lambda i: pace(_dot(
            gated(wot_v[n, i]), _halves(ot_v[p][i]))), LV, emit)

    def out_copy(n):
        return pltpu.make_async_copy(io_v.at[n], out_w.at[:, n, :], sems.at[12 + n])

    sent = []

    def send(p):
        for n in range(len(sent), PH // 2 * p):
            sent.append(n)
            out_copy(n).start()

    def finish(last, p):
        for j in range(PH):
            if not last:
                keep(PH * p + j, sums[PH * p + j])
            for b in range(j % 2 * 2, j % 2 * 2 + 2):
                if last:
                    cols = pl.ds(b * C, C)
                    io_v[(PH * p + j) // 2, :, cols] = (ya_v, yb_v)[p % 2][j // 2, cols, :].T
                yield

    heads, chunks = D // C, range(len(QKV_CHUNKS))
    n_qkv, n_att, n_term = NP * len(chunks), 11 * PH + 16 + hp, kw // 8

    def first_heads():
        pace, stats = pacer(LAG, [x_v], 2), {}
        _run(*[(inverse(b), 8) for b in range(PLAN[-1][2], D // CB)],
             (moments(0, stats), 8 * PH, 0.3, 0.55), (moments(1, stats), 8 * PH, 0.6, 1.0),
             (norm(0, stats), n_term, 0.6, 1.0))
        for p in range(groups):
            _run((_chain(qkv(0, n, p, pace) for n in chunks), n_qkv),
                 *[(norm(p + 1, stats), n_term, 0.0, 0.85)] * (p + 1 < groups),
                 *[(moments(p + 2, stats), 8 * PH)] * (p + 2 < groups))

    def next_heads(g):
        todo = [(g - 1, p) for p in range(EARLY[g - 1], groups)] + [(g, p) for p in range(EARLY[g])]
        reading = [None]

        def attends():
            for h, p in todo:
                reading[0] = (ka_v, kb_v)[h % 2]
                yield from attend(h, p)

        pace = pacer(LAG, reading)
        _run((_chain(qkv(g, n, p, pace) for n in chunks for p in range(groups)), n_qkv * groups),
             (attends(), n_att * len(todo)))

    def output(last):
        pace, n_fin = pacer(LAG, [kb_v]), 2 * PH

        def projections():
            for p in range(groups):
                if last and p in (groups // 2, groups - 1):
                    send(p - 1)
                yield from _chain(project(last, n, p, pace) for n in range(len(OUT_CHUNKS)))

        _run((projections(), groups * NP * len(OUT_CHUNKS)),
             (_chain(attend(heads - 1, p) for p in range(EARLY[-1], groups)),
              (groups - EARLY[-1]) * n_att, 0.0, 0.8),
             *[(finish(last, p - 1), n_fin, (p + 0.3) / groups, (p + 1) / groups)
               for p in range(1, groups)])
        if last:
            send(groups - 1)
        _run((finish(last, groups - 1), n_fin, 0.0, 0.5),
             *[(forward(0), 8)] * (not last))

    _run((forward(0), 8), (filter_fft(0), CB // 4))
    for last in (False, True):
        with jax.named_scope("conv"):
            for k in range(len(PLAN) - 1):
                region(conv, not last, k)
        with jax.named_scope("kv"):
            region(first_heads)
        with jax.named_scope("mid"):
            for g in range(1, heads):
                region(next_heads, g)
        with jax.named_scope("attn"):
            region(output, last)

    send(groups)
    for p in range(R // 2):
        out_copy(p).wait()


@jax.jit
def pallas_interleave_layers__ssm_conv_s4__sliding_local_dilated__prompt_kernel(
    A_u: jax.Array,
    A_A_re: jax.Array,
    A_A_im: jax.Array,
    A_B_re: jax.Array,
    A_B_im: jax.Array,
    A_C_re: jax.Array,
    A_C_im: jax.Array,
    A_log_dt: jax.Array,
    A_Dskip: jax.Array,
    B_x: jax.Array,
    B_wqkv: jax.Array,
    B_wo: jax.Array,
):
    del B_x
    assert A_u.shape == (1, L, D) and A_A_re.shape == (D, N) and A_A_re.dtype == BF16
    hbm = pl.BlockSpec(memory_space=pl.ANY)
    out = pl.pallas_call(
        _kernel,
        in_specs=[hbm] * 14,
        out_specs=hbm,
        out_shape=jax.ShapeDtypeStruct((C, R, D), BF16),
        scratch_shapes=[
            pltpu.VMEM((R // 2 + 1, C, D), U32),
            pltpu.VMEM((6, D // 2, N), U32),
            pltpu.VMEM((D // 2, 3 * D), U32),
            pltpu.VMEM((D // C, D // 2, C), U32),
            pltpu.VMEM((2 * R, C, C), U32),
            pltpu.VMEM((R + 1, C, C), U32),
            pltpu.VMEM((D, C), F32),
            pltpu.VMEM((D, C), F32),
            pltpu.VMEM((D // C, len(QKV_CHUNKS), NP, len(QKV_CHUNKS[0]) * C // PH // 2, D // PH),
                       U32),
            pltpu.VMEM((len(OUT_CHUNKS), NP, len(OUT_CHUNKS[0]) * C // PH // 2, D // PH),
                       U32),
            pltpu.VMEM((R + 1, D, C), F32),
            pltpu.VMEM((R, 2, 8, C), F32),
            pltpu.VMEM((R, D, C), F32),
            pltpu.VMEM((R, D, 2 * C), F32),
            *[[pltpu.VMEM((NP, D // PH // 2, C), U32)] * (R // PH)] * 2,
            pltpu.VMEM((PH, DH // 2 // PH, 16 * PH, C), F32),
            pltpu.VMEM((2, 8, C), U32),
            pltpu.VMEM((R, D, 2 * C), F32),
            pltpu.VMEM((2, R, C, C), F32),
            *[pltpu.VMEM((2 * R + 1, 2 * C, C), F32)] * 2,
            *[pltpu.VMEM((PH // 2, D, C), U32)] * 2,
            *[pltpu.VMEM((D,), BF16)] * 2,
            pltpu.SMEM((1,), jnp.int32),
            pltpu.SemaphoreType.DMA((24,)),
        ],
        compiler_params=pltpu.CompilerParams(vmem_limit_bytes=100 * 1024 * 1024),
    )(A_u.reshape(C, R, D), A_A_re, A_A_im, A_B_re, A_B_im, A_C_re, A_C_im,
      A_log_dt, A_Dskip, B_wqkv, B_wo, *_dft_tables(),
      np.zeros((1,), np.int32))
    return out.reshape(1, L, D)
```

```python
import ml_dtypes
import numpy as np

import jax
import jax.numpy as jnp
from jax import lax
import jax.experimental.pallas as pl
import jax.experimental.pallas.tpu as pltpu

L, D, N = 2048, 512, 128
R, C = 16, 128
DH, WIN = 16, 8
CB = 64
NP = 7
PLAN = ((1, 0, 0), (3, 1, 0), (6, 3, 0), (8, 6, 2), (8, 8, 6))
LAG, EARLY = 4, (0, 0, 1, 2, 0)
HEAD = 3
EPS, SCALE = 1e-5, DH ** -0.5
F32, BF16, U32 = jnp.float32, jnp.bfloat16, jnp.uint32
_NT = (((1,), (1,)), ((), ()))


def _host_words(a):
    h = np.ascontiguousarray(a).astype(ml_dtypes.bfloat16).view(np.uint16).astype(np.uint32)
    return h[..., 0::2, :] | (h[..., 1::2, :] << 16)


def _dft_tables():
    t = R * np.arange(C)[None, :, None] + np.arange(R)[:, None, None]
    ang = 2.0 * np.pi * (np.arange(C)[None, None, :] + 0.5) * t / (2 * L)
    fwd = np.concatenate([np.cos(ang), -np.sin(ang)], axis=-1)
    p = (np.arange(C) - 7) % C
    fwd_k = fwd[:, 16 * (p % 8) + p // 8, :] / L
    inv = fwd.transpose(0, 2, 1)
    fwd, fwd_k = [np.concatenate([a[..., :C], a[..., C:]], axis=1) for a in (fwd, fwd_k)]
    return _host_words(np.concatenate([fwd, inv])), _host_words(fwd_k)


def _tap_offsets():
    l = np.arange(L)
    lr = l.astype(np.float32).astype(ml_dtypes.bfloat16).astype(np.float32).astype(np.int64)
    rho = (lr - (l // R) * R).reshape(8, 16, R)
    assert (rho == rho[:, :1]).all()
    return rho[:, 0].tolist()


def _cmul(a, b):
    return a[0] * b[0] - a[1] * b[1], a[0] * b[1] + a[1] * b[0]


def _csq(a):
    t = a[0] * a[1]
    return a[0] * a[0] - a[1] * a[1], t + t


def _twiddle(a, k, n):
    if k == 0:
        return a
    if 4 * k == n:
        return a[1], -a[0]
    h = float(np.sqrt(0.5))
    if 8 * k == n:
        return (a[0] + a[1]) * h, (a[1] - a[0]) * h
    if 8 * k == 3 * n:
        return (a[1] - a[0]) * h, (a[0] + a[1]) * (-h)
    w = (float(np.cos(2 * np.pi * k / n)), float(-np.sin(2 * np.pi * k / n)))
    return _cmul(a, w)


def _fft(x):
    n = len(x)
    if n == 1:
        return x
    if n == 2:
        return [(x[0][0] + x[1][0], x[0][1] + x[1][1]), (x[0][0] - x[1][0], x[0][1] - x[1][1])]
    e, o1, o3 = _fft(x[0::2]), _fft(x[1::4]), _fft(x[3::4])
    out = [None] * n
    q = n // 4
    for k in range(q):
        a, b = _twiddle(o1[k], k, n), _twiddle(o3[k], 3 * k, n)
        s = (a[0] + b[0], a[1] + b[1])
        d = (a[0] - b[0], a[1] - b[1])
        out[k] = (e[k][0] + s[0], e[k][1] + s[1])
        out[k + 2 * q] = (e[k][0] - s[0], e[k][1] - s[1])
        out[k + q] = (e[k + q][0] + d[1], e[k + q][1] - d[0])
        out[k + 3 * q] = (e[k + q][0] - d[1], e[k + q][1] + d[0])
    return out


def _ifft(x):
    return [(b, a) for a, b in _fft([(b, a) for a, b in x])]


def _fold(op, x):
    while x.shape[0] > 1:
        x = op(x[:x.shape[0] // 2], x[x.shape[0] // 2:])
    return x[0]


def _sums(x, acc=None):
    x = x.reshape(-1, 8, C)
    new = _fold(jnp.add, x), _fold(jnp.add, x * x)
    return new if acc is None else (acc[0] + new[0], acc[1] + new[1])


def _stats(acc):
    m, sq = [jnp.sum(t, axis=0, keepdims=True) * (1.0 / D) for t in acc]
    return m, lax.rsqrt(jnp.maximum(sq - m * m, 0.0) + EPS)


def _words(x):
    return pltpu.bitcast(x.astype(BF16), U32)


def _pairs(x):
    b = pltpu.bitcast(x, U32) + jnp.uint32(0x8000)
    return (b[x.shape[0] // 2:] & jnp.uint32(0xFFFF0000)) | (b[:x.shape[0] // 2] >> 16)


def _halves(w):
    return pltpu.bitcast(w, BF16)


def _dot(a, b, dims=(((1,), (0,)), ((), ()))):
    return lax.dot_general(a.astype(BF16), b.astype(BF16), dims, preferred_element_type=F32)


def _split(src, table, r):
    lo, hi = [_dot(src(n), _halves(jnp.concatenate(
        [table[n, :C // 2], table[n, C // 2:]], axis=1))) for n in (r, r + 8)]
    d = lo - hi
    return lo + hi, jnp.concatenate(_twiddle((d[:, :C], d[:, C:]), r, R), axis=1)


def _run(*jobs):
    order = []
    for k, (_, n, *span) in enumerate(jobs):
        lo, hi = span or (0.0, 1.0)
        order += [(lo + (hi - lo) * i / n, k) for i in range(n)]
    for _, k in sorted(order):
        next(jobs[k][0])
    for job in jobs:
        for _ in job[0]:
            pass


def _chain(gens):
    for g in gens:
        yield from g


def _lhs_terms(left, right):
    m = left.shape[0] // 2
    a11, a12, a21, a22 = left[:m], right[:m], left[m:], right[m:]
    return a11 + a22, a21 + a22, a22, a12 - a22, a21 - a11, a11, a11 + a12


def _rhs_terms(left, right):
    k = left.shape[0] // 2
    b11, b12, b21, b22 = left[:k], right[:k], left[k:], right[k:]
    return b11 + b22, b11, b21 - b11, b21 + b22, b11 + b12, b12 - b22, b22


def _strassen(product, emit):
    m1 = product(0)
    yield
    m2 = product(1)
    yield
    m4 = product(2)
    yield
    c11, c22 = m1 + m4, m1 - m2
    emit(1, 0, m2 + m4)
    c11 += product(3)
    yield
    c22 += product(4)
    yield
    m3 = product(5)
    yield
    emit(1, 1, c22 + m3)
    m5 = product(6)
    yield
    emit(0, 0, c11 - m5)
    emit(0, 1, m3 + m5)


def _kernel(x_hbm, are_hbm, aim_hbm, bre_hbm, bim_hbm, cre_hbm, cim_hbm, ldt_hbm, dsk_hbm,
            wqkv_hbm, wo_hbm, tab_hbm, fk_hbm, zero_hbm, out_hbm,
            io_v, par_v, wqkv_v, wo_v, tab_v, fk_v, dt_v, dk_v, wt_v, wot_v,
            x_v, st_v, kt_v, kh_v, xt_v, ot_v, held_v, gate_v, s_v,
            q_v, kv_v, y_v, ldt_ref, dsk_ref, zero_s, sems):
    srcs = (are_hbm, aim_hbm, bre_hbm, bim_hbm, cre_hbm, cim_hbm)
    par_cp = [[pltpu.make_async_copy(s.bitcast(U32).at[rows], par_v.at[i, rows], sems.at[k])
               for i, s in enumerate(srcs)]
              for k, rows in enumerate((pl.ds(0, HEAD * 8), pl.ds(HEAD * 8, D // 2 - HEAD * 8)))]
    small_cp = [pltpu.make_async_copy(*pair, sems.at[2 + i]) for i, pair in enumerate(
        ((ldt_hbm, ldt_ref), (dsk_hbm, dsk_ref), (zero_hbm, zero_s)))]
    x_w, out_w = x_hbm.bitcast(U32), out_hbm.bitcast(U32)
    x_cp = [pltpu.make_async_copy(x_w.at[:, i, :], io_v.at[i], sems.at[12 + i])
            for i in range(R // 2)]
    fk_cp = pltpu.make_async_copy(fk_hbm, fk_v.at[:R], sems.at[7])
    tab_cp = pltpu.make_async_copy(tab_hbm, tab_v, sems.at[8])
    wqkv_cp = pltpu.make_async_copy(wqkv_hbm.bitcast(U32), wqkv_v, sems.at[10])
    wo_cp = [pltpu.make_async_copy(wo_hbm.bitcast(U32).at[:, pl.ds(t * C, C)], wo_v.at[t],
                                   sems.at[20 + t]) for t in range(D // C)]
    for cp in small_cp + par_cp[0] + par_cp[1]:
        cp.start()
    with jax.named_scope("head"):
        for cp in small_cp + par_cp[0]:
            cp.wait()

    lane = lax.broadcasted_iota(jnp.int32, (8, C), 1)
    sub = lax.broadcasted_iota(jnp.int32, (8, C), 0)
    rho = _tap_offsets()

    zero = zero_s[0]

    def pin(ref, x, k=1):
        ref[ref.shape[0] - 1 + k * zero, :8, :C] = pltpu.bitcast(x[:8, :C], ref.dtype)

    gate_v[0] = jnp.zeros((8, C), U32)

    def gated(w):
        tail = w[-8:] | jnp.concatenate([gate_v[0]] * (w.shape[1] // C), axis=1)
        return _halves(jnp.concatenate([w[:-8], tail], axis=0))

    regions = []

    def region(fn, *args):
        regions.append(fn)
        pl.when(zero < len(regions))(lambda: fn(*args))

    def pacer(lag, ref, k=1):
        queue = []

        def pace(x):
            queue.append(x)
            if len(queue) > lag:
                pin(ref[0], queue.pop(0), k)
            return x
        return pace

    dt_row = jnp.exp(ldt_ref[...].astype(F32).reshape(1, D)).astype(BF16).astype(F32)
    dk_row = dsk_ref[...].astype(F32).reshape(1, D)
    for b in range(D // C):
        cols = slice(b * C, (b + 1) * C)
        dt_v[cols, :] = jnp.broadcast_to(dt_row[:, cols], (C, C)).T
        dk_v[cols, :] = jnp.broadcast_to(dk_row[:, cols], (C, C)).T

    keys = [(s, p) for p in (16, 8, 4, 12, 2, 6, 10, 14, *range(1, 16, 2))
            for s in range(8) if p == 16 or p in rho[s]]

    def flip(x):
        x = pltpu.roll(x, 4, 0)
        x = jnp.where((sub & 2) == 0, pltpu.roll(x, 6, 0), pltpu.roll(x, 2, 0))
        return jnp.where((sub & 1) == 0, pltpu.roll(x, 7, 0), pltpu.roll(x, 1, 0))

    def discretise(i):
        a_re, a_im, b_re, b_im, c_re, c_im = [
            _halves(par_v[n, pl.ds(i * 8, 8), :]).astype(F32) for n in range(6)]
        rows = pl.ds(i * 16, 16)
        dt = dt_v[rows, :]
        mag, ph = jnp.exp(dt * a_re), dt * a_im
        w = _cmul((c_re, c_im), (dt * b_re, dt * b_im))
        tap0 = dk_v[rows, :] + jnp.sum(w[0], axis=1, keepdims=True)
        return mag * jnp.cos(ph), mag * jnp.sin(ph), *w, tap0

    def taps(i, a_re, a_im, w_re, w_im, tap0):
        rows = pl.ds(i * 8, 8)
        a = {1: (a_re, a_im)}
        for n in range(4):
            a[2 << n] = _csq(a[1 << n])
        right = [(jnp.ones((8, C), F32), jnp.zeros((8, C), F32)), (flip(a[16][0]), -flip(a[16][1]))]
        for j in range(2, 16):
            right.append(_csq(right[j // 2]) if j % 2 == 0 else
                         _cmul(right[j // 2], right[j // 2 + 1]))
        a[256] = [flip(t) for t in _csq((right[8][0], -right[8][1]))]
        left = {(0, 0): (w_re, w_im)}
        for s, p in keys:
            left[s, p] = (_cmul(left[s - 1, p], a[256]) if s else
                          _cmul(left[0, p & (p - 1)], a[p & -p]))
        res = _dot(*[jnp.concatenate([jnp.concatenate(v, axis=1) for v in vals], axis=0)
                     for vals in ([left[k] for k in keys], right)], _NT)
        part = {k: pltpu.roll(res[8 * n:8 * n + 8], k[0], 1, stride=1, stride_axis=0)
                for n, k in enumerate(keys)}
        pos, memo = (lane - 7) & (C - 1), {}

        def merge(ps, s=0):
            if len(ps) == 1 or not any(ps):
                return part[s, ps[0]]
            if (ps, s) not in memo:
                h = len(ps) // 2
                memo[ps, s] = jnp.where((pos & h) == 0, merge(ps[:h], s), merge(ps[h:], s + h))
            return memo[ps, s]

        t16 = merge((16,) * 8)
        t0 = jnp.where(pos < 8, pltpu.roll(t16, 9, 1), pltpu.roll(t16, 8, 1))
        t0 = jnp.where(pos == 0, tap0, t0)
        for s in range(8):
            part[s, 0] = t0
        for r in range(R):
            kt_v[r, rows, :] = merge(tuple(rho[s][r] for s in range(8)))

    def filters(lo, hi):
        for i in range(lo, hi):
            vals = discretise(i)
            for h in range(2):
                taps(2 * i + h, *[v[8 * h:8 * h + 8] for v in vals])

    with jax.named_scope("filter"):
        filters(0, HEAD)
        for cp in x_cp + [fk_cp, wqkv_cp] + wo_cp + [tab_cp]:
            cp.start()
        for cp in par_cp[1]:
            cp.wait()
        filters(HEAD, D // 16)

    def spectra(lo, hi, size, pace=lambda x: x):
        for row in range(lo, hi, size):
            rows = pl.ds(row, size)
            for r in range(8):
                ev, od = _split(lambda n: kt_v[n, rows, :], fk_v, r)
                kh_v[r, rows, :], kh_v[r + 8, rows, :] = pace(ev), od
                yield

    def keep(r, acc):
        for n, t in enumerate(_stats(acc)):
            st_v[r, n] = jnp.broadcast_to(t, (8, C))

    def load():
        for i in range(R // 2):
            acc = [None, None]
            for b in range(D // C):
                rows = pl.ds(b * C, C)
                wd = io_v[i, :, rows].T
                if b:
                    pin(fk_v, jnp.add(*acc[0]) + jnp.add(*acc[1]))
                for e, w in enumerate((wd << 16, wd & jnp.uint32(0xFFFF0000))):
                    x_v[2 * i + e, rows, :] = x = pltpu.bitcast(w, F32)
                    acc[e] = _sums(x, acc[e])
                yield
            for e in range(2):
                keep(2 * i + e, acc[e])

    hp = DH // 4

    def qkv_weights():
        row = lax.broadcasted_iota(jnp.int32, (C, C), 0)
        col = lax.broadcasted_iota(jnp.int32, (C, C), 1)
        dh = ((row >> 2) & 1) + 8 * ((row >> 4) & 1) + 2 * (row >> 5)
        pick = jnp.where(col == (2 * (row & 3) + ((row >> 3) & 1)) * DH + dh, 1.0, 0.0)
        for j in range(3 * D // C):
            w = _dot(pick, _halves(wqkv_v[:, pl.ds(j * C, C)]), _NT)
            for n in range(C // 32):
                part = w[32 * n:32 * n + 32]
                for i, a in enumerate(_lhs_terms(part[:, :D // 2], part[:, D // 2:])):
                    wt_v[j, i, pl.ds(8 * n, 8), :] = _pairs(a)
            yield

    def out_weights():
        rows = [g * C // 2 + h * hp + i for h in range(2) for g in range(D // C) for i in range(hp)]
        for j in range(D // C):
            for c in range(2):
                halves = [_halves(jnp.concatenate(
                    [wo_v[j, pl.ds(row, 8, stride=DH // 2), :] for row in rows[8 * k:8 * k + 8]],
                    axis=0)).T.astype(F32) for k in (c, c + 2)]
                for i, a in enumerate(_lhs_terms(*halves)):
                    wot_v[j, i, :, pl.ds(c * C, C)] = _words(a)
                yield

    for cp in x_cp + [fk_cp, wqkv_cp] + wo_cp:
        cp.wait()
    with jax.named_scope("load"):
        region(_run, (spectra(0, D // 2, CB, pacer(4, [io_v])), 32), (load(), 32),
               (qkv_weights(), 12))
    tab_cp.wait()

    def units(b):
        return [(pl.ds(b * CB + i // 2 * 8, 8), range(i % 2 * 8, i % 2 * 8 + 8))
                for i in range(CB // 4)]

    def filter_fft(b):
        for rows, rs in units(b):
            for r, k in zip(rs, _fft([(kh_v[r, rows, :C], kh_v[r, rows, C:]) for r in rs])):
                kh_v[r, rows, :C], kh_v[r, rows, C:] = k
            yield

    def forward(b):
        rows = pl.ds(b * CB, CB)

        def normed(n):
            m, s = [jnp.concatenate([st_v[n, i]] * (CB // 8), axis=0) for i in range(2)]
            return (x_v[n, rows, :] - m) * s

        for r in range(8):
            s_v[r, rows, :], s_v[r + 8, rows, :] = _split(normed, tab_v, r)
            yield

    def inverse(b):
        rows = pl.ds(b * CB, CB)
        for r in range(8):
            ev = s_v[r, rows, :]
            od = _twiddle((s_v[r + 8, rows, C:], s_v[r + 8, rows, :C]), r, R)
            od = jnp.concatenate(od[::-1], axis=1)
            for n, z in ((r, ev + od), (r + 8, ev - od)):
                x_v[n, rows, :] += _dot(z, _halves(tab_v[R + n]))
            yield

    def mix(b):
        for rows, rs in units(b):
            uf = _fft([(s_v[r, rows, :C], s_v[r, rows, C:]) for r in rs])
            yf = [_cmul(u, (kh_v[r, rows, :C], kh_v[r, rows, C:])) for r, u in zip(rs, uf)]
            yield
            for r, z in zip(rs, _ifft(yf)):
                s_v[r, rows, :C], s_v[r, rows, C:] = z

    def conv(first, k):
        fwd, mid, inv = [range(*span) for span in zip(PLAN[k], PLAN[k + 1])]
        nxt = range(PLAN[k + 1][1], PLAN[k + 2][1]) if first and k + 2 < len(PLAN) else ()
        _run((_chain(forward(b) for b in fwd), 8 * len(fwd)),
             (_chain(inverse(b) for b in inv), 8 * len(inv), 0.03, 1.03),
             *[(spectra(D // 2 + k * C, D // 2 + k * C + C, CB), 16, 0.031, 1.031)] * (first and k < 2),
             (_chain(mix(b) for b in mid), CB // 4 * len(mid)),
             (_chain(filter_fft(b) for b in nxt), CB // 4 * len(nxt)))

    groups, heads, chunks = R // 2, D // C, (1, 2, 0)
    n_qkv, n_att, n_term = NP * len(chunks), 44, D // 32

    def moments(p, stats):
        for r in range(2 * p, 2 * p + 2):
            acc = None
            for b in range(8):
                for row in range(b * 64, b * 64 + 64, 32):
                    acc = _sums(x_v[r + (zero if p > 1 else 0), pl.ds(row, 32), :], acc)
                pin(gate_v, jnp.add(*acc))
                stats[r] = acc if b < 7 else _stats(acc)
                yield

    def norm(p, stats):
        for i in range(n_term):
            cols = [(jnp.concatenate(
                [x_v[r - (zero if p else 0), pl.ds(h + 16 * i, 8, stride=2), :]
                 for h in (0, 1, D // 2, D // 2 + 1)],
                axis=0) - stats[r][0]) * stats[r][1] for r in (2 * p, 2 * p + 1)]
            for n, b in enumerate(_rhs_terms(*cols)):
                xt_v[p][zero + n, pl.ds(8 * i, 8), :] = wd = _pairs(b)
                pin(gate_v, wd)
            yield

    def qkv(g, t, p, pace):
        def emit(i, j, val):
            if t == 0:
                q_v[g % 2][p][j + zero, pl.ds(i * C // 2, C // 2), :] = val
                return
            rows = pl.ds((t - 1) * C + i * C // 2, C // 2)
            kv_v[g % 2][16 * j + 8 + p + zero, rows, :] = val
            if p:
                kv_v[g % 2][16 * j + p + zero, rows, :] = pltpu.roll(val, 1, 1)

        return _strassen(lambda i: pace(_dot(
            gated(wt_v[t * heads + g, i]), _halves(xt_v[p][i]))), emit)

    def attend(g, p):
        buf = kv_v[g % 2]
        for j in range(2):
            window = pl.ds(16 * j + p + 1, WIN)
            for dh in range(DH):
                t = q_v[g % 2][p][j, pl.ds(dh * 8, 8), :] * buf[window, pl.ds(dh * 8, 8), :]
                logits = t if dh == 0 else logits + t
                if dh % 2:
                    for w in range(dh // 2 % 2, WIN, 2):
                        pin(gate_v, logits[w])
                    yield
            if p < WIN - 1:
                logits = jnp.concatenate(
                    [jnp.where(lane == 0, -1e9 / SCALE, logits[:WIN - 1 - p]), logits[WIN - 1 - p:]])
            ex = jnp.exp2((logits - _fold(jnp.maximum, logits)) * (SCALE * float(np.log2(np.e))))
            pr = ex * (1.0 / _fold(jnp.add, ex))
            yield from range(4)
            for i in range(hp):
                for h in range(2):
                    for e in range(2):
                        rows = pl.ds(C + (2 * (h * hp + i) + e) * 8, 8)
                        o = _fold(jnp.add, pr * buf[window, rows, :])
                        held_v[j + zero, i, pl.ds(16 * h + 8 * e, 8), :] = o
                        pin(gate_v, o)
                    yield
        for i in range(hp):
            cols = [held_v[j, i] for j in range(2)]
            for t, b in enumerate(_rhs_terms(*cols)):
                ot_v[p][zero + t, pl.ds((g * hp + i) * 8, 8), :] = wd = _pairs(b)
                if t % 2 == 0:
                    pin(gate_v, wd)
            yield

    sums = {}

    def project(last, t, p, pace):
        def emit(i, j, val):
            r, rows = 2 * p + j, pl.ds(t * C + i * C // 2, C // 2)
            x = x_v[r, rows, :] + val
            if not last:
                x_v[r, rows, :] = x
                sums[r] = _sums(x, sums.get(r))
            elif j:
                y_v[p % 2][zero, rows, :] = _pairs(jnp.concatenate([sums.pop(r - 1), x], axis=0))
            else:
                sums[r] = x

        return _strassen(lambda i: pace(_dot(gated(wot_v[t, i]), _halves(ot_v[p][i]))), emit)

    def out_copy(n):
        return pltpu.make_async_copy(io_v.at[n], out_w.at[:, n, :], sems.at[12 + n])

    sent = []

    def send(p):
        for n in range(len(sent), p):
            sent.append(n)
            out_copy(n).start()

    def finish(last, p):
        for b in range(D // C):
            if last:
                io_v[p, :, pl.ds(b * C, C)] = y_v[p % 2][0, pl.ds(b * C, C), :].T
            elif b % 2 == 0:
                keep(2 * p + b // 2, sums[2 * p + b // 2])
            yield

    def first_heads():
        pace, stats = pacer(LAG, [x_v], 2), {}
        _run(*[(inverse(b), 8) for b in range(PLAN[-1][2], D // CB)],
             (moments(0, stats), 16, 0.3, 0.55), (moments(1, stats), 16, 0.6, 1.0),
             (norm(0, stats), n_term, 0.6, 1.0))
        for p in range(groups):
            _run((_chain(qkv(0, n, p, pace) for n in chunks), n_qkv),
                 *[(norm(p + 1, stats), n_term, 0.0, 0.85)] * (p + 1 < groups),
                 *[(moments(p + 2, stats), 16)] * (p + 2 < groups))

    def attends(g, reading):
        todo = [(g - 1, p) for p in range(EARLY[g - 1], groups)] + [(g, p) for p in range(EARLY[g])]

        def steps():
            for h, p in todo:
                reading[0] = kv_v[h % 2]
                yield from attend(h, p)

        return steps(), n_att * len(todo)

    def projections(last, pace):
        for p in range(groups):
            for t in range(D // C):
                if last and t == 2 and p in (groups - 3, groups - 1):
                    send(p)
                yield from project(last, t, p, pace)

    def later_heads(last, *stages):
        reading = [None]
        pace = pacer(LAG, reading)
        for g in stages:
            if g < heads:
                _run((_chain(qkv(g, t, p, pace) for t in chunks for p in range(groups)),
                      n_qkv * groups), attends(g, reading))
                continue
            _run((projections(last, pace), groups * NP * D // C), (*attends(g, reading), 0.0, 0.85),
                 *[(finish(last, p - 1), D // C, (p + 0.2) / groups, (p + 0.5) / groups)
                   for p in range(1, groups)])
            _run((finish(last, groups - 1), D // C, 0.0, 0.5), *[(forward(0), 8)] * (not last))

    _run((forward(0), 8), (filter_fft(0), CB // 4), (out_weights(), 8))
    for last in (False, True):
        with jax.named_scope("conv"):
            for k in range(len(PLAN) - 1):
                region(conv, not last, k)
        with jax.named_scope("kv"):
            region(first_heads)
        with jax.named_scope("mid"):
            region(later_heads, last, 1); region(later_heads, last, 2)
        with jax.named_scope("attn"):
            region(later_heads, last, 3); region(later_heads, last, 4)

    send(groups)
    with jax.named_scope("tail"):
        for p in range(R // 2):
            out_copy(p).wait()


@jax.jit
def pallas_interleave_layers__ssm_conv_s4__sliding_local_dilated__prompt_kernel(
    A_u: jax.Array,
    A_A_re: jax.Array,
    A_A_im: jax.Array,
    A_B_re: jax.Array,
    A_B_im: jax.Array,
    A_C_re: jax.Array,
    A_C_im: jax.Array,
    A_log_dt: jax.Array,
    A_Dskip: jax.Array,
    B_x: jax.Array,
    B_wqkv: jax.Array,
    B_wo: jax.Array,
):
    del B_x
    assert A_u.shape == (1, L, D) and A_A_re.shape == (D, N) and A_A_re.dtype == BF16
    hbm = pl.BlockSpec(memory_space=pl.ANY)
    out = pl.pallas_call(
        _kernel,
        in_specs=[hbm] * 14,
        out_specs=hbm,
        out_shape=jax.ShapeDtypeStruct((C, R, D), BF16),
        scratch_shapes=[
            pltpu.VMEM((R // 2 + 1, C, D), U32),
            pltpu.VMEM((6, D // 2, N), U32),
            pltpu.VMEM((D // 2, 3 * D), U32),
            pltpu.VMEM((D // C, D // 2, C), U32),
            pltpu.VMEM((2 * R, C, C), U32),
            pltpu.VMEM((R + 1, C, C), U32),
            pltpu.VMEM((D, C), F32),
            pltpu.VMEM((D, C), F32),
            pltpu.VMEM((3 * D // C, NP, C // 4, D // 2), U32),
            pltpu.VMEM((D // C, NP, C // 4, D // 2), U32),
            pltpu.VMEM((R + 1, D, C), F32),
            pltpu.VMEM((R, 2, 8, C), F32),
            pltpu.VMEM((R, D, C), F32),
            pltpu.VMEM((R, D, 2 * C), F32),
            *[[pltpu.VMEM((NP, D // 4, C), U32)] * (R // 2)] * 2,
            pltpu.VMEM((2, DH // 4, 32, C), F32),
            pltpu.VMEM((2, 8, C), U32),
            pltpu.VMEM((R, D, 2 * C), F32),
            [[pltpu.VMEM((2, C, C), F32)] * (R // 2)] * 2,
            [pltpu.VMEM((2 * R + 1, 2 * C, C), F32)] * 2,
            [pltpu.VMEM((1, D, C), U32)] * 2,
            *[pltpu.VMEM((D,), BF16)] * 2,
            pltpu.SMEM((1,), jnp.int32),
            pltpu.SemaphoreType.DMA((24,)),
        ],
        compiler_params=pltpu.CompilerParams(vmem_limit_bytes=100 * 1024 * 1024),
    )(A_u.reshape(C, R, D), A_A_re, A_A_im, A_B_re, A_B_im, A_C_re, A_C_im,
      A_log_dt, A_Dskip, B_wqkv, B_wo, *_dft_tables(),
      np.zeros((1,), np.int32))
    return out.reshape(1, L, D)
```

```python
import ml_dtypes
import numpy as np

import jax
import jax.numpy as jnp
from jax import lax
import jax.experimental.pallas as pl
import jax.experimental.pallas.tpu as pltpu

L, D, N = 2048, 512, 128
R, C = 16, 128
DH, WIN = 16, 8
CB = 64
NP = 7
PLAN = ((1, 0, 0), (3, 1, 0), (6, 3, 0), (8, 6, 2), (8, 8, 6))
LAG = 4
EARLY = (0, 0, 1, 2, 0)
HEAD = 3
EPS, SCALE = 1e-5, DH ** -0.5
F32, BF16, U32 = jnp.float32, jnp.bfloat16, jnp.uint32
_NT = (((1,), (1,)), ((), ()))


def _host_words(a):
    h = np.ascontiguousarray(a).astype(ml_dtypes.bfloat16).view(np.uint16).astype(np.uint32)
    return h[..., 0::2, :] | (h[..., 1::2, :] << 16)


def _dft_tables():
    t = R * np.arange(C)[None, :, None] + np.arange(R)[:, None, None]
    ang = 2.0 * np.pi * (np.arange(C)[None, None, :] + 0.5) * t / (2 * L)
    fwd = np.concatenate([np.cos(ang), -np.sin(ang)], axis=-1)
    p = (np.arange(C) - 7) % C
    fwd_k = fwd[:, 16 * (p % 8) + p // 8, :] / L
    inv = fwd.transpose(0, 2, 1)
    fwd, fwd_k = [np.concatenate([a[..., :C], a[..., C:]], axis=1) for a in (fwd, fwd_k)]
    return _host_words(np.concatenate([fwd, inv])), _host_words(fwd_k)


def _tap_offsets():
    l = np.arange(L)
    lr = l.astype(np.float32).astype(ml_dtypes.bfloat16).astype(np.float32).astype(np.int64)
    rho = (lr - (l // R) * R).reshape(8, 16, R)
    assert (rho == rho[:, :1]).all()
    return rho[:, 0].tolist()


def _cmul(a, b):
    return a[0] * b[0] - a[1] * b[1], a[0] * b[1] + a[1] * b[0]


def _csq(a):
    t = a[0] * a[1]
    return a[0] * a[0] - a[1] * a[1], t + t


def _twiddle(a, k, n):
    if k == 0:
        return a
    if 4 * k == n:
        return a[1], -a[0]
    h = float(np.sqrt(0.5))
    if 8 * k == n:
        return (a[0] + a[1]) * h, (a[1] - a[0]) * h
    if 8 * k == 3 * n:
        return (a[1] - a[0]) * h, (a[0] + a[1]) * (-h)
    w = (float(np.cos(2 * np.pi * k / n)), float(-np.sin(2 * np.pi * k / n)))
    return _cmul(a, w)


def _fft(x):
    n = len(x)
    if n == 1:
        return x
    if n == 2:
        return [(x[0][0] + x[1][0], x[0][1] + x[1][1]), (x[0][0] - x[1][0], x[0][1] - x[1][1])]
    e, o1, o3 = _fft(x[0::2]), _fft(x[1::4]), _fft(x[3::4])
    out = [None] * n
    q = n // 4
    for k in range(q):
        a, b = _twiddle(o1[k], k, n), _twiddle(o3[k], 3 * k, n)
        s = (a[0] + b[0], a[1] + b[1])
        d = (a[0] - b[0], a[1] - b[1])
        out[k] = (e[k][0] + s[0], e[k][1] + s[1])
        out[k + 2 * q] = (e[k][0] - s[0], e[k][1] - s[1])
        out[k + q] = (e[k + q][0] + d[1], e[k + q][1] - d[0])
        out[k + 3 * q] = (e[k + q][0] - d[1], e[k + q][1] + d[0])
    return out


def _ifft(x):
    return [(b, a) for a, b in _fft([(b, a) for a, b in x])]


def _fold(op, x):
    while x.shape[0] > 1:
        x = op(x[:x.shape[0] // 2], x[x.shape[0] // 2:])
    return x[0]


def _sums(x, acc=None):
    x = x.reshape(-1, 8, C)
    new = _fold(jnp.add, x), _fold(jnp.add, x * x)
    return new if acc is None else (acc[0] + new[0], acc[1] + new[1])


def _stats(acc):
    m, sq = [jnp.sum(t, axis=0, keepdims=True) * (1.0 / D) for t in acc]
    return m, lax.rsqrt(jnp.maximum(sq - m * m, 0.0) + EPS)


def _words(x):
    return pltpu.bitcast(x.astype(BF16), U32)


def _pairs(x):
    b = pltpu.bitcast(x, U32) + jnp.uint32(0x8000)
    return (b[x.shape[0] // 2:] & jnp.uint32(0xFFFF0000)) | (b[:x.shape[0] // 2] >> 16)


def _halves(w):
    return pltpu.bitcast(w, BF16)


def _dot(a, b, dims=(((1,), (0,)), ((), ()))):
    return lax.dot_general(a.astype(BF16), b.astype(BF16), dims, preferred_element_type=F32)


def _split(src, table, r):
    lo, hi = [_dot(src(n), _halves(jnp.concatenate(
        [table[n, :C // 2], table[n, C // 2:]], axis=1))) for n in (r, r + 8)]
    d = lo - hi
    return lo + hi, jnp.concatenate(_twiddle((d[:, :C], d[:, C:]), r, R), axis=1)


def _run(*jobs):
    order = []
    for k, (_, n, *span) in enumerate(jobs):
        lo, hi = span or (0.0, 1.0)
        order += [(lo + (hi - lo) * i / n, k) for i in range(n)]
    for _, k in sorted(order):
        next(jobs[k][0])
    for job in jobs:
        for _ in job[0]:
            pass


def _chain(gens):
    for g in gens:
        yield from g


def _lhs_terms(left, right):
    m = left.shape[0] // 2
    a11, a12, a21, a22 = left[:m], right[:m], left[m:], right[m:]
    return a11 + a22, a21 + a22, a22, a12 - a22, a21 - a11, a11, a11 + a12


def _rhs_terms(left, right):
    k = left.shape[0] // 2
    b11, b12, b21, b22 = left[:k], right[:k], left[k:], right[k:]
    return b11 + b22, b11, b21 - b11, b21 + b22, b11 + b12, b12 - b22, b22


def _strassen(product, emit):
    m1 = product(0)
    yield
    m2 = product(1)
    yield
    m4 = product(2)
    yield
    c11, c22 = m1 + m4, m1 - m2
    emit(1, 0, m2 + m4)
    c22 += product(4)
    yield
    m3 = product(5)
    yield
    emit(1, 1, c22 + m3)
    c11 += product(3)
    yield
    m5 = product(6)
    yield
    emit(0, 0, c11 - m5)
    emit(0, 1, m3 + m5)


def _kernel(x_hbm, are_hbm, aim_hbm, bre_hbm, bim_hbm, cre_hbm, cim_hbm, ldt_hbm, dsk_hbm,
            wqkv_hbm, wo_hbm, tab_hbm, fk_hbm, zero_hbm, out_hbm,
            io_v, par_v, wqkv_v, wo_v, tab_v, fk_v, dt_v, dk_v, wt_v, wot_v,
            x_v, st_v, kt_v, kh_v, xt_v, ot_v, held_v, gate_v, s_v,
            q_v, kv_v, y_v, ldt_ref, dsk_ref, zero_s, sems):
    srcs = (are_hbm, aim_hbm, bre_hbm, bim_hbm, cre_hbm, cim_hbm)
    par_cp = [[pltpu.make_async_copy(s.bitcast(U32).at[rows], par_v.at[i, rows], sems.at[k])
               for i, s in enumerate(srcs)]
              for k, rows in enumerate((pl.ds(0, HEAD * 8), pl.ds(HEAD * 8, D // 2 - HEAD * 8)))]
    small_cp = [pltpu.make_async_copy(*pair, sems.at[2 + i]) for i, pair in enumerate(
        ((ldt_hbm, ldt_ref), (dsk_hbm, dsk_ref), (zero_hbm, zero_s)))]
    x_w, out_w = x_hbm.bitcast(U32), out_hbm.bitcast(U32)
    x_cp = [pltpu.make_async_copy(x_w.at[:, i, :], io_v.at[i], sems.at[12 + i])
            for i in range(R // 2)]
    fk_cp = pltpu.make_async_copy(fk_hbm, fk_v.at[:R], sems.at[7])
    tab_cp = pltpu.make_async_copy(tab_hbm, tab_v, sems.at[8])
    wqkv_cp = pltpu.make_async_copy(wqkv_hbm.bitcast(U32), wqkv_v, sems.at[10])
    wo_cp = [pltpu.make_async_copy(wo_hbm.bitcast(U32).at[:, pl.ds(t * C, C)],
                                   wo_v.at[t, :D // 2], sems.at[20 + t])
             for t in range(D // C)]
    for cp in small_cp + par_cp[0] + par_cp[1]:
        cp.start()
    for cp in small_cp + par_cp[0]:
        cp.wait()
    for cp in x_cp + [fk_cp, wqkv_cp] + wo_cp + [tab_cp]:
        cp.start()

    lane = lax.broadcasted_iota(jnp.int32, (8, C), 1)
    sub = lax.broadcasted_iota(jnp.int32, (8, C), 0)
    rho = _tap_offsets()

    zero = zero_s[0]

    def pin(ref, x, k=1):
        ref[ref.shape[0] - 1 + k * zero, :8, :C] = pltpu.bitcast(x[:8, :C], ref.dtype)

    gate_v[0] = jnp.zeros((8, C), U32)

    def gated(w):
        tail = w[-8:] | jnp.concatenate([gate_v[0]] * (w.shape[1] // C), axis=1)
        return _halves(jnp.concatenate([w[:-8], tail], axis=0))

    regions = []

    def region(fn, *args):
        regions.append(fn)
        pl.when(zero < len(regions))(lambda: fn(*args))

    def pacer(lag, ref, k=1):
        queue = []

        def pace(x):
            queue.append(x)
            if len(queue) > lag:
                pin(ref[0], queue.pop(0), k)
            return x
        return pace

    dt_row = jnp.exp(ldt_ref[...].astype(F32).reshape(1, D)).astype(BF16).astype(F32)
    dk_row = dsk_ref[...].astype(F32).reshape(1, D)
    for b in range(D // C):
        cols = slice(b * C, (b + 1) * C)
        dt_v[cols, :] = jnp.broadcast_to(dt_row[:, cols], (C, C)).T
        dk_v[cols, :] = jnp.broadcast_to(dk_row[:, cols], (C, C)).T

    keys = [(s, p) for p in (16, 8, 4, 12, 2, 6, 10, 14, *range(1, 16, 2))
            for s in range(8) if p == 16 or p in rho[s]]

    def flip(x):
        x = pltpu.roll(x, 4, 0)
        x = jnp.where((sub & 2) == 0, pltpu.roll(x, 6, 0), pltpu.roll(x, 2, 0))
        return jnp.where((sub & 1) == 0, pltpu.roll(x, 7, 0), pltpu.roll(x, 1, 0))

    def discretise(i):
        a_re, a_im, b_re, b_im, c_re, c_im = [
            _halves(par_v[n, pl.ds(i * 8, 8), :]).astype(F32) for n in range(6)]
        rows = pl.ds(i * 16, 16)
        dt = dt_v[rows, :]
        mag, ph = jnp.exp(dt * a_re), dt * a_im
        w = _cmul((c_re, c_im), (dt * b_re, dt * b_im))
        tap0 = dk_v[rows, :] + jnp.sum(w[0], axis=1, keepdims=True)
        return mag * jnp.cos(ph), mag * jnp.sin(ph), *w, tap0

    def taps(i, a_re, a_im, w_re, w_im, tap0):
        rows = pl.ds(i * 8, 8)
        a = {1: (a_re, a_im)}
        for n in range(4):
            a[2 << n] = _csq(a[1 << n])
        right = [(jnp.ones((8, C), F32), jnp.zeros((8, C), F32)), (flip(a[16][0]), -flip(a[16][1]))]
        for j in range(2, 16):
            right.append(_csq(right[j // 2]) if j % 2 == 0 else
                         _cmul(right[j // 2], right[j // 2 + 1]))
        a[256] = [flip(t) for t in _csq((right[8][0], -right[8][1]))]
        left = {(0, 0): (w_re, w_im)}
        for s, p in keys:
            left[s, p] = (_cmul(left[s - 1, p], a[256]) if s else
                          _cmul(left[0, p & (p - 1)], a[p & -p]))
        res = _dot(*[jnp.concatenate([jnp.concatenate(v, axis=1) for v in vals], axis=0)
                     for vals in ([left[k] for k in keys], right)], _NT)
        part = {k: pltpu.roll(res[8 * n:8 * n + 8], k[0], 1, stride=1, stride_axis=0)
                for n, k in enumerate(keys)}
        pos, memo = (lane - 7) & (C - 1), {}

        def merge(ps, s=0):
            if len(ps) == 1 or not any(ps):
                return part[s, ps[0]]
            if (ps, s) not in memo:
                h = len(ps) // 2
                memo[ps, s] = jnp.where((pos & h) == 0, merge(ps[:h], s), merge(ps[h:], s + h))
            return memo[ps, s]

        t16 = merge((16,) * 8)
        t0 = jnp.where(pos < 8, pltpu.roll(t16, 9, 1), pltpu.roll(t16, 8, 1))
        t0 = jnp.where(pos == 0, tap0, t0)
        for s in range(8):
            part[s, 0] = t0
        for r in range(R):
            kt_v[r, rows, :] = merge(tuple(rho[s][r] for s in range(8)))

    def filters(lo, hi):
        for i in range(lo, hi):
            vals = discretise(i)
            for h in range(2):
                taps(2 * i + h, *[v[8 * h:8 * h + 8] for v in vals])

    with jax.named_scope("filter"):
        filters(0, HEAD)
        for cp in par_cp[1]:
            cp.wait()
        filters(HEAD, D // 16)

    def spectra(lo, hi, size, pace=lambda x: x):
        for row in range(lo, hi, size):
            rows = pl.ds(row, size)
            for r in range(8):
                ev, od = _split(lambda n: kt_v[n, rows, :], fk_v, r)
                kh_v[r, rows, :], kh_v[r + 8, rows, :] = pace(ev), od
                yield

    def keep(r, acc):
        for n, t in enumerate(_stats(acc)):
            st_v[r, n] = jnp.broadcast_to(t, (8, C))

    def load():
        for i in range(R // 2):
            acc = [None, None]
            for b in range(D // C):
                rows = pl.ds(b * C, C)
                wd = io_v[i, :, rows].T
                if b:
                    pin(fk_v, jnp.add(*acc[0]) + jnp.add(*acc[1]))
                for e, w in enumerate((wd << 16, wd & jnp.uint32(0xFFFF0000))):
                    x_v[2 * i + e, rows, :] = x = pltpu.bitcast(w, F32)
                    acc[e] = _sums(x, acc[e])
                yield
            for e in range(2):
                keep(2 * i + e, acc[e])

    hp = DH // 4

    def qkv_weights():
        row = lax.broadcasted_iota(jnp.int32, (C, C), 0)
        col = lax.broadcasted_iota(jnp.int32, (C, C), 1)
        dh = ((row >> 2) & 1) + 8 * ((row >> 4) & 1) + 2 * (row >> 5)
        pick = jnp.where(col == (2 * (row & 3) + ((row >> 3) & 1)) * DH + dh, 1.0, 0.0)
        for j in range(3 * D // C):
            w = _dot(pick, _halves(wqkv_v[:, pl.ds(j * C, C)]), _NT)
            for n in range(C // 32):
                part = w[32 * n:32 * n + 32]
                for i, a in enumerate(_lhs_terms(part[:, :D // 2], part[:, D // 2:])):
                    wt_v[j, i, pl.ds(8 * n, 8), :] = _pairs(a)
            yield

    def out_weights():
        rows = [g * C // 2 + h * hp + i for h in range(2) for g in range(D // C) for i in range(hp)]
        for j in range(D // C):
            for c in range(2):
                halves = [_halves(jnp.concatenate(
                    [wo_v[j, pl.ds(row, 8, stride=DH // 2), :] for row in rows[8 * k:8 * k + 8]],
                    axis=0)).T.astype(F32) for k in (c, c + 2)]
                for i, a in enumerate(_lhs_terms(*halves)):
                    wot_v[j, i, :, pl.ds(c * C, C)] = _words(a)
                yield

    for cp in x_cp + [fk_cp, wqkv_cp] + wo_cp:
        cp.wait()
    with jax.named_scope("load"):
        region(_run, (spectra(0, D // 2, CB, pacer(4, [io_v])), 32), (load(), 32),
               (qkv_weights(), 12))
    tab_cp.wait()

    def units(b):
        return [(pl.ds(b * CB + i // 2 * 8, 8), range(i % 2 * 8, i % 2 * 8 + 8))
                for i in range(CB // 4)]

    def filter_fft(b):
        for rows, rs in units(b):
            for r, k in zip(rs, _fft([(kh_v[r, rows, :C], kh_v[r, rows, C:]) for r in rs])):
                kh_v[r, rows, :C], kh_v[r, rows, C:] = k
            yield

    def forward(b):
        rows = pl.ds(b * CB, CB)

        def normed(n):
            m, s = [jnp.concatenate([st_v[n, i]] * (CB // 8), axis=0) for i in range(2)]
            return (x_v[n, rows, :] - m) * s

        for r in range(8):
            s_v[r, rows, :], s_v[r + 8, rows, :] = _split(normed, tab_v, r)
            yield

    def inverse(b):
        rows = pl.ds(b * CB, CB)
        for r in range(8):
            ev = s_v[r, rows, :]
            od = _twiddle((s_v[r + 8, rows, C:], s_v[r + 8, rows, :C]), r, R)
            od = jnp.concatenate(od[::-1], axis=1)
            for n, z in ((r, ev + od), (r + 8, ev - od)):
                x_v[n, rows, :] += _dot(z, _halves(tab_v[R + n]))
            yield

    def mix(b):
        for rows, rs in units(b):
            uf = _fft([(s_v[r, rows, :C], s_v[r, rows, C:]) for r in rs])
            yf = [_cmul(u, (kh_v[r, rows, :C], kh_v[r, rows, C:])) for r, u in zip(rs, uf)]
            yield
            for r, z in zip(rs, _ifft(yf)):
                s_v[r, rows, :C], s_v[r, rows, C:] = z

    def conv(first, k):
        fwd, mid, inv = [range(*span) for span in zip(PLAN[k], PLAN[k + 1])]
        nxt = range(PLAN[k + 1][1], PLAN[k + 2][1]) if first and k + 2 < len(PLAN) else ()
        _run((_chain(forward(b) for b in fwd), 8 * len(fwd)),
             (_chain(inverse(b) for b in inv), 8 * len(inv), 0.03, 1.03),
             *[(spectra(D // 2 + k * C, D // 2 + k * C + C, CB), 16, 0.031, 1.031)] * (first and k < 2),
             (_chain(mix(b) for b in mid), CB // 4 * len(mid)),
             (_chain(filter_fft(b) for b in nxt), CB // 4 * len(nxt)))

    groups, heads, chunks = R // 2, D // C, (1, 2, 0)
    n_qkv, n_att, n_term = NP * len(chunks), 44, D // 32

    def moments(p, stats):
        for r in range(2 * p, 2 * p + 2):
            acc = None
            for b in range(8):
                for row in range(b * 64, b * 64 + 64, 32):
                    acc = _sums(x_v[r + (zero if p > 1 else 0), pl.ds(row, 32), :], acc)
                pin(gate_v, jnp.add(*acc))
                stats[r] = acc if b < 7 else _stats(acc)
                yield

    def norm(p, stats):
        for i in range(n_term):
            cols = [(jnp.concatenate(
                [x_v[r - (zero if p else 0), pl.ds(h + 16 * i, 8, stride=2), :]
                 for h in (0, 1, D // 2, D // 2 + 1)],
                axis=0) - stats[r][0]) * stats[r][1] for r in (2 * p, 2 * p + 1)]
            for n, b in enumerate(_rhs_terms(*cols)):
                xt_v[p][zero + n, pl.ds(8 * i, 8), :] = wd = _pairs(b)
                pin(gate_v, wd)
            yield

    def qkv(g, t, p, pace):
        def emit(i, j, val):
            if t == 0:
                q_v[g % 2][p][j + zero, pl.ds(i * C // 2, C // 2), :] = val
                return
            rows = pl.ds((t - 1) * C + i * C // 2, C // 2)
            kv_v[g % 2][16 * j + 8 + p + zero, rows, :] = val
            if p:
                kv_v[g % 2][16 * j + p + zero, rows, :] = pltpu.roll(val, 1, 1)

        return _strassen(lambda i: pace(_dot(
            gated(wt_v[t * heads + g, i]), _halves(xt_v[p][i]))), emit)

    def attend(g, p):
        buf = kv_v[g % 2]
        for j in range(2):
            window = pl.ds(16 * j + p + 1, WIN)
            for dh in range(DH):
                t = q_v[g % 2][p][j, pl.ds(dh * 8, 8), :] * buf[window, pl.ds(dh * 8, 8), :]
                logits = t if dh == 0 else logits + t
                if dh % 2:
                    for w in range(dh // 2 % 2, WIN, 2):
                        pin(gate_v, logits[w])
                    yield
            if p < WIN - 1:
                logits = jnp.concatenate(
                    [jnp.where(lane == 0, -1e9 / SCALE, logits[:WIN - 1 - p]), logits[WIN - 1 - p:]])
            ex = jnp.exp2((logits - _fold(jnp.maximum, logits)) * (SCALE * float(np.log2(np.e))))
            pr = ex * (1.0 / _fold(jnp.add, ex))
            yield from range(4)
            for i in range(hp):
                for h in range(2):
                    for e in range(2):
                        rows = pl.ds(C + (2 * (h * hp + i) + e) * 8, 8)
                        o = _fold(jnp.add, pr * buf[window, rows, :])
                        held_v[j + zero, i, pl.ds(16 * h + 8 * e, 8), :] = o
                        pin(gate_v, o)
                    yield
        for i in range(hp):
            cols = [held_v[j, i] for j in range(2)]
            for t, b in enumerate(_rhs_terms(*cols)):
                ot_v[p][zero + t, pl.ds((g * hp + i) * 8, 8), :] = wd = _pairs(b)
                if t % 2 == 0:
                    pin(gate_v, wd)
            yield

    sums = {}

    def project(last, t, p, pace):
        def emit(i, j, val):
            r, rows = 2 * p + j, pl.ds(t * C + i * C // 2, C // 2)
            x = x_v[r, rows, :] + val
            if not last:
                x_v[r, rows, :] = x
                sums[r] = _sums(x, sums.get(r))
            elif j:
                y_v[p % 2][zero, rows, :] = _pairs(jnp.concatenate([sums.pop(r - 1), x], axis=0))
            else:
                sums[r] = x

        return _strassen(lambda i: pace(_dot(gated(wot_v[t, i]), _halves(ot_v[p][i]))), emit)

    def out_copy(n):
        return pltpu.make_async_copy(io_v.at[n], out_w.at[:, n, :], sems.at[12 + n])

    sent = []

    def send(p):
        for n in range(len(sent), p):
            sent.append(n)
            out_copy(n).start()

    def finish(last, p):
        for b in range(D // C):
            if last:
                io_v[p, :, pl.ds(b * C, C)] = y_v[p % 2][0, pl.ds(b * C, C), :].T
            elif b % 2 == 0:
                keep(2 * p + b // 2, sums[2 * p + b // 2])
            yield

    def first_heads():
        pace, stats = pacer(LAG, [x_v], 2), {}
        _run(*[(inverse(b), 8) for b in range(PLAN[-1][2], D // CB)],
             (moments(0, stats), 16, 0.3, 0.55), (moments(1, stats), 16, 0.6, 1.0),
             (norm(0, stats), n_term, 0.6, 1.0))
        for p in range(groups):
            _run((_chain(qkv(0, n, p, pace) for n in chunks), n_qkv),
                 *[(norm(p + 1, stats), n_term, 0.0, 0.85)] * (p + 1 < groups),
                 *[(moments(p + 2, stats), 16)] * (p + 2 < groups))

    def attends(g, reading):
        todo = [(g - 1, p) for p in range(EARLY[g - 1], groups)] + [(g, p) for p in range(EARLY[g])]

        def steps():
            for h, p in todo:
                reading[0] = kv_v[h % 2]
                yield from attend(h, p)

        return steps(), n_att * len(todo)

    def projections(last, pace):
        for p in range(groups):
            for t in range(D // C):
                if last and t == 2 and p in (groups - 4, groups - 2):
                    send(p)
                yield from project(last, t, p, pace)

    def next_heads(g):
        reading = [None]
        pace = pacer(LAG, reading)
        _run((_chain(qkv(g, t, p, pace) for t in chunks for p in range(groups)), n_qkv * groups),
             attends(g, reading))

    def output(last):
        reading = [None]
        _run((projections(last, pacer(LAG, reading)), groups * NP * D // C),
             (*attends(heads, reading), 0.0, 0.85),
             *[(finish(last, p - 1), D // C, (p + 0.2) / groups, (p + 0.5) / groups)
               for p in range(1, groups)])
        if last:
            send(groups - 1)
        _run((finish(last, groups - 1), D // C, 0.0, 0.5), *[(forward(0), 8)] * (not last))

    _run((forward(0), 8), (filter_fft(0), CB // 4), (out_weights(), 8))
    for last in (False, True):
        with jax.named_scope("conv"):
            for k in range(len(PLAN) - 1):
                region(conv, not last, k)
        with jax.named_scope("kv"):
            region(first_heads)
        with jax.named_scope("mid"):
            for g in range(1, heads):
                region(next_heads, g)
        with jax.named_scope("attn"):
            region(output, last)

    send(groups)
    for p in range(groups):
        out_copy(p).wait()


@jax.jit
def pallas_interleave_layers__ssm_conv_s4__sliding_local_dilated__prompt_kernel(
    A_u: jax.Array,
    A_A_re: jax.Array,
    A_A_im: jax.Array,
    A_B_re: jax.Array,
    A_B_im: jax.Array,
    A_C_re: jax.Array,
    A_C_im: jax.Array,
    A_log_dt: jax.Array,
    A_Dskip: jax.Array,
    B_x: jax.Array,
    B_wqkv: jax.Array,
    B_wo: jax.Array,
):
    del B_x
    assert A_u.shape == (1, L, D) and A_A_re.shape == (D, N) and A_A_re.dtype == BF16
    hbm = pl.BlockSpec(memory_space=pl.ANY)
    out = pl.pallas_call(
        _kernel,
        in_specs=[hbm] * 14,
        out_specs=hbm,
        out_shape=jax.ShapeDtypeStruct((C, R, D), BF16),
        scratch_shapes=[
            pltpu.VMEM((R // 2 + 1, C, D), U32),
            pltpu.VMEM((6, D // 2, N), U32),
            pltpu.VMEM((D // 2, 3 * D), U32),
            pltpu.VMEM((D // C, D // 2 + 8, C), U32),
            pltpu.VMEM((2 * R, C, C), U32),
            pltpu.VMEM((R + 1, C, C), U32),
            pltpu.VMEM((D, C), F32),
            pltpu.VMEM((D, C), F32),
            pltpu.VMEM((3 * D // C, NP, C // 4, D // 2), U32),
            pltpu.VMEM((D // C, NP, C // 4, D // 2), U32),
            pltpu.VMEM((R + 1, D + 8, C), F32),
            pltpu.VMEM((R, 2, 8, C), F32),
            pltpu.VMEM((R, D, C), F32),
            pltpu.VMEM((R, D, 2 * C), F32),
            *[[pltpu.VMEM((NP, D // 4, C), U32)] * (R // 2)] * 2,
            pltpu.VMEM((2, DH // 4, 32, C), F32),
            pltpu.VMEM((2, 8, C), U32),
            pltpu.VMEM((R, D, 2 * C), F32),
            [[pltpu.VMEM((2, C, C), F32)] * (R // 2)] * 2,
            [pltpu.VMEM((2 * R + 1, 2 * C, C), F32)] * 2,
            [pltpu.VMEM((1, D, C), U32)] * 2,
            *[pltpu.VMEM((D,), BF16)] * 2,
            pltpu.SMEM((1,), jnp.int32),
            pltpu.SemaphoreType.DMA((24,)),
        ],
        compiler_params=pltpu.CompilerParams(vmem_limit_bytes=100 * 1024 * 1024),
    )(A_u.reshape(C, R, D), A_A_re, A_A_im, A_B_re, A_B_im, A_C_re, A_C_im,
      A_log_dt, A_Dskip, B_wqkv, B_wo, *_dft_tables(),
      np.zeros((1,), np.int32))
    return out.reshape(1, L, D)
```

```python
import ml_dtypes
import numpy as np

import jax
import jax.numpy as jnp
from jax import lax
import jax.experimental.pallas as pl
import jax.experimental.pallas.tpu as pltpu

L, D, N = 2048, 512, 128
R, C = 16, 128
DH, WIN = 16, 8
CB = 64
NP = 7
PLAN = ((1, 0, 0), (3, 1, 0), (6, 3, 0), (8, 6, 2), (8, 8, 6))
LAG = 4
EARLY = (0, 0, 1, 2, 0)
HEAD = 3
EPS, SCALE = 1e-5, DH ** -0.5
F32, BF16, U32 = jnp.float32, jnp.bfloat16, jnp.uint32
_NT = (((1,), (1,)), ((), ()))


def _host_words(a):
    h = np.ascontiguousarray(a).astype(ml_dtypes.bfloat16).view(np.uint16).astype(np.uint32)
    return h[..., 0::2, :] | (h[..., 1::2, :] << 16)


def _dft_tables():
    t = R * np.arange(C)[None, :, None] + np.arange(R)[:, None, None]
    ang = 2.0 * np.pi * (np.arange(C)[None, None, :] + 0.5) * t / (2 * L)
    fwd = np.concatenate([np.cos(ang), -np.sin(ang)], axis=-1)
    p = (np.arange(C) - 7) % C
    fwd_k = fwd[:, 16 * (p % 8) + p // 8, :] / L
    inv = fwd.transpose(0, 2, 1)
    fwd, fwd_k = [np.concatenate([a[..., :C], a[..., C:]], axis=1) for a in (fwd, fwd_k)]
    return _host_words(np.concatenate([fwd, inv])), _host_words(fwd_k)


def _tap_offsets():
    l = np.arange(L)
    lr = l.astype(np.float32).astype(ml_dtypes.bfloat16).astype(np.float32).astype(np.int64)
    rho = (lr - (l // R) * R).reshape(8, 16, R)
    assert (rho == rho[:, :1]).all()
    return rho[:, 0].tolist()


def _cmul(a, b):
    return a[0] * b[0] - a[1] * b[1], a[0] * b[1] + a[1] * b[0]


def _csq(a):
    t = a[0] * a[1]
    return a[0] * a[0] - a[1] * a[1], t + t


def _twiddle(a, k, n):
    if k == 0:
        return a
    if 4 * k == n:
        return a[1], -a[0]
    h = float(np.sqrt(0.5))
    if 8 * k == n:
        return (a[0] + a[1]) * h, (a[1] - a[0]) * h
    if 8 * k == 3 * n:
        return (a[1] - a[0]) * h, (a[0] + a[1]) * (-h)
    w = (float(np.cos(2 * np.pi * k / n)), float(-np.sin(2 * np.pi * k / n)))
    return _cmul(a, w)


def _fft(x):
    n = len(x)
    if n == 1:
        return x
    if n == 2:
        return [(x[0][0] + x[1][0], x[0][1] + x[1][1]), (x[0][0] - x[1][0], x[0][1] - x[1][1])]
    e, o1, o3 = _fft(x[0::2]), _fft(x[1::4]), _fft(x[3::4])
    out = [None] * n
    q = n // 4
    for k in range(q):
        a, b = _twiddle(o1[k], k, n), _twiddle(o3[k], 3 * k, n)
        s = (a[0] + b[0], a[1] + b[1])
        d = (a[0] - b[0], a[1] - b[1])
        out[k] = (e[k][0] + s[0], e[k][1] + s[1])
        out[k + 2 * q] = (e[k][0] - s[0], e[k][1] - s[1])
        out[k + q] = (e[k + q][0] + d[1], e[k + q][1] - d[0])
        out[k + 3 * q] = (e[k + q][0] - d[1], e[k + q][1] + d[0])
    return out


def _ifft(x):
    return [(b, a) for a, b in _fft([(b, a) for a, b in x])]


def _fold(op, x):
    while x.shape[0] > 1:
        x = op(x[:x.shape[0] // 2], x[x.shape[0] // 2:])
    return x[0]


def _sums(x, acc=None):
    x = x.reshape(-1, 8, C)
    new = _fold(jnp.add, x), _fold(jnp.add, x * x)
    return new if acc is None else (acc[0] + new[0], acc[1] + new[1])


def _stats(acc):
    m, sq = [jnp.sum(t, axis=0, keepdims=True) * (1.0 / D) for t in acc]
    return m, lax.rsqrt(jnp.maximum(sq - m * m, 0.0) + EPS)


def _words(x):
    return pltpu.bitcast(x.astype(BF16), U32)


def _pairs(x):
    b = pltpu.bitcast(x, U32) + jnp.uint32(0x8000)
    return (b[x.shape[0] // 2:] & jnp.uint32(0xFFFF0000)) | (b[:x.shape[0] // 2] >> 16)


def _halves(w):
    return pltpu.bitcast(w, BF16)


def _dot(a, b, dims=(((1,), (0,)), ((), ()))):
    return lax.dot_general(a.astype(BF16), b.astype(BF16), dims, preferred_element_type=F32)


def _split(src, table, r):
    lo, hi = [_dot(src(n), _halves(jnp.concatenate(
        [table[n, :C // 2], table[n, C // 2:]], axis=1))) for n in (r, r + 8)]
    d = lo - hi
    return lo + hi, jnp.concatenate(_twiddle((d[:, :C], d[:, C:]), r, R), axis=1)


def _run(*jobs):
    order = []
    for k, (_, n, *span) in enumerate(jobs):
        lo, hi = span or (0.0, 1.0)
        order += [(lo + (hi - lo) * i / n, k) for i in range(n)]
    for _, k in sorted(order):
        next(jobs[k][0])
    for job in jobs:
        for _ in job[0]:
            pass


def _chain(gens):
    for g in gens:
        yield from g


def _lhs_terms(left, right):
    m = left.shape[0] // 2
    a11, a12, a21, a22 = left[:m], right[:m], left[m:], right[m:]
    return a11 + a22, a21 + a22, a22, a12 - a22, a21 - a11, a11, a11 + a12


def _rhs_terms(left, right):
    k = left.shape[0] // 2
    b11, b12, b21, b22 = left[:k], right[:k], left[k:], right[k:]
    return b11 + b22, b11, b21 - b11, b21 + b22, b11 + b12, b12 - b22, b22


def _strassen(product, emit):
    m1 = product(0)
    yield
    m2 = product(1)
    yield
    m4 = product(2)
    yield
    c11, c22 = m1 + m4, m1 - m2
    emit(1, 0, m2 + m4)
    c22 += product(4)
    yield
    m3 = product(5)
    yield
    emit(1, 1, c22 + m3)
    c11 += product(3)
    yield
    m5 = product(6)
    yield
    emit(0, 0, c11 - m5)
    emit(0, 1, m3 + m5)


def _kernel(x_hbm, are_hbm, aim_hbm, bre_hbm, bim_hbm, cre_hbm, cim_hbm, ldt_hbm, dsk_hbm,
            wqkv_hbm, wo_hbm, tab_hbm, fk_hbm, zero_hbm, out_hbm,
            io_v, par_v, wqkv_v, wo_v, tab_v, fk_v, dt_v, dk_v, wt_v, wot_v,
            x_v, st_v, kt_v, kh_v, xt_v, ot_v, held_v, gate_v, s_v,
            q_v, kv_v, y_v, ldt_ref, dsk_ref, zero_s, sems):
    srcs = (are_hbm, aim_hbm, bre_hbm, bim_hbm, cre_hbm, cim_hbm)
    par_cp = [[pltpu.make_async_copy(s.bitcast(U32).at[rows], par_v.at[i, rows], sems.at[k])
               for i, s in enumerate(srcs)]
              for k, rows in enumerate((pl.ds(0, HEAD * 8), pl.ds(HEAD * 8, D // 2 - HEAD * 8)))]
    small_cp = [pltpu.make_async_copy(*pair, sems.at[2 + i]) for i, pair in enumerate(
        ((ldt_hbm, ldt_ref), (dsk_hbm, dsk_ref), (zero_hbm, zero_s)))]
    x_w, out_w = x_hbm.bitcast(U32), out_hbm.bitcast(U32)
    x_cp = [pltpu.make_async_copy(x_w.at[:, i, :], io_v.at[i], sems.at[12 + i])
            for i in range(R // 2)]
    fk_cp = pltpu.make_async_copy(fk_hbm, fk_v.at[:R], sems.at[7])
    tab_cp = pltpu.make_async_copy(tab_hbm, tab_v, sems.at[8])
    wqkv_cp = pltpu.make_async_copy(wqkv_hbm.bitcast(U32), wqkv_v, sems.at[10])
    wo_cp = [pltpu.make_async_copy(wo_hbm.bitcast(U32).at[:, pl.ds(t * C, C)],
                                   wo_v.at[t, :D // 2], sems.at[20 + t])
             for t in range(D // C)]
    for cp in small_cp + par_cp[0] + par_cp[1]:
        cp.start()
    for cp in small_cp + par_cp[0]:
        cp.wait()
    for cp in x_cp + [fk_cp, wqkv_cp] + wo_cp + [tab_cp]:
        cp.start()

    lane = lax.broadcasted_iota(jnp.int32, (8, C), 1)
    sub = lax.broadcasted_iota(jnp.int32, (8, C), 0)
    rho = _tap_offsets()

    zero = zero_s[0]

    spare = {n: n - 1 + 2 * zero for n in (2, R // 2 + 1, R + 1, 2 * R + 1)}

    def pin(ref, x):
        x = x if x.dtype == ref.dtype else pltpu.bitcast(x, ref.dtype)
        ref[spare[ref.shape[0]], :x.shape[0], :C] = x

    gate_v[0, :8] = jnp.zeros((8, C), F32)

    def gated(w):
        tail = w[-8:] | jnp.concatenate([pltpu.bitcast(gate_v[0, :8], U32)] * 2, axis=1)
        return _halves(jnp.concatenate([w[:-8], tail], axis=0))

    regions = []

    def region(fn, *args):
        regions.append(fn)
        pl.when(zero < len(regions))(lambda: fn(*args))

    def pacer(lag, ref):
        queue = []

        def pace(x):
            queue.append(x)
            if len(queue) > lag:
                pin(ref[0], queue.pop(0)[:8, :C])
            return x
        return pace

    dt_row = jnp.exp(ldt_ref[...].astype(F32).reshape(1, D)).astype(BF16).astype(F32)
    dk_row = dsk_ref[...].astype(F32).reshape(1, D)
    for b in range(D // C):
        cols = slice(b * C, (b + 1) * C)
        dt_v[cols, :] = jnp.broadcast_to(dt_row[:, cols], (C, C)).T
        dk_v[cols, :] = jnp.broadcast_to(dk_row[:, cols], (C, C)).T

    keys = [(s, p) for p in (16, 8, 4, 12, 2, 6, 10, 14, *range(1, 16, 2))
            for s in range(8) if p == 16 or p in rho[s]]

    pos = (lane - 7) & (C - 1)
    lower = {h: (pos & h) == 0 for h in (1, 2, 4)}
    upper = {h: (sub & h) == 0 for h in (1, 2)}

    def flip(x):
        x = pltpu.roll(x, 4, 0)
        x = lax.select(upper[2], pltpu.roll(x, 6, 0), pltpu.roll(x, 2, 0))
        return lax.select(upper[1], pltpu.roll(x, 7, 0), pltpu.roll(x, 1, 0))

    def discretise(i):
        a_re, a_im, b_re, b_im, c_re, c_im = [
            _halves(par_v[n, pl.ds(i * 8, 8), :]).astype(F32) for n in range(6)]
        rows = pl.ds(i * 16, 16)
        dt = dt_v[rows, :]
        mag, ph = jnp.exp(dt * a_re), dt * a_im
        w = _cmul((c_re, c_im), (dt * b_re, dt * b_im))
        tap0 = dk_v[rows, :] + jnp.sum(w[0], axis=1, keepdims=True)
        return mag * jnp.cos(ph), mag * jnp.sin(ph), *w, tap0

    def taps(i, a_re, a_im, w_re, w_im, tap0):
        rows = pl.ds(i * 8, 8)
        a = {1: (a_re, a_im)}
        for n in range(4):
            a[2 << n] = _csq(a[1 << n])
        right = [(jnp.ones((8, C), F32), jnp.zeros((8, C), F32)), (flip(a[16][0]), -flip(a[16][1]))]
        for j in range(2, 16):
            right.append(_csq(right[j // 2]) if j % 2 == 0 else
                         _cmul(right[j // 2], right[j // 2 + 1]))
        a[256] = [flip(t) for t in _csq((right[8][0], -right[8][1]))]
        left = {(0, 0): (w_re, w_im)}
        for s, p in keys:
            left[s, p] = (_cmul(left[s - 1, p], a[256]) if s else
                          _cmul(left[0, p & (p - 1)], a[p & -p]))
        res = _dot(*[jnp.concatenate([jnp.concatenate(v, axis=1) for v in vals], axis=0)
                     for vals in ([left[k] for k in keys], right)], _NT)
        part = {k: pltpu.roll(res[8 * n:8 * n + 8], k[0], 1, stride=1, stride_axis=0)
                for n, k in enumerate(keys)}
        memo = {}

        def merge(ps, s=0):
            if len(ps) == 1 or not any(ps):
                return part[s, ps[0]]
            if (ps, s) not in memo:
                h = len(ps) // 2
                memo[ps, s] = lax.select(lower[h], merge(ps[:h], s), merge(ps[h:], s + h))
            return memo[ps, s]

        t16 = merge((16,) * 8)
        t0 = jnp.where(pos < 8, pltpu.roll(t16, 9, 1), pltpu.roll(t16, 8, 1))
        t0 = jnp.where(pos == 0, tap0, t0)
        for s in range(8):
            part[s, 0] = t0
        for r in range(R):
            kt_v[r, rows, :] = merge(tuple(rho[s][r] for s in range(8)))

    def filters(lo, hi):
        for i in range(lo, hi):
            vals = discretise(i)
            for h in range(2):
                taps(2 * i + h, *[v[8 * h:8 * h + 8] for v in vals])

    with jax.named_scope("filter"):
        filters(0, HEAD)
        for cp in par_cp[1]:
            cp.wait()
        filters(HEAD, D // 16)

    def spectra(lo, hi, size, pace=lambda x: x):
        for row in range(lo, hi, size):
            rows = pl.ds(row, size)
            for r in range(8):
                ev, od = _split(lambda n: kt_v[n, rows, :], fk_v, r)
                kh_v[r, rows, :], kh_v[r + 8, rows, :] = pace(ev), od
                yield

    def keep(r, acc):
        for n, t in enumerate(_stats(acc)):
            st_v[r, n] = jnp.broadcast_to(t, (8, C))

    def load():
        for i in range(R // 2):
            acc = [None, None]
            for b in range(D // C):
                rows = pl.ds(b * C, C)
                wd = io_v[i, :, rows].T
                if b:
                    pin(fk_v, jnp.add(*acc[0]) + jnp.add(*acc[1]))
                for e, w in enumerate((wd << 16, wd & jnp.uint32(0xFFFF0000))):
                    x_v[2 * i + e, rows, :] = x = pltpu.bitcast(w, F32)
                    acc[e] = _sums(x, acc[e])
                yield
            for e in range(2):
                keep(2 * i + e, acc[e])

    hp = DH // 4

    def qkv_weights():
        row = lax.broadcasted_iota(jnp.int32, (C, C), 0)
        col = lax.broadcasted_iota(jnp.int32, (C, C), 1)
        dh = ((row >> 2) & 1) + 8 * ((row >> 4) & 1) + 2 * (row >> 5)
        pick = jnp.where(col == (2 * (row & 3) + ((row >> 3) & 1)) * DH + dh, 1.0, 0.0)
        for j in range(3 * D // C):
            w = _dot(pick, _halves(wqkv_v[:, pl.ds(j * C, C)]), _NT)
            for n in range(C // 32):
                part = w[32 * n:32 * n + 32]
                for i, a in enumerate(_lhs_terms(part[:, :D // 2], part[:, D // 2:])):
                    wt_v[j, i, pl.ds(8 * n, 8), :] = _pairs(a)
            yield

    def out_weights():
        rows = [g * C // 2 + h * hp + i for h in range(2) for g in range(D // C) for i in range(hp)]
        for j in range(D // C):
            for c in range(2):
                halves = [_halves(jnp.concatenate(
                    [wo_v[j, pl.ds(row, 8, stride=DH // 2), :] for row in rows[8 * k:8 * k + 8]],
                    axis=0)).T.astype(F32) for k in (c, c + 2)]
                for i, a in enumerate(_lhs_terms(*halves)):
                    wot_v[j, i, :, pl.ds(c * C, C)] = _words(a)
                yield

    for cp in x_cp + [fk_cp, wqkv_cp] + wo_cp:
        cp.wait()
    with jax.named_scope("load"):
        region(_run, (spectra(0, D // 2, CB, pacer(4, [io_v])), 32), (load(), 32),
               (qkv_weights(), 12))
    tab_cp.wait()

    def units(b):
        return [(pl.ds(b * CB + i // 2 * 8, 8), range(i % 2 * 8, i % 2 * 8 + 8))
                for i in range(CB // 4)]

    def filter_fft(b):
        for rows, rs in units(b):
            for r, k in zip(rs, _fft([(kh_v[r, rows, :C], kh_v[r, rows, C:]) for r in rs])):
                kh_v[r, rows, :C], kh_v[r, rows, C:] = k
            yield

    def forward(b):
        rows = pl.ds(b * CB, CB)

        def normed(n):
            m, s = [jnp.concatenate([st_v[n, i]] * (CB // 8), axis=0) for i in range(2)]
            return (x_v[n, rows, :] - m) * s

        for r in range(8):
            s_v[r, rows, :], s_v[r + 8, rows, :] = _split(normed, tab_v, r)
            yield

    def inverse(b):
        rows = pl.ds(b * CB, CB)
        for r in range(8):
            ev = s_v[r, rows, :]
            od = _twiddle((s_v[r + 8, rows, C:], s_v[r + 8, rows, :C]), r, R)
            od = jnp.concatenate(od[::-1], axis=1)
            for n, z in ((r, ev + od), (r + 8, ev - od)):
                x_v[n, rows, :] += _dot(z, _halves(tab_v[R + n]))
            yield

    def mix(b):
        for rows, rs in units(b):
            uf = _fft([(s_v[r, rows, :C], s_v[r, rows, C:]) for r in rs])
            yf = [_cmul(u, (kh_v[r, rows, :C], kh_v[r, rows, C:])) for r, u in zip(rs, uf)]
            yield
            for r, z in zip(rs, _ifft(yf)):
                s_v[r, rows, :C], s_v[r, rows, C:] = z

    def conv(first, k):
        fwd, mid, inv = [range(*span) for span in zip(PLAN[k], PLAN[k + 1])]
        nxt = range(PLAN[k + 1][1], PLAN[k + 2][1]) if first and k + 2 < len(PLAN) else ()
        _run((_chain(forward(b) for b in fwd), 8 * len(fwd)),
             (_chain(inverse(b) for b in inv), 8 * len(inv), 0.03, 1.03),
             *[(spectra(D // 2 + k * C, D // 2 + k * C + C, CB), 16, 0.031, 1.031)] * (first and k < 2),
             (_chain(mix(b) for b in mid), CB // 4 * len(mid)),
             (_chain(filter_fft(b) for b in nxt), CB // 4 * len(nxt)))

    groups, heads, chunks = R // 2, D // C, (1, 2, 0)
    n_qkv, n_att, n_term = NP * len(chunks), 44, D // 32

    def moments(p, stats):
        for r in range(2 * p, 2 * p + 2):
            acc = None
            for b in range(8):
                for row in range(b * 64, b * 64 + 64, 32):
                    acc = _sums(x_v[r + (zero if p > 1 else 0), pl.ds(row, 32), :], acc)
                pin(gate_v, jnp.add(*acc))
                stats[r] = acc if b < 7 else _stats(acc)
                yield

    def norm(p, stats):
        for i in range(n_term):
            cols = [(jnp.concatenate(
                [x_v[r - (zero if p else 0), pl.ds(h + 16 * i, 8, stride=2), :]
                 for h in (0, 1, D // 2, D // 2 + 1)],
                axis=0) - stats[r][0]) * stats[r][1] for r in (2 * p, 2 * p + 1)]
            for n, b in enumerate(_rhs_terms(*cols)):
                xt_v[p][zero + n, pl.ds(8 * i, 8), :] = wd = _pairs(b)
                pin(gate_v, wd)
            yield

    def qkv(g, t, p, pace):
        def emit(i, j, val):
            if t == 0:
                q_v[g % 2][p][j + zero, pl.ds(i * C // 2, C // 2), :] = val
                return
            rows = pl.ds((t - 1) * C + i * C // 2, C // 2)
            kv_v[g % 2][16 * j + 8 + p + zero, rows, :] = val
            if p:
                kv_v[g % 2][16 * j + p + zero, rows, :] = pltpu.roll(val, 1, 1)

        return _strassen(lambda i: pace(_dot(
            gated(wt_v[t * heads + g, i]), _halves(xt_v[p][i]))), emit)

    def attend(g, p):
        buf = kv_v[g % 2]
        for j in range(2):
            window = pl.ds(16 * j + p + 1, WIN)
            for dh in range(DH):
                t = q_v[g % 2][p][j, pl.ds(dh * 8, 8), :] * buf[window, pl.ds(dh * 8, 8), :]
                logits = t if dh == 0 else logits + t
                if dh % 2:
                    w = dh // 2 % 2 * 4
                    pin(gate_v, logits[w:w + 4].reshape(32, C))
                    yield
            if p < WIN - 1:
                logits = jnp.concatenate(
                    [jnp.where(lane == 0, -1e9 / SCALE, logits[:WIN - 1 - p]), logits[WIN - 1 - p:]])
            ex = jnp.exp2((logits - _fold(jnp.maximum, logits)) * (SCALE * float(np.log2(np.e))))
            pr = ex * (1.0 / _fold(jnp.add, ex))
            yield from range(4)
            for i in range(hp):
                for h in range(2):
                    for e in range(2):
                        rows = pl.ds(C + (2 * (h * hp + i) + e) * 8, 8)
                        o = _fold(jnp.add, pr * buf[window, rows, :])
                        held_v[j + zero, i, pl.ds(16 * h + 8 * e, 8), :] = o
                        pin(gate_v, o)
                    yield
        for i in range(hp):
            cols = [held_v[j, i] for j in range(2)]
            for t, b in enumerate(_rhs_terms(*cols)):
                ot_v[p][zero + t, pl.ds((g * hp + i) * 8, 8), :] = wd = _pairs(b)
                if t % 2 == 0:
                    pin(gate_v, wd)
            yield

    sums = {}

    def project(last, t, p, pace):
        def emit(i, j, val):
            r, rows = 2 * p + j, pl.ds(t * C + i * C // 2, C // 2)
            x = x_v[r, rows, :] + val
            if not last:
                x_v[r, rows, :] = x
                sums[r] = _sums(x, sums.get(r))
            elif j:
                y_v[p % 2][zero, rows, :] = _pairs(jnp.concatenate([sums.pop(r - 1), x], axis=0))
            else:
                sums[r] = x

        return _strassen(lambda i: pace(_dot(gated(wot_v[t, i]), _halves(ot_v[p][i]))), emit)

    def out_copy(n):
        return pltpu.make_async_copy(io_v.at[n], out_w.at[:, n, :], sems.at[12 + n])

    sent = []

    def send(p):
        for n in range(len(sent), p):
            sent.append(n)
            out_copy(n).start()

    def finish(last, p):
        for b in range(D // C):
            if last:
                io_v[p, :, pl.ds(b * C, C)] = y_v[p % 2][0, pl.ds(b * C, C), :].T
            elif b % 2 == 0:
                keep(2 * p + b // 2, sums[2 * p + b // 2])
            yield

    def first_heads():
        pace, stats = pacer(LAG, [x_v]), {}
        _run(*[(inverse(b), 8) for b in range(PLAN[-1][2], D // CB)],
             (moments(0, stats), 16, 0.3, 0.55), (moments(1, stats), 16, 0.6, 1.0),
             (norm(0, stats), n_term, 0.6, 1.0))
        for p in range(groups):
            _run((_chain(qkv(0, n, p, pace) for n in chunks), n_qkv),
                 *[(norm(p + 1, stats), n_term, 0.0, 0.85)] * (p + 1 < groups),
                 *[(moments(p + 2, stats), 16)] * (p + 2 < groups))

    def attends(g, reading):
        todo = [(g - 1, p) for p in range(EARLY[g - 1], groups)] + [(g, p) for p in range(EARLY[g])]

        def steps():
            for h, p in todo:
                reading[0] = kv_v[h % 2]
                yield from attend(h, p)

        return steps(), n_att * len(todo)

    def projections(last, pace):
        for p in range(groups):
            for t in range(D // C):
                if last and t == 2 and p in (groups - 4, groups - 2):
                    send(p)
                yield from project(last, t, p, pace)

    def next_heads(g):
        reading = [None]
        pace = pacer(LAG, reading)
        _run((_chain(qkv(g, t, p, pace) for t in chunks for p in range(groups)), n_qkv * groups),
             attends(g, reading))

    def output(last):
        reading = [None]
        _run((projections(last, pacer(LAG, reading)), groups * NP * D // C),
             (*attends(heads, reading), 0.0, 0.85),
             *[(finish(last, p - 1), D // C, (p + 0.2) / groups, (p + 0.5) / groups)
               for p in range(1, groups)])
        if last:
            send(groups - 1)
        _run((finish(last, groups - 1), D // C, 0.0, 0.5), *[(forward(0), 8)] * (not last))

    _run((forward(0), 8), (filter_fft(0), CB // 4), (out_weights(), 8))
    for last in (False, True):
        with jax.named_scope("conv"):
            for k in range(len(PLAN) - 1):
                region(conv, not last, k)
        with jax.named_scope("kv"):
            region(first_heads)
        with jax.named_scope("mid"):
            for g in range(1, heads):
                region(next_heads, g)
        with jax.named_scope("attn"):
            region(output, last)

    send(groups)
    for p in range(groups):
        out_copy(p).wait()


@jax.jit
def pallas_interleave_layers__ssm_conv_s4__sliding_local_dilated__prompt_kernel(
    A_u: jax.Array,
    A_A_re: jax.Array,
    A_A_im: jax.Array,
    A_B_re: jax.Array,
    A_B_im: jax.Array,
    A_C_re: jax.Array,
    A_C_im: jax.Array,
    A_log_dt: jax.Array,
    A_Dskip: jax.Array,
    B_x: jax.Array,
    B_wqkv: jax.Array,
    B_wo: jax.Array,
):
    del B_x
    assert A_u.shape == (1, L, D) and A_A_re.shape == (D, N) and A_A_re.dtype == BF16
    hbm = pl.BlockSpec(memory_space=pl.ANY)
    out = pl.pallas_call(
        _kernel,
        in_specs=[hbm] * 14,
        out_specs=hbm,
        out_shape=jax.ShapeDtypeStruct((C, R, D), BF16),
        scratch_shapes=[
            pltpu.VMEM((R // 2 + 1, C, D), U32),
            pltpu.VMEM((6, D // 2, N), U32),
            pltpu.VMEM((D // 2, 3 * D), U32),
            pltpu.VMEM((D // C, D // 2 + 8, C), U32),
            pltpu.VMEM((2 * R, C, C), U32),
            pltpu.VMEM((R + 1, C, C), U32),
            pltpu.VMEM((D, C), F32),
            pltpu.VMEM((D, C), F32),
            pltpu.VMEM((3 * D // C, NP, C // 4, D // 2), U32),
            pltpu.VMEM((D // C, NP, C // 4, D // 2), U32),
            pltpu.VMEM((R + 1, D + 8, C), F32),
            pltpu.VMEM((R, 2, 8, C), F32),
            pltpu.VMEM((R, D, C), F32),
            pltpu.VMEM((R, D, 2 * C), F32),
            *[[pltpu.VMEM((NP, D // 4, C), U32)] * (R // 2)] * 2,
            pltpu.VMEM((2, DH // 4, 32, C), F32),
            pltpu.VMEM((2, 32, C), F32),
            pltpu.VMEM((R, D, 2 * C), F32),
            [[pltpu.VMEM((2, C, C), F32)] * (R // 2)] * 2,
            [pltpu.VMEM((2 * R + 1, 2 * C, C), F32)] * 2,
            [pltpu.VMEM((1, D, C), U32)] * 2,
            *[pltpu.VMEM((D,), BF16)] * 2,
            pltpu.SMEM((1,), jnp.int32),
            pltpu.SemaphoreType.DMA((24,)),
        ],
        compiler_params=pltpu.CompilerParams(vmem_limit_bytes=100 * 1024 * 1024),
    )(A_u.reshape(C, R, D), A_A_re, A_A_im, A_B_re, A_B_im, A_C_re, A_C_im,
      A_log_dt, A_Dskip, B_wqkv, B_wo, *_dft_tables(),
      np.zeros((1,), np.int32))
    return out.reshape(1, L, D)
```

```python
import ml_dtypes
import numpy as np

import jax
import jax.numpy as jnp
from jax import lax
import jax.experimental.pallas as pl
import jax.experimental.pallas.tpu as pltpu

L, D, N = 2048, 512, 128
R, C = 16, 128
DH, WIN = 16, 8
CB = 64
NP = 7
PLAN = ((1, 0, 0), (3, 1, 0), (6, 3, 0), (8, 6, 2), (8, 8, 6))
LAG = 4
EARLY = (0, 0, 1, 2, 0)
HEAD = 3
EPS, SCALE = 1e-5, DH ** -0.5
F32, BF16, U32 = jnp.float32, jnp.bfloat16, jnp.uint32
_NT = (((1,), (1,)), ((), ()))


def _host_words(a):
    h = np.ascontiguousarray(a).astype(ml_dtypes.bfloat16).view(np.uint16).astype(np.uint32)
    return h[..., 0::2, :] | (h[..., 1::2, :] << 16)


def _dft_tables():
    t = R * np.arange(C)[None, :, None] + np.arange(R)[:, None, None]
    ang = 2.0 * np.pi * (np.arange(C)[None, None, :] + 0.5) * t / (2 * L)
    fwd = np.concatenate([np.cos(ang), -np.sin(ang)], axis=-1)
    p = (np.arange(C) - 7) % C
    fwd_k = fwd[:, 16 * (p % 8) + p // 8, :] / L
    inv = fwd.transpose(0, 2, 1)
    fwd, fwd_k = [np.concatenate([a[..., :C], a[..., C:]], axis=1) for a in (fwd, fwd_k)]
    return _host_words(np.concatenate([fwd, inv])), _host_words(fwd_k)


def _tap_offsets():
    l = np.arange(L)
    lr = l.astype(np.float32).astype(ml_dtypes.bfloat16).astype(np.float32).astype(np.int64)
    rho = (lr - (l // R) * R).reshape(8, 16, R)
    assert (rho == rho[:, :1]).all()
    return rho[:, 0].tolist()


def _cmul(a, b):
    return a[0] * b[0] - a[1] * b[1], a[0] * b[1] + a[1] * b[0]


def _csq(a):
    t = a[0] * a[1]
    return a[0] * a[0] - a[1] * a[1], t + t


def _twiddle(a, k, n):
    if k == 0:
        return a
    if 4 * k == n:
        return a[1], -a[0]
    h = float(np.sqrt(0.5))
    if 8 * k == n:
        return (a[0] + a[1]) * h, (a[1] - a[0]) * h
    if 8 * k == 3 * n:
        return (a[1] - a[0]) * h, (a[0] + a[1]) * (-h)
    w = (float(np.cos(2 * np.pi * k / n)), float(-np.sin(2 * np.pi * k / n)))
    return _cmul(a, w)


def _fft(x):
    n = len(x)
    if n == 1:
        return x
    if n == 2:
        return [(x[0][0] + x[1][0], x[0][1] + x[1][1]), (x[0][0] - x[1][0], x[0][1] - x[1][1])]
    e, o1, o3 = _fft(x[0::2]), _fft(x[1::4]), _fft(x[3::4])
    out = [None] * n
    q = n // 4
    for k in range(q):
        a, b = _twiddle(o1[k], k, n), _twiddle(o3[k], 3 * k, n)
        s = (a[0] + b[0], a[1] + b[1])
        d = (a[0] - b[0], a[1] - b[1])
        out[k] = (e[k][0] + s[0], e[k][1] + s[1])
        out[k + 2 * q] = (e[k][0] - s[0], e[k][1] - s[1])
        out[k + q] = (e[k + q][0] + d[1], e[k + q][1] - d[0])
        out[k + 3 * q] = (e[k + q][0] - d[1], e[k + q][1] + d[0])
    return out


def _ifft(x):
    return [(b, a) for a, b in _fft([(b, a) for a, b in x])]


def _fold(op, x):
    while x.shape[0] > 1:
        x = op(x[:x.shape[0] // 2], x[x.shape[0] // 2:])
    return x[0]


def _sums(x, acc=None):
    x = x.reshape(-1, 8, C)
    new = _fold(jnp.add, x), _fold(jnp.add, x * x)
    return new if acc is None else (acc[0] + new[0], acc[1] + new[1])


def _stats(acc):
    m, sq = [jnp.sum(t, axis=0, keepdims=True) * (1.0 / D) for t in acc]
    return m, lax.rsqrt(jnp.maximum(sq - m * m, 0.0) + EPS)


def _words(x):
    return pltpu.bitcast(x.astype(BF16), U32)


def _pairs(x):
    b = pltpu.bitcast(x, U32) + jnp.uint32(0x8000)
    return (b[x.shape[0] // 2:] & jnp.uint32(0xFFFF0000)) | (b[:x.shape[0] // 2] >> 16)


def _halves(w):
    return pltpu.bitcast(w, BF16)


def _dot(a, b, dims=(((1,), (0,)), ((), ()))):
    return lax.dot_general(a.astype(BF16), b.astype(BF16), dims, preferred_element_type=F32)


def _split(src, table, r):
    lo, hi = [_dot(src(n), _halves(jnp.concatenate(
        [table[n, :C // 2], table[n, C // 2:]], axis=1))) for n in (r, r + 8)]
    d = lo - hi
    return lo + hi, jnp.concatenate(_twiddle((d[:, :C], d[:, C:]), r, R), axis=1)


def _run(*jobs):
    order = []
    for k, (_, n, *span) in enumerate(jobs):
        lo, hi = span or (0.0, 1.0)
        order += [(lo + (hi - lo) * i / n, k) for i in range(n)]
    for _, k in sorted(order):
        next(jobs[k][0])
    for job in jobs:
        for _ in job[0]:
            pass


def _chain(gens):
    for g in gens:
        yield from g


def _lhs_terms(left, right):
    m = left.shape[0] // 2
    a11, a12, a21, a22 = left[:m], right[:m], left[m:], right[m:]
    return a11 + a22, a21 + a22, a22, a12 - a22, a21 - a11, a11, a11 + a12


def _rhs_terms(left, right):
    k = left.shape[0] // 2
    b11, b12, b21, b22 = left[:k], right[:k], left[k:], right[k:]
    return b11 + b22, b11, b21 - b11, b21 + b22, b11 + b12, b12 - b22, b22


def _strassen(product, emit):
    m1 = product(0)
    yield
    m2 = product(1)
    yield
    m4 = product(2)
    yield
    c11, c22 = m1 + m4, m1 - m2
    emit(1, 0, m2 + m4)
    c22 += product(4)
    yield
    m3 = product(5)
    yield
    emit(1, 1, c22 + m3)
    c11 += product(3)
    yield
    m5 = product(6)
    yield
    emit(0, 0, c11 - m5)
    emit(0, 1, m3 + m5)


def _kernel(x_hbm, are_hbm, aim_hbm, bre_hbm, bim_hbm, cre_hbm, cim_hbm, ldt_hbm, dsk_hbm,
            wqkv_hbm, wo_hbm, tab_hbm, fk_hbm, zero_hbm, out_hbm,
            io_v, par_v, wqkv_v, wo_v, tab_v, fk_v, dt_v, dk_v, wt_v, wot_v,
            x_v, st_v, kt_v, kh_v, xt_v, ot_v, held_v, gate_v, s_v,
            q_v, kv_v, y_v, ldt_ref, dsk_ref, zero_s, sems):
    srcs = (are_hbm, aim_hbm, bre_hbm, bim_hbm, cre_hbm, cim_hbm)
    par_cp = [[pltpu.make_async_copy(s.bitcast(U32).at[rows], par_v.at[i, rows], sems.at[k])
               for i, s in enumerate(srcs)]
              for k, rows in enumerate((pl.ds(0, HEAD * 8), pl.ds(HEAD * 8, D // 2 - HEAD * 8)))]
    small_cp = [pltpu.make_async_copy(*pair, sems.at[2 + i]) for i, pair in enumerate(
        ((ldt_hbm, ldt_ref), (dsk_hbm, dsk_ref), (zero_hbm, zero_s)))]
    x_w, out_w = x_hbm.bitcast(U32), out_hbm.bitcast(U32)
    x_cp = [pltpu.make_async_copy(x_w.at[:, i, :], io_v.at[i], sems.at[12 + i])
            for i in range(R // 2)]
    fk_cp = pltpu.make_async_copy(fk_hbm, fk_v.at[:R], sems.at[7])
    tab_cp = pltpu.make_async_copy(tab_hbm, tab_v, sems.at[8])
    wqkv_cp = pltpu.make_async_copy(wqkv_hbm.bitcast(U32), wqkv_v, sems.at[10])
    wo_cp = [pltpu.make_async_copy(wo_hbm.bitcast(U32).at[:, pl.ds(t * C, C)],
                                   wo_v.at[t, :D // 2], sems.at[20 + t])
             for t in range(D // C)]
    for cp in small_cp + par_cp[0] + par_cp[1]:
        cp.start()
    for cp in small_cp + par_cp[0]:
        cp.wait()
    for cp in x_cp + [fk_cp, wqkv_cp] + wo_cp + [tab_cp]:
        cp.start()

    lane = lax.broadcasted_iota(jnp.int32, (8, C), 1)
    sub = lax.broadcasted_iota(jnp.int32, (8, C), 0)
    rho = _tap_offsets()

    zero = zero_s[0]

    spare = {n: n - 1 + 2 * zero for n in (2, R // 2 + 1, R + 1, 2 * R + 1)}

    def pin(ref, x):
        x = x if x.dtype == ref.dtype else pltpu.bitcast(x, ref.dtype)
        ref[spare[ref.shape[0]], :x.shape[0], :C] = x

    gate_v[0, :8] = jnp.zeros((8, C), F32)

    def gated(w):
        tail = w[-8:] | jnp.concatenate([pltpu.bitcast(gate_v[0, :8], U32)] * 2, axis=1)
        return _halves(jnp.concatenate([w[:-8], tail], axis=0))

    regions = []

    def region(fn, *args):
        regions.append(fn)
        pl.when(zero < len(regions))(lambda: fn(*args))

    def pacer(lag, ref):
        queue = []

        def pace(x):
            queue.append(x)
            if len(queue) > lag:
                pin(ref[0], queue.pop(0)[:8, :C])
            return x
        return pace

    dt_row = jnp.exp(ldt_ref[...].astype(F32).reshape(1, D)).astype(BF16).astype(F32)
    dk_row = dsk_ref[...].astype(F32).reshape(1, D)
    for b in range(D // C):
        cols = slice(b * C, (b + 1) * C)
        dt_v[cols, :] = jnp.broadcast_to(dt_row[:, cols], (C, C)).T
        dk_v[cols, :] = jnp.broadcast_to(dk_row[:, cols], (C, C)).T

    keys = [(s, p) for p in (16, 8, 4, 12, 2, 6, 10, 14, *range(1, 16, 2))
            for s in range(8) if p == 16 or p in rho[s]]

    pos = (lane - 7) & (C - 1)
    lower = {h: (pos & h) == 0 for h in (1, 2, 4)}
    upper = {h: (sub & h) == 0 for h in (1, 2)}

    def flip(x):
        x = pltpu.roll(x, 4, 0)
        x = lax.select(upper[2], pltpu.roll(x, 6, 0), pltpu.roll(x, 2, 0))
        return lax.select(upper[1], pltpu.roll(x, 7, 0), pltpu.roll(x, 1, 0))

    def discretise(i):
        a_re, a_im, b_re, b_im, c_re, c_im = [
            _halves(par_v[n, pl.ds(i * 8, 8), :]).astype(F32) for n in range(6)]
        rows = pl.ds(i * 16, 16)
        dt = dt_v[rows, :]
        mag, ph = jnp.exp(dt * a_re), dt * a_im
        w = _cmul((c_re, c_im), (dt * b_re, dt * b_im))
        tap0 = dk_v[rows, :] + jnp.sum(w[0], axis=1, keepdims=True)
        return mag * jnp.cos(ph), mag * jnp.sin(ph), *w, tap0

    def taps(i, a_re, a_im, w_re, w_im, tap0):
        rows = pl.ds(i * 8, 8)
        a = {1: (a_re, a_im)}
        for n in range(4):
            a[2 << n] = _csq(a[1 << n])
        right = [(jnp.ones((8, C), F32), jnp.zeros((8, C), F32)), (flip(a[16][0]), -flip(a[16][1]))]
        for j in range(2, 16):
            right.append(_csq(right[j // 2]) if j % 2 == 0 else
                         _cmul(right[j // 2], right[j // 2 + 1]))
        a[256] = [flip(t) for t in _csq((right[8][0], -right[8][1]))]
        left = {(0, 0): (w_re, w_im)}
        for s, p in keys:
            left[s, p] = (_cmul(left[s - 1, p], a[256]) if s else
                          _cmul(left[0, p & (p - 1)], a[p & -p]))
        res = _dot(*[jnp.concatenate([jnp.concatenate(v, axis=1) for v in vals], axis=0)
                     for vals in ([left[k] for k in keys], right)], _NT)
        part = {k: pltpu.roll(res[8 * n:8 * n + 8], k[0], 1, stride=1, stride_axis=0)
                for n, k in enumerate(keys)}
        memo = {}

        def merge(ps, s=0):
            if len(ps) == 1 or not any(ps):
                return part[s, ps[0]]
            if (ps, s) not in memo:
                h = len(ps) // 2
                memo[ps, s] = lax.select(lower[h], merge(ps[:h], s), merge(ps[h:], s + h))
            return memo[ps, s]

        t16 = merge((16,) * 8)
        t0 = jnp.where(pos < 8, pltpu.roll(t16, 9, 1), pltpu.roll(t16, 8, 1))
        t0 = jnp.where(pos == 0, tap0, t0)
        for s in range(8):
            part[s, 0] = t0
        for r in range(R):
            kt_v[r, rows, :] = merge(tuple(rho[s][r] for s in range(8)))

    def filters(lo, hi):
        for i in range(lo, hi):
            vals = discretise(i)
            for h in range(2):
                taps(2 * i + h, *[v[8 * h:8 * h + 8] for v in vals])

    with jax.named_scope("filter"):
        filters(0, HEAD)
        for cp in par_cp[1]:
            cp.wait()
        filters(HEAD, D // 16)

    def spectra(lo, hi, size, pace=lambda x: x):
        for row in range(lo, hi, size):
            rows = pl.ds(row, size)
            for r in range(8):
                ev, od = _split(lambda n: kt_v[n, rows, :], fk_v, r)
                kh_v[r, rows, :], kh_v[r + 8, rows, :] = pace(ev), od
                yield

    def keep(r, acc):
        for n, t in enumerate(_stats(acc)):
            st_v[r, n] = jnp.broadcast_to(t, (8, C))

    def load():
        for i in range(R // 2):
            acc = [None, None]
            for b in range(D // C):
                rows = pl.ds(b * C, C)
                wd = io_v[i, :, rows].T
                if b:
                    pin(fk_v, jnp.add(*acc[0]) + jnp.add(*acc[1]))
                for e, w in enumerate((wd << 16, wd & jnp.uint32(0xFFFF0000))):
                    x_v[2 * i + e, rows, :] = x = pltpu.bitcast(w, F32)
                    acc[e] = _sums(x, acc[e])
                yield
            for e in range(2):
                keep(2 * i + e, acc[e])

    hp = DH // 4

    def qkv_weights():
        row = lax.broadcasted_iota(jnp.int32, (C, C), 0)
        col = lax.broadcasted_iota(jnp.int32, (C, C), 1)
        dh = ((row >> 2) & 1) + 8 * ((row >> 4) & 1) + 2 * (row >> 5)
        pick = jnp.where(col == (2 * (row & 3) + ((row >> 3) & 1)) * DH + dh, 1.0, 0.0)
        for j in range(3 * D // C):
            w = _dot(pick, _halves(wqkv_v[:, pl.ds(j * C, C)]), _NT)
            for n in range(C // 32):
                part = w[32 * n:32 * n + 32]
                for i, a in enumerate(_lhs_terms(part[:, :D // 2], part[:, D // 2:])):
                    wt_v[j, i, pl.ds(8 * n, 8), :] = _pairs(a)
            yield

    def out_weights():
        rows = [g * C // 2 + h * hp + i for h in range(2) for g in range(D // C) for i in range(hp)]
        for j in range(D // C):
            for c in range(2):
                halves = [_halves(jnp.concatenate(
                    [wo_v[j, pl.ds(row, 8, stride=DH // 2), :] for row in rows[8 * k:8 * k + 8]],
                    axis=0)).T.astype(F32) for k in (c, c + 2)]
                for i, a in enumerate(_lhs_terms(*halves)):
                    wot_v[j, i, :, pl.ds(c * C, C)] = _words(a)
                yield

    for cp in x_cp + [fk_cp, wqkv_cp] + wo_cp:
        cp.wait()
    with jax.named_scope("load"):
        region(_run, (spectra(0, D // 2, CB, pacer(4, [io_v])), 32), (load(), 32),
               (qkv_weights(), 12))
    tab_cp.wait()

    def units(b):
        return [(pl.ds(i % 2 * 8, 8), pl.ds(b * CB + i // 2 * 8, 8)) for i in range(CB // 4)]

    def bins(ref, idx):
        return list(zip(*[jnp.split(ref[(*idx, pl.ds(c, C))], 8) for c in (0, C)]))

    def put(ref, idx, vals):
        for c, part in zip((0, C), zip(*vals)):
            ref[(*idx, pl.ds(c, C))] = jnp.concatenate(part)

    def filter_fft(b):
        for idx in units(b):
            put(kh_v, idx, _fft(bins(kh_v, idx)))
            yield

    def forward(b):
        rows = pl.ds(b * CB, CB)

        def normed(n):
            m, s = [jnp.concatenate([st_v[n, i]] * (CB // 8), axis=0) for i in range(2)]
            return (x_v[n, rows, :] - m) * s

        for r in range(8):
            s_v[r, rows, :], s_v[r + 8, rows, :] = _split(normed, tab_v, r)
            yield

    def inverse(b):
        rows = pl.ds(b * CB, CB)
        for r in range(8):
            ev = s_v[r, rows, :]
            od = _twiddle((s_v[r + 8, rows, C:], s_v[r + 8, rows, :C]), r, R)
            od = jnp.concatenate(od[::-1], axis=1)
            for n, z in ((r, ev + od), (r + 8, ev - od)):
                x_v[n, rows, :] += _dot(z, _halves(tab_v[R + n]))
            yield

    def mix(b):
        for idx in units(b):
            yf = [_cmul(u, k) for u, k in zip(_fft(bins(s_v, idx)), bins(kh_v, idx))]
            yield
            put(s_v, idx, _ifft(yf))

    def conv(first, k):
        fwd, mid, inv = [range(*span) for span in zip(PLAN[k], PLAN[k + 1])]
        nxt = range(PLAN[k + 1][1], PLAN[k + 2][1]) if first and k + 2 < len(PLAN) else ()
        _run((_chain(forward(b) for b in fwd), 8 * len(fwd)),
             (_chain(inverse(b) for b in inv), 8 * len(inv), 0.03, 1.03),
             *[(spectra(D // 2 + k * C, D // 2 + k * C + C, CB), 16, 0.031, 1.031)] * (first and k < 2),
             (_chain(mix(b) for b in mid), CB // 4 * len(mid)),
             (_chain(filter_fft(b) for b in nxt), CB // 4 * len(nxt)))

    groups, heads, chunks = R // 2, D // C, (1, 2, 0)
    n_qkv, n_att, n_term = NP * len(chunks), 44, D // 32

    def moments(p, stats):
        for r in range(2 * p, 2 * p + 2):
            acc = None
            for b in range(8):
                for row in range(b * 64, b * 64 + 64, 32):
                    acc = _sums(x_v[r + (zero if p > 1 else 0), pl.ds(row, 32), :], acc)
                pin(gate_v, jnp.add(*acc))
                stats[r] = acc if b < 7 else _stats(acc)
                yield

    def norm(p, stats):
        for i in range(n_term):
            cols = [(jnp.concatenate(
                [x_v[r - (zero if p else 0), pl.ds(h + 16 * i, 8, stride=2), :]
                 for h in (0, 1, D // 2, D // 2 + 1)],
                axis=0) - stats[r][0]) * stats[r][1] for r in (2 * p, 2 * p + 1)]
            for n, b in enumerate(_rhs_terms(*cols)):
                xt_v[p][zero + n, pl.ds(8 * i, 8), :] = wd = _pairs(b)
                pin(gate_v, wd)
            yield

    def qkv(g, t, p, pace):
        def emit(i, j, val):
            if t == 0:
                q_v[g % 2][p][j + zero, pl.ds(i * C // 2, C // 2), :] = val
                return
            rows = pl.ds((t - 1) * C + i * C // 2, C // 2)
            kv_v[g % 2][16 * j + 8 + p + zero, rows, :] = val
            if p:
                kv_v[g % 2][16 * j + p + zero, rows, :] = pltpu.roll(val, 1, 1)

        return _strassen(lambda i: pace(_dot(
            gated(wt_v[t * heads + g, i]), _halves(xt_v[p][i]))), emit)

    def attend(g, p):
        buf = kv_v[g % 2]
        for j in range(2):
            window = pl.ds(16 * j + p + 1, WIN)
            for dh in range(DH):
                t = q_v[g % 2][p][j, pl.ds(dh * 8, 8), :] * buf[window, pl.ds(dh * 8, 8), :]
                logits = t if dh == 0 else logits + t
                if dh % 2:
                    w = dh // 2 % 2 * 4
                    pin(gate_v, logits[w:w + 4].reshape(32, C))
                    yield
            if p < WIN - 1:
                logits = jnp.concatenate(
                    [jnp.where(lane == 0, -1e9 / SCALE, logits[:WIN - 1 - p]), logits[WIN - 1 - p:]])
            ex = jnp.exp2((logits - _fold(jnp.maximum, logits)) * (SCALE * float(np.log2(np.e))))
            pr = ex * (1.0 / _fold(jnp.add, ex))
            yield from range(4)
            for i in range(hp):
                for h in range(2):
                    for e in range(2):
                        rows = pl.ds(C + (2 * (h * hp + i) + e) * 8, 8)
                        o = _fold(jnp.add, pr * buf[window, rows, :])
                        held_v[j + zero, i, pl.ds(16 * h + 8 * e, 8), :] = o
                        pin(gate_v, o)
                    yield
        for i in range(hp):
            cols = [held_v[j, i] for j in range(2)]
            for t, b in enumerate(_rhs_terms(*cols)):
                ot_v[p][zero + t, pl.ds((g * hp + i) * 8, 8), :] = wd = _pairs(b)
                if t in (0, 5):
                    pin(gate_v, wd)
            yield

    sums = {}

    def project(last, t, p, pace):
        def emit(i, j, val):
            r, rows = 2 * p + j, pl.ds(t * C + i * C // 2, C // 2)
            x = x_v[r, rows, :] + val
            if not last:
                x_v[r, rows, :] = x
                sums[r] = _sums(x, sums.get(r))
            elif j:
                y_v[p % 2][zero, rows, :] = _pairs(jnp.concatenate([sums.pop(r - 1), x], axis=0))
            else:
                sums[r] = x

        return _strassen(lambda i: pace(_dot(gated(wot_v[t, i]), _halves(ot_v[p][i]))), emit)

    def out_copy(n):
        return pltpu.make_async_copy(io_v.at[n], out_w.at[:, n, :], sems.at[12 + n])

    sent = []

    def send(p):
        for n in range(len(sent), p):
            sent.append(n)
            out_copy(n).start()

    def finish(last, p):
        for b in range(D // C):
            if last:
                io_v[p, :, pl.ds(b * C, C)] = y_v[p % 2][0, pl.ds(b * C, C), :].T
            elif b % 2 == 0:
                keep(2 * p + b // 2, sums[2 * p + b // 2])
            yield

    def first_heads():
        pace, stats = pacer(LAG, [x_v]), {}
        _run(*[(inverse(b), 8) for b in range(PLAN[-1][2], D // CB)],
             (moments(0, stats), 16, 0.3, 0.55), (moments(1, stats), 16, 0.6, 1.0),
             (norm(0, stats), n_term, 0.6, 1.0))
        for p in range(groups):
            _run((_chain(qkv(0, n, p, pace) for n in chunks), n_qkv),
                 *[(norm(p + 1, stats), n_term, 0.0, 0.85)] * (p + 1 < groups),
                 *[(moments(p + 2, stats), 16)] * (p + 2 < groups))

    def attends(g, reading):
        todo = [(g - 1, p) for p in range(EARLY[g - 1], groups)] + [(g, p) for p in range(EARLY[g])]

        def steps():
            for h, p in todo:
                reading[0] = kv_v[h % 2]
                yield from attend(h, p)

        return steps(), n_att * len(todo)

    def projections(last, pace):
        for p in range(groups):
            for t in range(D // C):
                if last and t == 2 and p in (groups - 4, groups - 2):
                    send(p)
                yield from project(last, t, p, pace)

    def next_heads(g):
        reading = [None]
        pace = pacer(LAG, reading)
        _run((_chain(qkv(g, t, p, pace) for t in chunks for p in range(groups)), n_qkv * groups),
             attends(g, reading))

    def output(last):
        reading = [None]
        _run((projections(last, pacer(LAG, reading)), groups * NP * D // C),
             (*attends(heads, reading), 0.0, 0.85),
             *[(finish(last, p - 1), D // C, (p + 0.2) / groups, (p + 0.5) / groups)
               for p in range(1, groups)])
        if last:
            send(groups - 1)
        _run((finish(last, groups - 1), D // C, 0.0, 0.5), *[(forward(0), 8)] * (not last))

    _run((forward(0), 8), (filter_fft(0), CB // 4), (out_weights(), 8))
    for last in (False, True):
        with jax.named_scope("conv"):
            for k in range(len(PLAN) - 1):
                region(conv, not last, k)
        with jax.named_scope("kv"):
            region(first_heads)
        with jax.named_scope("mid"):
            for g in range(1, heads):
                region(next_heads, g)
        with jax.named_scope("attn"):
            region(output, last)

    send(groups)
    for p in range(groups):
        out_copy(p).wait()


@jax.jit
def pallas_interleave_layers__ssm_conv_s4__sliding_local_dilated__prompt_kernel(
    A_u: jax.Array,
    A_A_re: jax.Array,
    A_A_im: jax.Array,
    A_B_re: jax.Array,
    A_B_im: jax.Array,
    A_C_re: jax.Array,
    A_C_im: jax.Array,
    A_log_dt: jax.Array,
    A_Dskip: jax.Array,
    B_x: jax.Array,
    B_wqkv: jax.Array,
    B_wo: jax.Array,
):
    del B_x
    assert A_u.shape == (1, L, D) and A_A_re.shape == (D, N) and A_A_re.dtype == BF16
    hbm = pl.BlockSpec(memory_space=pl.ANY)
    out = pl.pallas_call(
        _kernel,
        in_specs=[hbm] * 14,
        out_specs=hbm,
        out_shape=jax.ShapeDtypeStruct((C, R, D), BF16),
        scratch_shapes=[
            pltpu.VMEM((R // 2 + 1, C, D), U32),
            pltpu.VMEM((6, D // 2, N), U32),
            pltpu.VMEM((D // 2, 3 * D), U32),
            pltpu.VMEM((D // C, D // 2 + 8, C), U32),
            pltpu.VMEM((2 * R, C, C), U32),
            pltpu.VMEM((R + 1, C, C), U32),
            pltpu.VMEM((D, C), F32),
            pltpu.VMEM((D, C), F32),
            pltpu.VMEM((3 * D // C, NP, C // 4, D // 2), U32),
            pltpu.VMEM((D // C, NP, C // 4, D // 2), U32),
            pltpu.VMEM((R + 1, D + 8, C), F32),
            pltpu.VMEM((R, 2, 8, C), F32),
            pltpu.VMEM((R, D, C), F32),
            pltpu.VMEM((R, D, 2 * C), F32),
            *[[pltpu.VMEM((NP, D // 4, C), U32)] * (R // 2)] * 2,
            pltpu.VMEM((2, DH // 4, 32, C), F32),
            pltpu.VMEM((2, 32, C), F32),
            pltpu.VMEM((R, D, 2 * C), F32),
            [[pltpu.VMEM((2, C, C), F32)] * (R // 2)] * 2,
            [pltpu.VMEM((2 * R + 1, 2 * C, C), F32)] * 2,
            [pltpu.VMEM((1, D, C), U32)] * 2,
            *[pltpu.VMEM((D,), BF16)] * 2,
            pltpu.SMEM((1,), jnp.int32),
            pltpu.SemaphoreType.DMA((24,)),
        ],
        compiler_params=pltpu.CompilerParams(vmem_limit_bytes=100 * 1024 * 1024),
    )(A_u.reshape(C, R, D), A_A_re, A_A_im, A_B_re, A_B_im, A_C_re, A_C_im,
      A_log_dt, A_Dskip, B_wqkv, B_wo, *_dft_tables(),
      np.zeros((1,), np.int32))
    return out.reshape(1, L, D)
```

```python
import ml_dtypes
import numpy as np

import jax
import jax.numpy as jnp
from jax import lax
import jax.experimental.pallas as pl
import jax.experimental.pallas.tpu as pltpu

L, D, N = 2048, 512, 128
R, C = 16, 128
DH, WIN = 16, 8
CB = 64
NP = 7
PLAN = ((1, 0, 0), (3, 1, 0), (6, 3, 0), (8, 6, 2), (8, 8, 6))
LAG = 4
EARLY = (0, 0, 1, 2, 0)
HEAD = 3
EPS, SCALE = 1e-5, DH ** -0.5
F32, BF16, U32 = jnp.float32, jnp.bfloat16, jnp.uint32
_NT = (((1,), (1,)), ((), ()))


def _host_words(a):
    h = np.ascontiguousarray(a).astype(ml_dtypes.bfloat16).view(np.uint16).astype(np.uint32)
    return h[..., 0::2, :] | (h[..., 1::2, :] << 16)


def _dft_tables():
    t = R * np.arange(C)[None, :, None] + np.arange(R)[:, None, None]
    ang = 2.0 * np.pi * (np.arange(C)[None, None, :] + 0.5) * t / (2 * L)
    fwd = np.concatenate([np.cos(ang), -np.sin(ang)], axis=-1)
    p = (np.arange(C) - 7) % C
    fwd_k = fwd[:, 16 * (p % 8) + p // 8, :] / L
    inv = fwd.transpose(0, 2, 1)
    fwd, fwd_k = [np.concatenate([a[..., :C], a[..., C:]], axis=1) for a in (fwd, fwd_k)]
    return _host_words(np.concatenate([fwd, inv])), _host_words(fwd_k)


def _tap_offsets():
    l = np.arange(L)
    lr = l.astype(np.float32).astype(ml_dtypes.bfloat16).astype(np.float32).astype(np.int64)
    rho = (lr - (l // R) * R).reshape(8, 16, R)
    assert (rho == rho[:, :1]).all()
    return rho[:, 0].tolist()


def _cmul(a, b):
    return a[0] * b[0] - a[1] * b[1], a[0] * b[1] + a[1] * b[0]


def _csq(a):
    t = a[0] * a[1]
    return a[0] * a[0] - a[1] * a[1], t + t


def _twiddle(a, k, n):
    if k == 0:
        return a
    if 4 * k == n:
        return a[1], -a[0]
    h = float(np.sqrt(0.5))
    if 8 * k == n:
        return (a[0] + a[1]) * h, (a[1] - a[0]) * h
    if 8 * k == 3 * n:
        return (a[1] - a[0]) * h, (a[0] + a[1]) * (-h)
    w = (float(np.cos(2 * np.pi * k / n)), float(-np.sin(2 * np.pi * k / n)))
    return _cmul(a, w)


def _fft(x):
    n = len(x)
    if n == 1:
        return x
    if n == 2:
        return [(x[0][0] + x[1][0], x[0][1] + x[1][1]), (x[0][0] - x[1][0], x[0][1] - x[1][1])]
    e, o1, o3 = _fft(x[0::2]), _fft(x[1::4]), _fft(x[3::4])
    out = [None] * n
    q = n // 4
    for k in range(q):
        a, b = _twiddle(o1[k], k, n), _twiddle(o3[k], 3 * k, n)
        s = (a[0] + b[0], a[1] + b[1])
        d = (a[0] - b[0], a[1] - b[1])
        out[k] = (e[k][0] + s[0], e[k][1] + s[1])
        out[k + 2 * q] = (e[k][0] - s[0], e[k][1] - s[1])
        out[k + q] = (e[k + q][0] + d[1], e[k + q][1] - d[0])
        out[k + 3 * q] = (e[k + q][0] - d[1], e[k + q][1] + d[0])
    return out


def _ifft(x):
    return [(b, a) for a, b in _fft([(b, a) for a, b in x])]


def _fold(op, x):
    while x.shape[0] > 1:
        x = op(x[:x.shape[0] // 2], x[x.shape[0] // 2:])
    return x[0]


def _sums(x, acc=None):
    x = x.reshape(-1, 8, C)
    new = _fold(jnp.add, x), _fold(jnp.add, x * x)
    return new if acc is None else (acc[0] + new[0], acc[1] + new[1])


def _stats(acc):
    m, sq = [jnp.sum(t, axis=0, keepdims=True) * (1.0 / D) for t in acc]
    return m, lax.rsqrt(jnp.maximum(sq - m * m, 0.0) + EPS)


def _words(x):
    return pltpu.bitcast(x.astype(BF16), U32)


def _pairs(x):
    b = pltpu.bitcast(x, U32) + jnp.uint32(0x8000)
    return (b[x.shape[0] // 2:] & jnp.uint32(0xFFFF0000)) | (b[:x.shape[0] // 2] >> 16)


def _halves(w):
    return pltpu.bitcast(w, BF16)


def _dot(a, b, dims=(((1,), (0,)), ((), ()))):
    return lax.dot_general(a.astype(BF16), b.astype(BF16), dims, preferred_element_type=F32)


def _split(src, table, r):
    lo, hi = [_dot(src(n), _halves(jnp.concatenate(
        [table[n, :C // 2], table[n, C // 2:]], axis=1))) for n in (r, r + 8)]
    d = lo - hi
    return lo + hi, jnp.concatenate(_twiddle((d[:, :C], d[:, C:]), r, R), axis=1)


def _run(*jobs):
    order = []
    for k, (_, n, *span) in enumerate(jobs):
        lo, hi = span or (0.0, 1.0)
        order += [(lo + (hi - lo) * i / n, k) for i in range(n)]
    for _, k in sorted(order):
        next(jobs[k][0])
    for job in jobs:
        for _ in job[0]:
            pass


def _chain(gens):
    for g in gens:
        yield from g


def _lhs_terms(left, right):
    m = left.shape[0] // 2
    a11, a12, a21, a22 = left[:m], right[:m], left[m:], right[m:]
    return a11 + a22, a21 + a22, a22, a12 - a22, a21 - a11, a11, a11 + a12


def _rhs_terms(left, right):
    k = left.shape[0] // 2
    b11, b12, b21, b22 = left[:k], right[:k], left[k:], right[k:]
    return b11 + b22, b11, b21 - b11, b21 + b22, b11 + b12, b12 - b22, b22


def _strassen(product, emit):
    m1 = product(0)
    yield
    m2 = product(1)
    yield
    m4 = product(2)
    yield
    c11, c22 = m1 + m4, m1 - m2
    emit(1, 0, m2 + m4)
    c22 += product(4)
    yield
    m3 = product(5)
    yield
    emit(1, 1, c22 + m3)
    c11 += product(3)
    yield
    m5 = product(6)
    yield
    emit(0, 0, c11 - m5)
    emit(0, 1, m3 + m5)


def _kernel(x_hbm, are_hbm, aim_hbm, bre_hbm, bim_hbm, cre_hbm, cim_hbm, ldt_hbm, dsk_hbm,
            wqkv_hbm, wo_hbm, tab_hbm, fk_hbm, zero_hbm, out_hbm,
            io_v, par_v, wqkv_v, wo_v, tab_v, fk_v, dt_v, dk_v, wt_v, wot_v,
            x_v, st_v, kt_v, kh_v, xt_v, ot_v, held_v, gate_v, s_v,
            q_v, kv_v, y_v, ldt_ref, dsk_ref, zero_s, sems):
    srcs = (are_hbm, aim_hbm, bre_hbm, bim_hbm, cre_hbm, cim_hbm)
    par_cp = [[pltpu.make_async_copy(s.bitcast(U32).at[rows], par_v.at[i, rows], sems.at[k])
               for i, s in enumerate(srcs)]
              for k, rows in enumerate((pl.ds(0, HEAD * 8), pl.ds(HEAD * 8, D // 2 - HEAD * 8)))]
    small_cp = [pltpu.make_async_copy(*pair, sems.at[2 + i]) for i, pair in enumerate(
        ((ldt_hbm, ldt_ref), (dsk_hbm, dsk_ref), (zero_hbm, zero_s)))]
    x_w, out_w = x_hbm.bitcast(U32), out_hbm.bitcast(U32)
    x_cp = [pltpu.make_async_copy(x_w.at[:, i, :], io_v.at[i], sems.at[12 + i])
            for i in range(R // 2)]
    fk_cp = pltpu.make_async_copy(fk_hbm, fk_v.at[:R], sems.at[7])
    tab_cp = pltpu.make_async_copy(tab_hbm, tab_v, sems.at[8])
    wqkv_cp = pltpu.make_async_copy(wqkv_hbm.bitcast(U32), wqkv_v, sems.at[10])
    wo_cp = [pltpu.make_async_copy(wo_hbm.bitcast(U32).at[:, pl.ds(t * C, C)],
                                   wo_v.at[t, :D // 2], sems.at[20 + t])
             for t in range(D // C)]
    for cp in small_cp + par_cp[0] + par_cp[1]:
        cp.start()
    for cp in small_cp + par_cp[0]:
        cp.wait()
    for cp in x_cp + [fk_cp, wqkv_cp] + wo_cp + [tab_cp]:
        cp.start()

    lane = lax.broadcasted_iota(jnp.int32, (8, C), 1)
    sub = lax.broadcasted_iota(jnp.int32, (8, C), 0)
    rho = _tap_offsets()

    zero = zero_s[0]

    spare = {n: n - 1 + 2 * zero for n in (2, R // 2 + 1, R + 1, 2 * R + 1)}

    def pin(ref, x):
        x = x if x.dtype == ref.dtype else pltpu.bitcast(x, ref.dtype)
        ref[spare[ref.shape[0]], :x.shape[0], :C] = x

    gate_v[0, :8] = jnp.zeros((8, C), F32)

    def gated(w):
        tail = w[-8:] | jnp.concatenate([pltpu.bitcast(gate_v[0, :8], U32)] * 2, axis=1)
        return _halves(jnp.concatenate([w[:-8], tail], axis=0))

    regions = []

    def region(fn, *args):
        regions.append(fn)
        pl.when(zero < len(regions))(lambda: fn(*args))

    def pacer(lag, ref):
        queue = []

        def pace(x):
            queue.append(x)
            if len(queue) > lag:
                pin(ref[0], queue.pop(0)[:8, :C])
            return x
        return pace

    dt_row = jnp.exp(ldt_ref[...].astype(F32).reshape(1, D)).astype(BF16).astype(F32)
    dk_row = dsk_ref[...].astype(F32).reshape(1, D)
    for b in range(D // C):
        cols = slice(b * C, (b + 1) * C)
        dt_v[cols, :] = jnp.broadcast_to(dt_row[:, cols], (C, C)).T
        dk_v[cols, :] = jnp.broadcast_to(dk_row[:, cols], (C, C)).T

    keys = [(s, p) for p in (16, 8, 4, 12, 2, 6, 10, 14, *range(1, 16, 2))
            for s in range(8) if p == 16 or p in rho[s]]

    pos = (lane - 7) & (C - 1)
    lower = {h: (pos & h) == 0 for h in (1, 2, 4)}
    upper = {h: (sub & h) == 0 for h in (1, 2)}

    def flip(x):
        x = pltpu.roll(x, 4, 0)
        x = lax.select(upper[2], pltpu.roll(x, 6, 0), pltpu.roll(x, 2, 0))
        return lax.select(upper[1], pltpu.roll(x, 7, 0), pltpu.roll(x, 1, 0))

    def discretise(i):
        a_re, a_im, b_re, b_im, c_re, c_im = [
            _halves(par_v[n, pl.ds(i * 8, 8), :]).astype(F32) for n in range(6)]
        rows = pl.ds(i * 16, 16)
        dt = dt_v[rows, :]
        mag, ph = jnp.exp(dt * a_re), dt * a_im
        w = _cmul((c_re, c_im), (dt * b_re, dt * b_im))
        tap0 = dk_v[rows, :] + jnp.sum(w[0], axis=1, keepdims=True)
        return mag * jnp.cos(ph), mag * jnp.sin(ph), *w, tap0

    def taps(i, a_re, a_im, w_re, w_im, tap0):
        rows = pl.ds(i * 8, 8)
        a = {1: (a_re, a_im)}
        for n in range(4):
            a[2 << n] = _csq(a[1 << n])
        right = [(jnp.ones((8, C), F32), jnp.zeros((8, C), F32)), (flip(a[16][0]), -flip(a[16][1]))]
        for j in range(2, 16):
            right.append(_csq(right[j // 2]) if j % 2 == 0 else
                         _cmul(right[j // 2], right[j // 2 + 1]))
        a[256] = [flip(t) for t in _csq((right[8][0], -right[8][1]))]
        left = {(0, 0): (w_re, w_im)}
        for s, p in keys:
            left[s, p] = (_cmul(left[s - 1, p], a[256]) if s else
                          _cmul(left[0, p & (p - 1)], a[p & -p]))
        res = _dot(*[jnp.concatenate([jnp.concatenate(v, axis=1) for v in vals], axis=0)
                     for vals in ([left[k] for k in keys], right)], _NT)
        part = {k: pltpu.roll(res[8 * n:8 * n + 8], k[0], 1, stride=1, stride_axis=0)
                for n, k in enumerate(keys)}
        memo = {}

        def merge(ps, s=0):
            if len(ps) == 1 or not any(ps):
                return part[s, ps[0]]
            if (ps, s) not in memo:
                h = len(ps) // 2
                memo[ps, s] = lax.select(lower[h], merge(ps[:h], s), merge(ps[h:], s + h))
            return memo[ps, s]

        t16 = merge((16,) * 8)
        t0 = jnp.where(pos < 8, pltpu.roll(t16, 9, 1), pltpu.roll(t16, 8, 1))
        t0 = jnp.where(pos == 0, tap0, t0)
        for s in range(8):
            part[s, 0] = t0
        for r in range(R):
            kt_v[r, rows, :] = merge(tuple(rho[s][r] for s in range(8)))

    def filters(lo, hi):
        for i in range(lo, hi):
            vals = discretise(i)
            for h in range(2):
                taps(2 * i + h, *[v[8 * h:8 * h + 8] for v in vals])

    with jax.named_scope("filter"):
        filters(0, HEAD)
        for cp in par_cp[1]:
            cp.wait()
        filters(HEAD, D // 16)

    def spectra(lo, hi, size, pace=lambda x: x):
        for row in range(lo, hi, size):
            rows = pl.ds(row, size)
            for r in range(8):
                ev, od = _split(lambda n: kt_v[n, rows, :], fk_v, r)
                kh_v[r, rows, :], kh_v[r + 8, rows, :] = pace(ev), od
                yield

    def keep(r, acc):
        for n, t in enumerate(_stats(acc)):
            st_v[r, n] = jnp.broadcast_to(t, (8, C))

    def load():
        for i in range(R // 2):
            acc = [None, None]
            for b in range(D // C):
                rows = pl.ds(b * C, C)
                wd = io_v[i, :, rows].T
                if b:
                    pin(fk_v, jnp.add(*acc[0]) + jnp.add(*acc[1]))
                for e, w in enumerate((wd << 16, wd & jnp.uint32(0xFFFF0000))):
                    x_v[2 * i + e, rows, :] = x = pltpu.bitcast(w, F32)
                    acc[e] = _sums(x, acc[e])
                yield
            for e in range(2):
                keep(2 * i + e, acc[e])

    hp = DH // 4

    def qkv_weights():
        row = lax.broadcasted_iota(jnp.int32, (C, C), 0)
        col = lax.broadcasted_iota(jnp.int32, (C, C), 1)
        dh = ((row >> 2) & 1) + 8 * ((row >> 4) & 1) + 2 * (row >> 5)
        pick = jnp.where(col == (2 * (row & 3) + ((row >> 3) & 1)) * DH + dh, 1.0, 0.0)
        for j in range(3 * D // C):
            w = _dot(pick, _halves(wqkv_v[:, pl.ds(j * C, C)]), _NT)
            for n in range(C // 32):
                part = w[32 * n:32 * n + 32]
                for i, a in enumerate(_lhs_terms(part[:, :D // 2], part[:, D // 2:])):
                    wt_v[j, i, pl.ds(8 * n, 8), :] = _pairs(a)
            yield

    def out_weights():
        rows = [g * C // 2 + h * hp + i for h in range(2) for g in range(D // C) for i in range(hp)]
        for j in range(D // C):
            for c in range(2):
                halves = [_halves(jnp.concatenate(
                    [wo_v[j, pl.ds(row, 8, stride=DH // 2), :] for row in rows[8 * k:8 * k + 8]],
                    axis=0)).T.astype(F32) for k in (c, c + 2)]
                for i, a in enumerate(_lhs_terms(*halves)):
                    wot_v[j, i, :, pl.ds(c * C, C)] = _words(a)
                yield

    for cp in x_cp + [fk_cp, wqkv_cp] + wo_cp:
        cp.wait()
    with jax.named_scope("load"):
        region(_run, (spectra(0, D // 2, CB, pacer(4, [io_v])), 32), (load(), 32),
               (qkv_weights(), 12))
    tab_cp.wait()

    def units(b):
        return [(pl.ds(i % 2 * 8, 8), pl.ds(b * CB + i // 2 * 8, 8)) for i in range(CB // 4)]

    def bins(ref, idx):
        return list(zip(*[jnp.split(ref[(*idx, pl.ds(c, C))], 8) for c in (0, C)]))

    def put(ref, idx, vals):
        for c, part in zip((0, C), zip(*vals)):
            ref[(*idx, pl.ds(c, C))] = jnp.concatenate(part)

    def filter_fft(b):
        for idx in units(b):
            put(kh_v, idx, _fft(bins(kh_v, idx)))
            yield

    def forward(b):
        rows = pl.ds(b * CB, CB)

        def normed(n):
            m, s = [jnp.concatenate([st_v[n, i]] * (CB // 8), axis=0) for i in range(2)]
            return (x_v[n, rows, :] - m) * s

        for r in range(8):
            s_v[r, rows, :], s_v[r + 8, rows, :] = _split(normed, tab_v, r)
            yield

    def inverse(b):
        rows = pl.ds(b * CB, CB)
        for r in range(8):
            ev = s_v[r, rows, :]
            od = _twiddle((s_v[r + 8, rows, C:], s_v[r + 8, rows, :C]), r, R)
            od = jnp.concatenate(od[::-1], axis=1)
            for n, z in ((r, ev + od), (r + 8, ev - od)):
                x_v[n, rows, :] += _dot(z, _halves(tab_v[R + n]))
            yield

    def mix(b):
        for idx in units(b):
            yf = [_cmul(u, k) for u, k in zip(_fft(bins(s_v, idx)), bins(kh_v, idx))]
            yield
            put(s_v, idx, _ifft(yf))

    def conv(first, k):
        fwd, mid, inv = [range(*span) for span in zip(PLAN[k], PLAN[k + 1])]
        nxt = range(PLAN[k + 1][1], PLAN[k + 2][1]) if first and k + 2 < len(PLAN) else ()
        _run((_chain(forward(b) for b in fwd), 8 * len(fwd)),
             (_chain(inverse(b) for b in inv), 8 * len(inv), 0.03, 1.03),
             *[(spectra(D // 2 + k * C, D // 2 + k * C + C, CB), 16, 0.031, 1.031)] * (first and k < 2),
             (_chain(mix(b) for b in mid), CB // 4 * len(mid)),
             (_chain(filter_fft(b) for b in nxt), CB // 4 * len(nxt)))

    groups, heads, chunks = R // 2, D // C, (1, 2, 0)
    n_qkv, n_att, n_term = NP * len(chunks), 44, D // 32

    def moments(p, stats):
        for r in range(2 * p, 2 * p + 2):
            acc = None
            for b in range(8):
                for row in range(b * 64, b * 64 + 64, 32):
                    acc = _sums(x_v[r + (zero if p > 1 else 0), pl.ds(row, 32), :], acc)
                pin(gate_v, jnp.add(*acc))
                stats[r] = acc if b < 7 else _stats(acc)
                yield

    def norm(p, stats):
        for i in range(n_term):
            cols = [(jnp.concatenate(
                [x_v[r - (zero if p else 0), pl.ds(h + 16 * i, 8, stride=2), :]
                 for h in (0, 1, D // 2, D // 2 + 1)],
                axis=0) - stats[r][0]) * stats[r][1] for r in (2 * p, 2 * p + 1)]
            for n, b in enumerate(_rhs_terms(*cols)):
                xt_v[p][zero + n, pl.ds(8 * i, 8), :] = wd = _pairs(b)
                pin(gate_v, wd)
            yield

    def qkv(g, t, p, pace):
        def emit(i, j, val):
            if t == 0:
                q_v[g % 2][p][j + zero, pl.ds(i * C // 2, C // 2), :] = val
                return
            rows = pl.ds((t - 1) * C + i * C // 2, C // 2)
            kv_v[g % 2][16 * j + 8 + p + zero, rows, :] = val
            if p:
                kv_v[g % 2][16 * j + p + zero, rows, :] = pltpu.roll(val, 1, 1)

        return _strassen(lambda i: pace(_dot(
            gated(wt_v[t * heads + g, i]), _halves(xt_v[p][i]))), emit)

    def attend(g, p):
        buf = kv_v[g % 2]
        for j in range(2):
            window = pl.ds(16 * j + p + 1, WIN)
            for dh in range(DH):
                t = q_v[g % 2][p][j, pl.ds(dh * 8, 8), :] * buf[window, pl.ds(dh * 8, 8), :]
                logits = t if dh == 0 else logits + t
                if dh % 2:
                    w = dh // 2 % 2 * 4
                    pin(gate_v, logits[w:w + 4].reshape(32, C))
                    yield
            if p < WIN - 1:
                logits = jnp.concatenate(
                    [jnp.where(lane == 0, -1e9 / SCALE, logits[:WIN - 1 - p]), logits[WIN - 1 - p:]])
            ex = jnp.exp2((logits - _fold(jnp.maximum, logits)) * (SCALE * float(np.log2(np.e))))
            pr = ex * (1.0 / _fold(jnp.add, ex))
            yield from range(4)
            for i in range(hp):
                for h in range(2):
                    row = C + (h * hp + i) * 16
                    o = jnp.concatenate([_fold(jnp.add, pr * buf[window, pl.ds(row + e, 8), :])
                                         for e in (0, 8)])
                    held_v[j + zero, i, pl.ds(16 * h, 16), :] = o
                    pin(gate_v, o)
                    yield
        for i in range(hp):
            cols = [held_v[j, i] for j in range(2)]
            for t, b in enumerate(_rhs_terms(*cols)):
                ot_v[p][zero + t, pl.ds((g * hp + i) * 8, 8), :] = wd = _pairs(b)
                if t in (0, 5):
                    pin(gate_v, wd)
            yield

    sums = {}

    def project(last, t, p, pace):
        def emit(i, j, val):
            r, rows = 2 * p + j, pl.ds(t * C + i * C // 2, C // 2)
            x = x_v[r, rows, :] + val
            if not last:
                x_v[r, rows, :] = x
                sums[r] = _sums(x, sums.get(r))
            elif j:
                y_v[p % 2][zero, rows, :] = _pairs(jnp.concatenate([sums.pop(r - 1), x], axis=0))
            else:
                sums[r] = x

        return _strassen(lambda i: pace(_dot(gated(wot_v[t, i]), _halves(ot_v[p][i]))), emit)

    def out_copy(n):
        return pltpu.make_async_copy(io_v.at[n], out_w.at[:, n, :], sems.at[12 + n])

    sent = []

    def send(p):
        for n in range(len(sent), p):
            sent.append(n)
            out_copy(n).start()

    def finish(last, p):
        for b in range(D // C):
            if last:
                io_v[p, :, pl.ds(b * C, C)] = y_v[p % 2][0, pl.ds(b * C, C), :].T
            elif b % 2 == 0:
                keep(2 * p + b // 2, sums[2 * p + b // 2])
            yield

    def first_heads():
        pace, stats = pacer(LAG, [x_v]), {}
        _run(*[(inverse(b), 8) for b in range(PLAN[-1][2], D // CB)],
             (moments(0, stats), 16, 0.3, 0.55), (moments(1, stats), 16, 0.6, 1.0),
             (norm(0, stats), n_term, 0.6, 1.0))
        for p in range(groups):
            _run((_chain(qkv(0, n, p, pace) for n in chunks), n_qkv),
                 *[(norm(p + 1, stats), n_term, 0.0, 0.85)] * (p + 1 < groups),
                 *[(moments(p + 2, stats), 16)] * (p + 2 < groups))

    def attends(g, reading):
        todo = [(g - 1, p) for p in range(EARLY[g - 1], groups)] + [(g, p) for p in range(EARLY[g])]

        def steps():
            for h, p in todo:
                reading[0] = kv_v[h % 2]
                yield from attend(h, p)

        return steps(), n_att * len(todo)

    def projections(last, pace):
        for p in range(groups):
            for t in range(D // C):
                if last and t == 2 and p in (groups - 4, groups - 2):
                    send(p)
                yield from project(last, t, p, pace)

    def next_heads(g):
        reading = [None]
        pace = pacer(LAG, reading)
        _run((_chain(qkv(g, t, p, pace) for t in chunks for p in range(groups)), n_qkv * groups),
             attends(g, reading))

    def output(last):
        reading = [None]
        _run((projections(last, pacer(LAG, reading)), groups * NP * D // C),
             (*attends(heads, reading), 0.0, 0.85),
             *[(finish(last, p - 1), D // C, (p + 0.2) / groups, (p + 0.5) / groups)
               for p in range(1, groups)])
        if last:
            send(groups - 1)
        _run((finish(last, groups - 1), D // C, 0.0, 0.5), *[(forward(0), 8)] * (not last))

    _run((forward(0), 8), (filter_fft(0), CB // 4), (out_weights(), 8))
    for last in (False, True):
        with jax.named_scope("conv"):
            for k in range(len(PLAN) - 1):
                region(conv, not last, k)
        with jax.named_scope("kv"):
            region(first_heads)
        with jax.named_scope("mid"):
            for g in range(1, heads):
                region(next_heads, g)
        with jax.named_scope("attn"):
            region(output, last)

    send(groups)
    for p in range(groups):
        out_copy(p).wait()


@jax.jit
def pallas_interleave_layers__ssm_conv_s4__sliding_local_dilated__prompt_kernel(
    A_u: jax.Array,
    A_A_re: jax.Array,
    A_A_im: jax.Array,
    A_B_re: jax.Array,
    A_B_im: jax.Array,
    A_C_re: jax.Array,
    A_C_im: jax.Array,
    A_log_dt: jax.Array,
    A_Dskip: jax.Array,
    B_x: jax.Array,
    B_wqkv: jax.Array,
    B_wo: jax.Array,
):
    del B_x
    assert A_u.shape == (1, L, D) and A_A_re.shape == (D, N) and A_A_re.dtype == BF16
    hbm = pl.BlockSpec(memory_space=pl.ANY)
    out = pl.pallas_call(
        _kernel,
        in_specs=[hbm] * 14,
        out_specs=hbm,
        out_shape=jax.ShapeDtypeStruct((C, R, D), BF16),
        scratch_shapes=[
            pltpu.VMEM((R // 2 + 1, C, D), U32),
            pltpu.VMEM((6, D // 2, N), U32),
            pltpu.VMEM((D // 2, 3 * D), U32),
            pltpu.VMEM((D // C, D // 2 + 8, C), U32),
            pltpu.VMEM((2 * R, C, C), U32),
            pltpu.VMEM((R + 1, C, C), U32),
            pltpu.VMEM((D, C), F32),
            pltpu.VMEM((D, C), F32),
            pltpu.VMEM((3 * D // C, NP, C // 4, D // 2), U32),
            pltpu.VMEM((D // C, NP, C // 4, D // 2), U32),
            pltpu.VMEM((R + 1, D + 8, C), F32),
            pltpu.VMEM((R, 2, 8, C), F32),
            pltpu.VMEM((R, D, C), F32),
            pltpu.VMEM((R, D, 2 * C), F32),
            *[[pltpu.VMEM((NP, D // 4, C), U32)] * (R // 2)] * 2,
            pltpu.VMEM((2, DH // 4, 32, C), F32),
            pltpu.VMEM((2, 32, C), F32),
            pltpu.VMEM((R, D, 2 * C), F32),
            [[pltpu.VMEM((2, C, C), F32)] * (R // 2)] * 2,
            [pltpu.VMEM((2 * R + 1, 2 * C, C), F32)] * 2,
            [pltpu.VMEM((1, D, C), U32)] * 2,
            *[pltpu.VMEM((D,), BF16)] * 2,
            pltpu.SMEM((1,), jnp.int32),
            pltpu.SemaphoreType.DMA((24,)),
        ],
        compiler_params=pltpu.CompilerParams(vmem_limit_bytes=100 * 1024 * 1024),
    )(A_u.reshape(C, R, D), A_A_re, A_A_im, A_B_re, A_B_im, A_C_re, A_C_im,
      A_log_dt, A_Dskip, B_wqkv, B_wo, *_dft_tables(),
      np.zeros((1,), np.int32))
    return out.reshape(1, L, D)
```
